```python
import jax
import jax.numpy as jnp

def _softmax(x, axis=-1):
    return jax.nn.softmax(x, axis=axis)

def _gelu(x):
    return jax.nn.gelu(x, approximate=True)

def _silu(x):
    return jax.nn.silu(x)

def _sigmoid(x):
    return jax.nn.sigmoid(x)

def _layernorm(x, axis=-1, eps=1e-05):
    m = jnp.mean(x, axis=axis, keepdims=True)
    v = jnp.var(x, axis=axis, keepdims=True)
    return (x - m) / jnp.sqrt(v + eps)

def _scatter_add(tgt, idx, src, axis=0):
    return tgt.at[idx].add(src)

def _segment_sum(src, seg, n):
    return jax.ops.segment_sum(src, seg, n)

class _Rng:

    def __init__(self, key):
        self._k = key

    def _next(self):
        self._k, sub = jax.random.split(self._k)
        return sub

    def normal(self, shape):
        return jax.random.normal(self._next(), shape, dtype=jnp.bfloat16)

    def randint(self, lo, hi, shape):
        return jax.random.randint(self._next(), shape, lo, hi, dtype=jnp.int32)

    def uniform(self, shape, lo=0.0, hi=1.0):
        return jax.random.uniform(self._next(), shape, jnp.bfloat16, lo, hi)

    def permutation(self, n):
        return jax.random.permutation(self._next(), n)
kernel_name = 'gated_mix__memory_aug_recurrent_mem_tr__moe_arch_mod__prompt'

def setup_inputs():
    _rng = _Rng(jax.random.key(int.from_bytes(__import__("os").urandom(4), "little")))
    _w = lambda a: (lambda t: t.astype(jnp.bfloat16) if jnp.issubdtype(t.dtype, jnp.floating) else t)(jnp.asarray(a))

    def _A_setup():
        B, S, Dm = (1, 2048, 1024)
        H, Dh = (32, 128)
        M, seg = (8, 32)
        seg = min(seg, S)
        S = S // seg * seg
        return {'x': _w((lambda *s: _rng.normal(s) * 0.05)(B, S, Dm)), 'mem0': _w((lambda *s: _rng.normal(s) * 0.05)(B, M, Dm)), 'Wq': _w((lambda *s: _rng.normal(s) * 0.05)(Dm, H, Dh) * Dm ** (-0.5)), 'Wk': _w((lambda *s: _rng.normal(s) * 0.05)(Dm, H, Dh) * Dm ** (-0.5)), 'Wv': _w((lambda *s: _rng.normal(s) * 0.05)(Dm, H, Dh) * Dm ** (-0.5)), 'Wo': _w((lambda *s: _rng.normal(s) * 0.05)(H, Dh, Dm) * (H * Dh) ** (-0.5)), 'seg_len': seg}
    _A_in = _A_setup()

    def _B_setup():
        B, S, D, F, C = (1, 2048, 1024, 3584, 8)
        return {'x': _w((lambda *s: _rng.normal(s) * 0.05)(B, S, D)), 'w_r': _w((lambda *s: _rng.normal(s) * 0.05)(D)), 'w_gate': _w((lambda *s: _rng.normal(s) * 0.05)(D, F)), 'w_up': _w((lambda *s: _rng.normal(s) * 0.05)(D, F)), 'w_down': _w((lambda *s: _rng.normal(s) * 0.05)(F, D))}
    _B_in = _B_setup()
    return {'A_x': _A_in['x'], 'A_mem0': _A_in['mem0'], 'A_Wq': _A_in['Wq'], 'A_Wk': _A_in['Wk'], 'A_Wv': _A_in['Wv'], 'A_Wo': _A_in['Wo'], 'A_seg_len': _A_in['seg_len'], 'B_x': _B_in['x'], 'B_w_r': _B_in['w_r'], 'B_w_gate': _B_in['w_gate'], 'B_w_up': _B_in['w_up'], 'B_w_down': _B_in['w_down'], 'gate_w': _w((lambda *s: _rng.normal(s) * 0.05)(1024))}

def reference(A_x, A_mem0, A_Wq, A_Wk, A_Wv, A_Wo, A_seg_len, B_x, B_w_r, B_w_gate, B_w_up, B_w_down, gate_w):

    def _A_ref(x, mem0, Wq, Wk, Wv, Wo, seg_len):
        B, S, Dm = x.shape
        H, Dh = (Wq.shape[1], Wq.shape[2])
        M = mem0.shape[1]
        scale = Dh ** (-0.5)
        n_seg = S // seg_len
        L = M + seg_len
        idx = jnp.arange(L)
        mask = (idx[:, None] < M) | (idx[:, None] >= idx[None, :])
        mem = mem0
        outs = []
        for s in range(n_seg):
            xs = x[:, s * seg_len:(s + 1) * seg_len, :].copy()
            h = jnp.concatenate([mem, xs], axis=1)
            q = jnp.einsum('btd,dhe->bhte', h, Wq)
            k = jnp.einsum('btd,dhe->bhte', h, Wk)
            v = jnp.einsum('btd,dhe->bhte', h, Wv)
            scores = jnp.einsum('bhqe,bhke->bhqk', q, k) * scale
            scores = jnp.where(mask[None, None], scores, -1000000000.0)
            p = _softmax(scores, axis=-1)
            o = jnp.einsum('bhqk,bhke->bhqe', p, v)
            o = jnp.einsum('bhte,hed->btd', o, Wo)
            mem = o[:, :M, :].copy()
            outs.append(o[:, M:, :])
        return jnp.concatenate(outs, axis=1)

    def _B_ref(x, w_r, w_gate, w_up, w_down):
        B, S, D = x.shape
        C = 8
        r = x @ w_r
        idx = jnp.argsort(-r, axis=-1)[:, :C]
        idx_e = jnp.repeat(idx.reshape(B, C, 1), D, axis=2)
        x_sel = jnp.take_along_axis(x, idx_e, axis=1)
        g = _silu(x_sel @ w_gate)
        u = x_sel @ w_up
        y = g * u @ w_down
        r_sel = _sigmoid(jnp.take_along_axis(r, idx, axis=1))
        y = y * r_sel.reshape(B, C, 1)
        b_off = (jnp.arange(B) * S).reshape(B, 1)
        flat_idx = (idx + b_off).reshape(B * C)
        zero = (x * 0.0).reshape(B * S, D)
        upd = _scatter_add(zero, flat_idx, y.reshape(B * C, D), axis=0)
        return x + upd.reshape(B, S, D)
    x = A_x
    g = _sigmoid((x * gate_w).sum(-1, keepdims=True))
    a = _A_ref(x, A_mem0, A_Wq, A_Wk, A_Wv, A_Wo, A_seg_len)
    b = _B_ref(x, B_w_r, B_w_gate, B_w_up, B_w_down)
    return g * a + (1 - g) * b
```

```python
import functools

import jax
import jax.experimental.pallas as pl
import jax.experimental.pallas.tpu as pltpu
import jax.numpy as jnp
import numpy as np
from jax import lax

_BF16 = jnp.bfloat16
_F32 = jnp.float32
_U32 = jnp.uint32
_LANES = 128
_TOP_C = 8


def _as_bf16(words):
  return pltpu.bitcast(words, _BF16)


def _cat_cols(parts):
  return parts[0] if len(parts) == 1 else jnp.concatenate(parts, axis=1)


def _kernel(
    x_hbm, mem0_ref, wq_hbm, wk_hbm, wv_hbm, wo_hbm, wr_ref, wg_hbm, wu_hbm,
    wd_hbm, gw_ref,
    out_hbm,
    x_s, wqkv_s, wo_s, wg_s, wu_s, wd_s, ring, o_s, a_s, mem_s, y_s, idx_s,
    out_s, sem_x, sem_w, sem_misc, sem_out,
    *, seq, dm, heads, n_mem, seg, ffn, lag_s, lag_pv, o_split,
):
  kt = dm // _LANES
  ft = ffn // _LANES
  n_seg = seq // seg
  n_rows = n_mem + seg
  ride = seg - n_mem
  ahead = seq - n_seg * ride
  ring_rows = ring.shape[1]
  n_pairs = heads // 2
  scale = float(_LANES) ** -0.5
  w_hbms = (wq_hbm, wk_hbm, wv_hbm)

  def x_copy(part, k):
    lo, n = (0, ahead) if part == 0 else (ahead, seq - ahead)
    return pltpu.make_async_copy(
        x_hbm.at[pl.ds(lo, n), pl.ds(k * _LANES, _LANES)],
        x_s.at[k, pl.ds(lo // 2, n // 2)].bitcast(_BF16),
        sem_x.at[part])

  def w_copy(j, m, p):
    return pltpu.make_async_copy(
        w_hbms[m].bitcast(_U32).at[:, p, j], wqkv_s.at[2 * j + p, m],
        sem_w.at[j])

  def col_copy(src, dst, n, sem):
    return pltpu.make_async_copy(
        src.at[:, pl.ds(n * _LANES, _LANES)], dst.at[n].bitcast(_BF16), sem)

  def pair_copies(j):
    return [w_copy(j, m, p) for m in range(3) for p in range(2)]

  gate_up_copies = (
      [col_copy(wg_hbm, wg_s, n, sem_misc.at[0]) for n in range(ft)]
      + [col_copy(wu_hbm, wu_s, n, sem_misc.at[0]) for n in range(ft)])
  down_copies = [col_copy(wd_hbm, wd_s, n, sem_misc.at[1]) for n in range(kt)]
  wo_copies = [col_copy(wo_hbm, wo_s, n, sem_misc.at[2]) for n in range(kt)]

  for k in range(kt):
    x_copy(0, k).start()
  for j in range(n_pairs):
    for cp in pair_copies(j):
      cp.start()
  for k in range(kt):
    x_copy(1, k).start()
  for cp in gate_up_copies + down_copies + wo_copies:
    cp.start()

  for k in range(kt):
    x_copy(0, k).wait()

  def project_ahead(j, carry):
    for cp in pair_copies(j):
      cp.wait()
    for m in range(3):
      even = wqkv_s[2 * j, m]
      odd = wqkv_s[2 * j + 1, m]
      wqkv_s[2 * j, m] = (even & np.uint32(0xFFFF)) | (odd << 16)
      wqkv_s[2 * j + 1, m] = (even >> 16) | (odd & np.uint32(0xFFFF0000))
    xa = _cat_cols([_as_bf16(x_s[k, 0:ahead // 2]) for k in range(kt)])
    for p in range(2):
      for m in range(3):
        w = _as_bf16(wqkv_s[2 * j + p, m])
        ring[3 * (2 * j + p) + m, 0:ahead] = jnp.dot(
            xa, w, preferred_element_type=_F32)
    return carry

  lax.fori_loop(0, n_pairs, project_ahead, 0)

  for k in range(kt):
    x_copy(1, k).wait()
  wr = jnp.broadcast_to(wr_ref[...].astype(_F32), (8, dm))
  sub = lax.broadcasted_iota(jnp.int32, (8, _LANES), 0)
  lane = lax.broadcasted_iota(jnp.int32, (8, _LANES), 1)
  blocks = seq // _LANES
  score = []
  for b in range(blocks):
    xb = _cat_cols([_as_bf16(x_s[k, b * 64:(b + 1) * 64]) for k in range(kt)])
    rb = lax.dot_general(wr, xb, (((1,), (1,)), ((), ())),
                         preferred_element_type=_F32)
    if b % 8 == 0:
      score.append(rb)
    else:
      score[-1] = jnp.where(sub == b % 8, rb, score[-1])
  score = jnp.concatenate(score, axis=0).astype(_BF16).astype(_F32)
  tok = (lax.broadcasted_iota(jnp.int32, score.shape, 0) * _LANES
         + lax.broadcasted_iota(jnp.int32, score.shape, 1)).astype(_F32)
  free = jnp.ones(score.shape, _F32)
  r_sel = jnp.zeros((8, _LANES), _F32)
  x_sel = [jnp.zeros((8, _LANES), _F32) for _ in range(kt)]
  row16 = lax.broadcasted_iota(jnp.int32, (16, _LANES), 0)
  for c in range(_TOP_C):
    cand = jnp.where((free > 0) & (score == score), score, -jnp.inf)
    best = jnp.max(jnp.max(cand, axis=1, keepdims=True), axis=0, keepdims=True)
    hit = jnp.where((free > 0) & (cand == best), tok, float(seq))
    pick = jnp.min(jnp.min(hit, axis=1, keepdims=True), axis=0, keepdims=True)
    chosen = tok == pick
    free = jnp.where(chosen, 0.0, free)
    r_c = jnp.where(chosen, score, 0.0)
    r_c = jnp.sum(jnp.sum(r_c, axis=1, keepdims=True), axis=0, keepdims=True)
    r_sel = jnp.where(sub == c, r_c, r_sel)
    t = jnp.clip(pick.astype(jnp.int32)[0, 0], 0, seq - 1)
    idx_s[c] = t
    base = pl.multiple_of((t // 16) * 8, 8)
    for k in range(kt):
      blk = _as_bf16(x_s[k, pl.ds(base, 8)]).astype(_F32)
      row = jnp.sum(jnp.where(row16 == t % 16, blk, 0.0), axis=0, keepdims=True)
      x_sel[k] = jnp.where(sub == c, row, x_sel[k])
  x_sel = _cat_cols(x_sel)

  for cp in gate_up_copies:
    cp.wait()
  act = []
  for n in range(ft):
    gt = jnp.dot(x_sel, _as_bf16(wg_s[n]), preferred_element_type=_F32)
    up = jnp.dot(x_sel, _as_bf16(wu_s[n]), preferred_element_type=_F32)
    act.append(gt * jax.nn.sigmoid(gt) * up)
  act = _cat_cols(act)
  for cp in down_copies:
    cp.wait()
  r_gate = jax.nn.sigmoid(r_sel)
  for n in range(kt):
    y = jnp.dot(act, _as_bf16(wd_s[n]), preferred_element_type=_F32) * r_gate
    for c in range(_TOP_C):
      y_s[c, :, n * _LANES:(n + 1) * _LANES] = jnp.broadcast_to(
          y[c:c + 1], (8, _LANES))

  n_keys = -(-n_rows // 16) * 16
  qi = lax.broadcasted_iota(jnp.int32, (n_rows, n_keys), 0)
  ki = lax.broadcasted_iota(jnp.int32, (n_rows, n_keys), 1)
  visible = ((qi < n_mem) | (qi >= ki)) & (ki < n_rows)
  hidden = jnp.where(ki < n_rows, -1e9, -jnp.inf).astype(_F32)
  key_pad = jnp.zeros((n_keys - n_rows, _LANES), _F32)

  mem_s[...] = mem0_ref[...].astype(_F32)
  a_s[...] = jnp.zeros(a_s.shape, _F32)

  def finish(t):
    row0 = pl.multiple_of(t * seg, seg)
    word0 = pl.multiple_of(t * (seg // 2), seg // 2)
    xt = _cat_cols(
        [_as_bf16(x_s[k, pl.ds(word0, seg // 2)]) for k in range(kt)]
    ).astype(_F32)
    g = jax.nn.sigmoid(
        jnp.sum(xt * gw_ref[...].astype(_F32), axis=-1, keepdims=True))
    tok_id = lax.broadcasted_iota(jnp.int32, (8, dm), 0)
    upd = []
    for i in range(seg // 8):
      u = jnp.zeros((8, dm), _F32)
      for c in range(_TOP_C):
        u = jnp.where(tok_id == idx_s[c] - row0 - 8 * i, y_s[c], u)
      upd.append(u)
    b = xt + jnp.concatenate(upd, axis=0)
    out_s[pl.ds(row0, seg), :] = (g * a_s[...] + (1.0 - g) * b).astype(_BF16)

  def out_copy(t):
    rows = pl.ds(pl.multiple_of(t * seg, seg), seg)
    return pltpu.make_async_copy(out_s.at[rows], out_hbm.at[rows], sem_out)

  def step(s, carry):
    @pl.when(s >= 2)
    def _():
      out_copy(s - 2).start()

    word0 = (ahead + s * ride - n_mem) // 2
    lhs = []
    for k in range(kt):
      xw = x_s[k, pl.ds(word0, seg // 2)]
      mk = mem_s[:, k * _LANES:(k + 1) * _LANES]
      mw = pltpu.bitcast(
          jnp.concatenate([mk, jnp.zeros_like(mk)], axis=0).astype(_BF16), _U32)
      head = jnp.where(sub < n_mem // 2, mw, xw[0:8])
      lhs.append(_as_bf16(jnp.concatenate([head, xw[8:]], axis=0)))
    lhs = _cat_cols(lhs)
    put = [pl.multiple_of(lax.rem(ahead + s * ride + 8 * i, ring_rows), 8)
           for i in range(ride // 8)]
    get = pl.multiple_of(lax.rem(s * seg, ring_rows), 8)

    qkv, probs = {}, {}

    def project(h):
      w = _cat_cols([_as_bf16(wqkv_s[h, m]) for m in range(3)])
      r = jnp.dot(lhs, w, preferred_element_type=_F32)
      parts = [r[:, m * _LANES:(m + 1) * _LANES] for m in range(3)]
      for m in range(3):
        for i in range(ride // 8):
          lo = n_mem + 8 * i
          ring[3 * h + m, pl.ds(put[i], 8)] = parts[m][lo:lo + 8]
      rows = [[parts[m][0:n_mem], ring[3 * h + m, pl.ds(get, seg)]]
              for m in range(3)]
      qkv[h] = (
          jnp.concatenate(rows[0], axis=0),
          jnp.concatenate(rows[1] + [key_pad], axis=0).astype(_BF16),
          jnp.concatenate(rows[2] + [key_pad], axis=0).astype(_BF16))

    def attend_scores(h):
      q, k, _ = qkv[h]
      sc = lax.dot_general(q, k, (((1,), (1,)), ((), ())),
                           preferred_element_type=_F32)
      sc = jnp.where(visible, sc * scale, hidden)
      p = jnp.exp(sc - jnp.max(sc, axis=-1, keepdims=True))
      probs[h] = (p, jnp.sum(p, axis=-1, keepdims=True))

    def attend_values(h):
      p, denom = probs[h]
      o = jnp.dot(p, qkv[h][2], preferred_element_type=_F32)
      o_s[:, h * _LANES:(h + 1) * _LANES] = o / denom

    k_part = heads * _LANES // o_split
    acc = [None]

    def out_project(i):
      w = _cat_cols([
          _as_bf16(wo_s[n, i * k_part // 2:(i + 1) * k_part // 2])
          for n in range(kt)])
      r = jnp.dot(o_s[:, i * k_part:(i + 1) * k_part], w,
                  preferred_element_type=_F32)
      acc[0] = r if acc[0] is None else acc[0] + r

    done = 0
    for h in range(heads + lag_pv):
      if h < heads:
        project(h)
      elif done < o_split - 1:
        out_project(done)
        done += 1
      if 0 <= h - lag_s < heads:
        attend_scores(h - lag_s)
      if 0 <= h - lag_pv < heads:
        attend_values(h - lag_pv)
      if h == 4:
        finish(jnp.maximum(s - 1, 0))
    while done < o_split:
      out_project(done)
      done += 1
    mem_s[...] = acc[0][0:n_mem]
    a_s[...] = acc[0][n_mem:]
    return carry

  for cp in wo_copies:
    cp.wait()
  lax.fori_loop(0, n_seg, step, 0)

  out_copy(n_seg - 2).start()
  finish(n_seg - 1)
  out_copy(n_seg - 1).start()
  pltpu.make_async_copy(out_s, out_hbm, sem_out).wait()


@functools.partial(jax.jit, static_argnames=("A_seg_len",))
def pallas_gated_mix__memory_aug_recurrent_mem_tr__moe_arch_mod__prompt_kernel(
    A_x: jax.Array,
    A_mem0: jax.Array,
    A_Wq: jax.Array,
    A_Wk: jax.Array,
    A_Wv: jax.Array,
    A_Wo: jax.Array,
    A_seg_len: int,
    B_x: jax.Array,
    B_w_r: jax.Array,
    B_w_gate: jax.Array,
    B_w_up: jax.Array,
    B_w_down: jax.Array,
    gate_w: jax.Array,
):
  del B_x
  batch, seq, dm = A_x.shape
  _, heads, dh = A_Wq.shape
  n_mem = A_mem0.shape[1]
  ffn = B_w_gate.shape[1]
  seg = int(A_seg_len)
  assert batch == 1 and dh == _LANES and (n_mem, seg) == (8, 32)
  kt, ft = dm // _LANES, ffn // _LANES
  ahead = seq - (seq // seg) * (seg - n_mem)
  ring_rows = -(-(ahead + seg) // seg) * seg

  hbm = pl.BlockSpec(memory_space=pl.ANY)
  vmem = pl.BlockSpec(memory_space=pltpu.VMEM)
  kernel = functools.partial(
      _kernel, seq=seq, dm=dm, heads=heads, n_mem=n_mem, seg=seg, ffn=ffn,
      lag_s=2, lag_pv=4, o_split=4)
  out = pl.pallas_call(
      kernel,
      out_shape=jax.ShapeDtypeStruct((seq, dm), A_x.dtype),
      in_specs=[hbm, vmem, hbm, hbm, hbm, hbm, vmem, hbm, hbm, hbm, vmem],
      out_specs=hbm,
      scratch_shapes=[
          pltpu.VMEM((kt, seq // 2, _LANES), _U32),
          pltpu.VMEM((heads, 3, dm // 2, _LANES), _U32),
          pltpu.VMEM((kt, heads * dh // 2, _LANES), _U32),
          pltpu.VMEM((ft, dm // 2, _LANES), _U32),
          pltpu.VMEM((ft, dm // 2, _LANES), _U32),
          pltpu.VMEM((kt, ffn // 2, _LANES), _U32),
          pltpu.VMEM((3 * heads, ring_rows, _LANES), _F32),
          pltpu.VMEM((n_mem + seg, heads * dh), _F32),
          pltpu.VMEM((seg, dm), _F32),
          pltpu.VMEM((n_mem, dm), _F32),
          pltpu.VMEM((_TOP_C, 8, dm), _F32),
          pltpu.SMEM((_TOP_C,), jnp.int32),
          pltpu.VMEM((seq, dm), _BF16),
          pltpu.SemaphoreType.DMA((2,)),
          pltpu.SemaphoreType.DMA((heads // 2,)),
          pltpu.SemaphoreType.DMA((3,)),
          pltpu.SemaphoreType.DMA,
      ],
      compiler_params=pltpu.CompilerParams(vmem_limit_bytes=120 * 2**20),
      name="gated_rmt_mod",
  )(
      A_x.reshape(seq, dm),
      A_mem0.reshape(n_mem, dm),
      A_Wq.reshape(dm // 2, 2, heads, dh),
      A_Wk.reshape(dm // 2, 2, heads, dh),
      A_Wv.reshape(dm // 2, 2, heads, dh),
      A_Wo.reshape(heads * dh, dm),
      B_w_r.reshape(1, dm),
      B_w_gate,
      B_w_up,
      B_w_down,
      gate_w.reshape(1, dm),
  )
  return out.reshape(batch, seq, dm)
```

```python
import functools

import jax
import jax.experimental.pallas as pl
import jax.experimental.pallas.tpu as pltpu
import jax.numpy as jnp
import numpy as np
from jax import lax

_BF16 = jnp.bfloat16
_F32 = jnp.float32
_U32 = jnp.uint32
_LANES = 128
_TOP_C = 8


def _as_bf16(words):
  return pltpu.bitcast(words, _BF16)


def _cat_cols(parts):
  return parts[0] if len(parts) == 1 else jnp.concatenate(parts, axis=1)


def _kernel(
    x_hbm, mem0_ref, wq_hbm, wk_hbm, wv_hbm, wo_hbm, wr_ref, wg_hbm, wu_hbm,
    wd_hbm, gw_ref,
    out_hbm,
    x_s, wqkv_s, wo_s, wg_s, wu_s, wd_s, ring, o_s, a_s, mem_s, y_s, idx_s,
    out_s, sem_x, sem_w, sem_misc, sem_out,
    *, seq, dm, heads, n_mem, seg, ffn, lag_s, lag_pv, o_split,
):
  kt = dm // _LANES
  ft = ffn // _LANES
  n_seg = seq // seg
  n_rows = n_mem + seg
  ride = seg - n_mem
  ahead = seq - n_seg * ride
  ring_rows = ring.shape[1]
  n_pairs = heads // 2
  scale = float(_LANES) ** -0.5
  w_hbms = (wq_hbm, wk_hbm, wv_hbm)

  def cols(n):
    return pl.ds(pl.multiple_of(n * _LANES, _LANES), _LANES)

  def x_copy(part, k):
    lo, n = (0, ahead) if part == 0 else (ahead, seq - ahead)
    return pltpu.make_async_copy(
        x_hbm.at[pl.ds(lo, n), cols(k)],
        x_s.at[k, pl.ds(lo // 2, n // 2)].bitcast(_BF16),
        sem_x.at[part])

  def pair_copies(j):
    return [
        pltpu.make_async_copy(
            w_hbms[m].bitcast(_U32).at[:, p, j], wqkv_s.at[2 * j + p, m],
            sem_w.at[j])
        for m in range(3) for p in range(2)]

  def col_copy(src, dst, n, sem):
    return pltpu.make_async_copy(
        src.at[:, cols(n)], dst.at[n].bitcast(_BF16), sem)

  wo_copy = lambda n: col_copy(wo_hbm, wo_s, n, sem_misc.at[0])
  wg_copy = lambda n: col_copy(wg_hbm, wg_s, n, sem_misc.at[1])
  wu_copy = lambda n: col_copy(wu_hbm, wu_s, n, sem_misc.at[1])
  wd_copy = lambda n: col_copy(wd_hbm, wd_s, n, sem_misc.at[2])

  def start_all(copies):
    for cp in copies:
      cp.start()

  def wait_all(copies):
    for cp in copies:
      cp.wait()

  def prefetch(j):
    half = n_pairs // 2 - 1

    @pl.when(j < half)
    def _():
      start_all(pair_copies(2 * j + 2) + pair_copies(2 * j + 3))

    @pl.when(j == half)
    def _():
      start_all([x_copy(1, k) for k in range(kt)])

    i = j - (half + 1)

    @pl.when((i >= 0) & (i < kt // 2))
    def _():
      start_all([wo_copy(2 * i), wo_copy(2 * i + 1)])

    i2 = i - kt // 2
    per = ft // 4

    @pl.when(i2 >= 0)
    def _():
      start_all([wg_copy(per * i2 + n) for n in range(per)]
                + [wu_copy(per * i2 + n) for n in range(per)])

  start_all([x_copy(0, k) for k in range(kt)] + pair_copies(0) + pair_copies(1))

  wait_all([x_copy(0, k) for k in range(kt)])

  def project_ahead(j, carry):
    wait_all(pair_copies(j))
    prefetch(j)
    for m in range(3):
      even = wqkv_s[2 * j, m]
      odd = wqkv_s[2 * j + 1, m]
      wqkv_s[2 * j, m] = (even & np.uint32(0xFFFF)) | (odd << 16)
      wqkv_s[2 * j + 1, m] = (even >> 16) | (odd & np.uint32(0xFFFF0000))
    xa = _cat_cols([_as_bf16(x_s[k, 0:ahead // 2]) for k in range(kt)])
    for p in range(2):
      for m in range(3):
        w = _as_bf16(wqkv_s[2 * j + p, m])
        ring[3 * (2 * j + p) + m, 0:ahead] = jnp.dot(
            xa, w, preferred_element_type=_F32)
    return carry

  lax.fori_loop(0, n_pairs, project_ahead, 0)
  start_all([wd_copy(n) for n in range(kt)])

  sub = lax.broadcasted_iota(jnp.int32, (8, _LANES), 0)

  def routed_ffn():
    wr = jnp.broadcast_to(wr_ref[...].astype(_F32), (8, dm))
    blocks = seq // _LANES
    score = []
    for b in range(blocks):
      xb = _cat_cols([_as_bf16(x_s[k, b * 64:(b + 1) * 64]) for k in range(kt)])
      rb = lax.dot_general(wr, xb, (((1,), (1,)), ((), ())),
                           preferred_element_type=_F32)
      if b % 8 == 0:
        score.append(rb)
      else:
        score[-1] = jnp.where(sub == b % 8, rb, score[-1])
    score = jnp.concatenate(score, axis=0).astype(_BF16).astype(_F32)
    tok = (lax.broadcasted_iota(jnp.int32, score.shape, 0) * _LANES
           + lax.broadcasted_iota(jnp.int32, score.shape, 1)).astype(_F32)
    free = jnp.ones(score.shape, _F32)
    r_sel = jnp.zeros((8, _LANES), _F32)
    x_sel = [jnp.zeros((8, _LANES), _F32) for _ in range(kt)]
    row16 = lax.broadcasted_iota(jnp.int32, (16, _LANES), 0)
    for c in range(_TOP_C):
      cand = jnp.where((free > 0) & (score == score), score, -jnp.inf)
      best = jnp.max(jnp.max(cand, axis=1, keepdims=True), axis=0, keepdims=True)
      hit = jnp.where((free > 0) & (cand == best), tok, float(seq))
      pick = jnp.min(jnp.min(hit, axis=1, keepdims=True), axis=0, keepdims=True)
      chosen = tok == pick
      free = jnp.where(chosen, 0.0, free)
      r_c = jnp.where(chosen, score, 0.0)
      r_c = jnp.sum(jnp.sum(r_c, axis=1, keepdims=True), axis=0, keepdims=True)
      r_sel = jnp.where(sub == c, r_c, r_sel)
      t = jnp.clip(pick.astype(jnp.int32)[0, 0], 0, seq - 1)
      idx_s[c] = t
      base = pl.multiple_of((t // 16) * 8, 8)
      for k in range(kt):
        blk = _as_bf16(x_s[k, pl.ds(base, 8)]).astype(_F32)
        row = jnp.sum(jnp.where(row16 == t % 16, blk, 0.0), axis=0, keepdims=True)
        x_sel[k] = jnp.where(sub == c, row, x_sel[k])
    x_sel = _cat_cols(x_sel)

    wait_all([wg_copy(n) for n in range(ft)] + [wu_copy(n) for n in range(ft)])
    act = []
    for n in range(ft):
      gt = jnp.dot(x_sel, _as_bf16(wg_s[n]), preferred_element_type=_F32)
      up = jnp.dot(x_sel, _as_bf16(wu_s[n]), preferred_element_type=_F32)
      act.append(gt * jax.nn.sigmoid(gt) * up)
    act = _cat_cols(act)
    wait_all([wd_copy(n) for n in range(kt)])
    r_gate = jax.nn.sigmoid(r_sel)
    for n in range(kt):
      y = jnp.dot(act, _as_bf16(wd_s[n]), preferred_element_type=_F32) * r_gate
      for c in range(_TOP_C):
        y_s[c, :, n * _LANES:(n + 1) * _LANES] = jnp.broadcast_to(
            y[c:c + 1], (8, _LANES))

  n_keys = -(-n_rows // 16) * 16
  qi = lax.broadcasted_iota(jnp.int32, (n_rows, n_keys), 0)
  ki = lax.broadcasted_iota(jnp.int32, (n_rows, n_keys), 1)
  visible = ((qi < n_mem) | (qi >= ki)) & (ki < n_rows)
  hidden = jnp.where(ki < n_rows, -1e9, -jnp.inf).astype(_F32)
  key_pad = jnp.zeros((n_keys - n_rows, _LANES), _F32)

  mem_s[...] = mem0_ref[...].astype(_F32)
  a_s[...] = jnp.zeros(a_s.shape, _F32)
  y_s[...] = jnp.zeros(y_s.shape, _F32)
  for c in range(_TOP_C):
    idx_s[c] = 0

  def finish(t):
    row0 = pl.multiple_of(t * seg, seg)
    word0 = pl.multiple_of(t * (seg // 2), seg // 2)
    xt = _cat_cols(
        [_as_bf16(x_s[k, pl.ds(word0, seg // 2)]) for k in range(kt)]
    ).astype(_F32)
    g = jax.nn.sigmoid(
        jnp.sum(xt * gw_ref[...].astype(_F32), axis=-1, keepdims=True))
    tok_id = lax.broadcasted_iota(jnp.int32, (8, dm), 0)
    upd = []
    for i in range(seg // 8):
      u = jnp.zeros((8, dm), _F32)
      for c in range(_TOP_C):
        u = jnp.where(tok_id == idx_s[c] - row0 - 8 * i, y_s[c], u)
      upd.append(u)
    b = xt + jnp.concatenate(upd, axis=0)
    out_s[pl.ds(row0, seg), :] = (g * a_s[...] + (1.0 - g) * b).astype(_BF16)

  def out_copy(t):
    rows = pl.ds(pl.multiple_of(t * seg, seg), seg)
    return pltpu.make_async_copy(out_s.at[rows], out_hbm.at[rows], sem_out)

  def step(s, carry):
    @pl.when(s >= 2)
    def _():
      out_copy(s - 2).start()

    pl.when(s == 1)(routed_ffn)

    word0 = (ahead + s * ride - n_mem) // 2
    lhs = []
    for k in range(kt):
      xw = x_s[k, pl.ds(word0, seg // 2)]
      mk = mem_s[:, k * _LANES:(k + 1) * _LANES]
      mw = pltpu.bitcast(
          jnp.concatenate([mk, jnp.zeros_like(mk)], axis=0).astype(_BF16), _U32)
      head = jnp.where(sub < n_mem // 2, mw, xw[0:8])
      lhs.append(_as_bf16(jnp.concatenate([head, xw[8:]], axis=0)))
    lhs = _cat_cols(lhs)
    put = [pl.multiple_of(lax.rem(ahead + s * ride + 8 * i, ring_rows), 8)
           for i in range(ride // 8)]
    get = pl.multiple_of(lax.rem(s * seg, ring_rows), 8)

    qkv, probs = {}, {}

    def project(h):
      w = _cat_cols([_as_bf16(wqkv_s[h, m]) for m in range(3)])
      r = jnp.dot(lhs, w, preferred_element_type=_F32)
      parts = [r[:, m * _LANES:(m + 1) * _LANES] for m in range(3)]
      for m in range(3):
        for i in range(ride // 8):
          lo = n_mem + 8 * i
          ring[3 * h + m, pl.ds(put[i], 8)] = parts[m][lo:lo + 8]
      rows = [[parts[m][0:n_mem], ring[3 * h + m, pl.ds(get, seg)]]
              for m in range(3)]
      qkv[h] = (
          jnp.concatenate(rows[0], axis=0),
          jnp.concatenate(rows[1] + [key_pad], axis=0).astype(_BF16),
          jnp.concatenate(rows[2] + [key_pad], axis=0).astype(_BF16))

    def attend_scores(h):
      q, k, _ = qkv[h]
      sc = lax.dot_general(q, k, (((1,), (1,)), ((), ())),
                           preferred_element_type=_F32)
      sc = jnp.where(visible, sc * scale, hidden)
      p = jnp.exp(sc - jnp.max(sc, axis=-1, keepdims=True))
      probs[h] = (p, jnp.sum(p, axis=-1, keepdims=True))

    def attend_values(h):
      p, denom = probs[h]
      o = jnp.dot(p, qkv[h][2], preferred_element_type=_F32)
      o_s[:, h * _LANES:(h + 1) * _LANES] = o / denom

    k_part = heads * _LANES // o_split
    acc = [None]

    def out_project(i):
      w = _cat_cols([
          _as_bf16(wo_s[n, i * k_part // 2:(i + 1) * k_part // 2])
          for n in range(kt)])
      r = jnp.dot(o_s[:, i * k_part:(i + 1) * k_part], w,
                  preferred_element_type=_F32)
      acc[0] = r if acc[0] is None else acc[0] + r

    done = 0
    for h in range(heads + lag_pv):
      if h < heads:
        project(h)
      elif done < o_split - 1:
        out_project(done)
        done += 1
      if 0 <= h - lag_s < heads:
        attend_scores(h - lag_s)
      if 0 <= h - lag_pv < heads:
        attend_values(h - lag_pv)
      if h == 4:
        finish(jnp.maximum(s - 1, 0))
    while done < o_split:
      out_project(done)
      done += 1
    mem_s[...] = acc[0][0:n_mem]
    a_s[...] = acc[0][n_mem:]
    return carry

  wait_all([x_copy(1, k) for k in range(kt)])
  wait_all([wo_copy(n) for n in range(kt)])
  lax.fori_loop(0, n_seg, step, 0)

  out_copy(n_seg - 2).start()
  finish(n_seg - 1)
  out_copy(n_seg - 1).start()
  pltpu.make_async_copy(out_s, out_hbm, sem_out).wait()


@functools.partial(jax.jit, static_argnames=("A_seg_len",))
def pallas_gated_mix__memory_aug_recurrent_mem_tr__moe_arch_mod__prompt_kernel(
    A_x: jax.Array,
    A_mem0: jax.Array,
    A_Wq: jax.Array,
    A_Wk: jax.Array,
    A_Wv: jax.Array,
    A_Wo: jax.Array,
    A_seg_len: int,
    B_x: jax.Array,
    B_w_r: jax.Array,
    B_w_gate: jax.Array,
    B_w_up: jax.Array,
    B_w_down: jax.Array,
    gate_w: jax.Array,
):
  del B_x
  batch, seq, dm = A_x.shape
  _, heads, dh = A_Wq.shape
  n_mem = A_mem0.shape[1]
  ffn = B_w_gate.shape[1]
  seg = int(A_seg_len)
  assert batch == 1 and dh == _LANES and (n_mem, seg) == (8, 32)
  kt, ft = dm // _LANES, ffn // _LANES
  ahead = seq - (seq // seg) * (seg - n_mem)
  ring_rows = -(-(ahead + seg) // seg) * seg

  hbm = pl.BlockSpec(memory_space=pl.ANY)
  vmem = pl.BlockSpec(memory_space=pltpu.VMEM)
  kernel = functools.partial(
      _kernel, seq=seq, dm=dm, heads=heads, n_mem=n_mem, seg=seg, ffn=ffn,
      lag_s=2, lag_pv=4, o_split=4)
  out = pl.pallas_call(
      kernel,
      out_shape=jax.ShapeDtypeStruct((seq, dm), A_x.dtype),
      in_specs=[hbm, vmem, hbm, hbm, hbm, hbm, vmem, hbm, hbm, hbm, vmem],
      out_specs=hbm,
      scratch_shapes=[
          pltpu.VMEM((kt, seq // 2, _LANES), _U32),
          pltpu.VMEM((heads, 3, dm // 2, _LANES), _U32),
          pltpu.VMEM((kt, heads * dh // 2, _LANES), _U32),
          pltpu.VMEM((ft, dm // 2, _LANES), _U32),
          pltpu.VMEM((ft, dm // 2, _LANES), _U32),
          pltpu.VMEM((kt, ffn // 2, _LANES), _U32),
          pltpu.VMEM((3 * heads, ring_rows, _LANES), _F32),
          pltpu.VMEM((n_mem + seg, heads * dh), _F32),
          pltpu.VMEM((seg, dm), _F32),
          pltpu.VMEM((n_mem, dm), _F32),
          pltpu.VMEM((_TOP_C, 8, dm), _F32),
          pltpu.SMEM((_TOP_C,), jnp.int32),
          pltpu.VMEM((seq, dm), _BF16),
          pltpu.SemaphoreType.DMA((2,)),
          pltpu.SemaphoreType.DMA((heads // 2,)),
          pltpu.SemaphoreType.DMA((3,)),
          pltpu.SemaphoreType.DMA,
      ],
      compiler_params=pltpu.CompilerParams(vmem_limit_bytes=120 * 2**20),
      name="gated_rmt_mod",
  )(
      A_x.reshape(seq, dm),
      A_mem0.reshape(n_mem, dm),
      A_Wq.reshape(dm // 2, 2, heads, dh),
      A_Wk.reshape(dm // 2, 2, heads, dh),
      A_Wv.reshape(dm // 2, 2, heads, dh),
      A_Wo.reshape(heads * dh, dm),
      B_w_r.reshape(1, dm),
      B_w_gate,
      B_w_up,
      B_w_down,
      gate_w.reshape(1, dm),
  )
  return out.reshape(batch, seq, dm)
```

```python
import functools

import jax
import jax.experimental.pallas as pl
import jax.experimental.pallas.tpu as pltpu
import jax.numpy as jnp
import numpy as np
from jax import lax

_BF16 = jnp.bfloat16
_F32 = jnp.float32
_U32 = jnp.uint32
_LANES = 128
_TOP_C = 8


def _as_bf16(words):
  return pltpu.bitcast(words, _BF16)


def _cat_cols(parts):
  return parts[0] if len(parts) == 1 else jnp.concatenate(parts, axis=1)


def _block(n):
  return slice(n * _LANES, (n + 1) * _LANES)


def _dot(a, b):
  return jnp.dot(a, b, preferred_element_type=_F32)


def _reduce_all(op, a):
  return op(op(a, axis=1, keepdims=True), axis=0, keepdims=True)


def _kernel(
    x_hbm, mem0_ref, wq_hbm, wk_hbm, wv_hbm, wo_hbm, wr_ref, wg_hbm, wu_hbm,
    wd_hbm, gw_ref,
    out_hbm,
    x_s, wqkv_s, wo_s, wg_s, wu_s, wd_s, ring, o_s, mem_s, g_s, mix_s, score_s,
    free_s, rsel_s, xsel_s, idx_s, out_s, sem_x, sem_w, sem_misc, sem_out,
    *, seq, dm, heads, n_mem, seg, ffn, lag_s, lag_pv, o_split, unroll, k_first,
):
  kt = dm // _LANES
  ft = ffn // _LANES
  n_seg = seq // seg
  n_rows = n_mem + seg
  ride = seg - n_mem
  ahead = seq - n_seg * ride
  ring_rows = ring.shape[1]
  n_pairs = heads // 2
  half = n_pairs // 2
  scale = float(_LANES) ** -0.5
  w_hbms = (wq_hbm, wk_hbm, wv_hbm)
  sub = lax.broadcasted_iota(jnp.int32, (8, _LANES), 0)
  lane = lax.broadcasted_iota(jnp.int32, (8, _LANES), 1)

  def cols(n):
    return pl.ds(pl.multiple_of(n * _LANES, _LANES), _LANES)

  def x_copies(part):
    lo, n = (0, ahead) if part == 0 else (ahead, seq - ahead)
    return [
        pltpu.make_async_copy(
            x_hbm.at[pl.ds(lo, n), cols(k)],
            x_s.at[k, pl.ds(lo // 2, n // 2)].bitcast(_BF16),
            sem_x.at[part])
        for k in range(kt)]

  def pair_copies(j):
    return [
        pltpu.make_async_copy(
            w_hbms[m].bitcast(_U32).at[:, p, j], wqkv_s.at[2 * j + p, m],
            sem_w.at[j])
        for m in range(3) for p in range(2)]

  def col_copy(src, dst, n, sem):
    return pltpu.make_async_copy(
        src.at[:, cols(n)], dst.at[n].bitcast(_BF16), sem)

  wo_copy = lambda n: col_copy(wo_hbm, wo_s, n, sem_misc.at[0])
  wg_copy = lambda n: col_copy(wg_hbm, wg_s, n, sem_misc.at[1])
  wu_copy = lambda n: col_copy(wu_hbm, wu_s, n, sem_misc.at[1])
  wd_copy = lambda n: col_copy(wd_hbm, wd_s, n, sem_misc.at[2])

  def start_all(copies):
    for cp in copies:
      cp.start()

  def wait_all(copies):
    for cp in copies:
      cp.wait()

  start_all(x_copies(0) + pair_copies(0) + pair_copies(1) + x_copies(1)
            + pair_copies(2))

  def project_ahead(j):
    for m in range(3):
      even = wqkv_s[2 * j, m]
      odd = wqkv_s[2 * j + 1, m]
      wqkv_s[2 * j, m] = (even & np.uint32(0xFFFF)) | (odd << 16)
      wqkv_s[2 * j + 1, m] = (even >> 16) | (odd & np.uint32(0xFFFF0000))
    xa = _cat_cols([_as_bf16(x_s[k, 0:ahead // 2]) for k in range(kt)])
    for p in range(2):
      for m in range(3):
        ring[3 * (2 * j + p) + m, 0:ahead] = _dot(
            xa, _as_bf16(wqkv_s[2 * j + p, m]))

  def gate_and_score(j):
    n = seq // half
    gw = gw_ref[...].astype(_F32)
    wr = wr_ref[...].astype(_F32)
    page = pl.ds(pl.multiple_of((j * n) // (8 * _LANES) * 8, 8), 8)
    lane0 = lax.rem(j * (n // 8), _LANES)
    score = score_s[page]
    for i in range(n // 16):
      words = pl.ds(pl.multiple_of(j * (n // 2) + 8 * i, 8), 8)
      rows = pl.ds(pl.multiple_of(j * n + 16 * i, 16), 16)
      xs = [_as_bf16(x_s[k, words]).astype(_F32) for k in range(kt)]
      lg = functools.reduce(jnp.add, [xs[k] * gw[k:k + 1] for k in range(kt)])
      r = functools.reduce(jnp.add, [xs[k] * wr[k:k + 1] for k in range(kt)])
      g = jax.nn.sigmoid(jnp.sum(lg, axis=-1, keepdims=True))
      r = jnp.sum(r, axis=-1, keepdims=True)
      g_s[rows] = jnp.broadcast_to(g, (16, _LANES))
      for k in range(kt):
        mix_s[k, rows] = (1.0 - g) * xs[k]
      for u in range(2):
        score = jnp.where(lane == lane0 + 2 * i + u, r[8 * u:8 * u + 8], score)
    score_s[page] = score

  def pick_next(c):
    score = score_s[...].astype(_BF16).astype(_F32)
    row = lax.broadcasted_iota(jnp.int32, score.shape, 0)
    col = lax.broadcasted_iota(jnp.int32, score.shape, 1)
    tok = ((row >> 3) * (8 * _LANES) + col * 8 + (row & 7)).astype(_F32)
    free = free_s[...] > 0
    cand = jnp.where(free & (score == score), score, -jnp.inf)
    best = _reduce_all(jnp.max, cand)
    pick = _reduce_all(
        jnp.min, jnp.where(free & (cand == best), tok, float(seq)))
    chosen = tok == pick
    free_s[...] = jnp.where(chosen, 0.0, free_s[...])
    r_c = _reduce_all(jnp.sum, jnp.where(chosen, score, 0.0))
    rsel_s[...] = jnp.where(sub == c, r_c, rsel_s[...])
    t = jnp.clip(pick.astype(jnp.int32)[0, 0], 0, seq - 1)
    idx_s[c] = t
    words = pl.ds(pl.multiple_of((t >> 4) * 8, 8), 8)
    row16 = lax.broadcasted_iota(jnp.int32, (16, _LANES), 0)
    for k in range(kt):
      blk = _as_bf16(x_s[k, words]).astype(_F32)
      xt = jnp.sum(jnp.where(row16 == (t & 15), blk, 0.0), axis=0,
                   keepdims=True)
      xsel_s[:, _block(k)] = jnp.where(sub == c, xt, xsel_s[:, _block(k)])

  def first_half(j, carry):
    wait_all(pair_copies(j))
    pl.when(j == ahead // (seq // half))(lambda: wait_all(x_copies(1)))
    gate_and_score(j)
    project_ahead(j)
    start_all(pair_copies(j + 3) + [wo_copy(j)])
    return carry

  def second_half(i, carry):
    j = half + i
    wait_all(pair_copies(j))
    pick_next(i)
    project_ahead(j)
    pl.when(j + 3 < n_pairs)(lambda: start_all(pair_copies(j + 3)))
    per = -(-ft // half)

    @pl.when(i < ft // per)
    def _():
      start_all([wg_copy(per * i + n) for n in range(per)]
                + [wu_copy(per * i + n) for n in range(per)])

    return carry

  score_s[...] = jnp.zeros(score_s.shape, _F32)
  free_s[...] = jnp.ones(free_s.shape, _F32)
  rsel_s[...] = jnp.zeros(rsel_s.shape, _F32)
  xsel_s[...] = jnp.zeros(xsel_s.shape, _F32)
  mem_s[...] = mem0_ref[...].astype(_F32)
  wait_all(x_copies(0))
  lax.fori_loop(0, half, first_half, 0)
  lax.fori_loop(0, half, second_half, 0)
  start_all([wd_copy(n) for n in range(kt)])

  def routed_ffn():
    x_sel = xsel_s[...]
    wait_all([wg_copy(n) for n in range(ft)] + [wu_copy(n) for n in range(ft)]
             + [wd_copy(n) for n in range(kt)])
    act = []
    for n in range(ft):
      gt = _dot(x_sel, _as_bf16(wg_s[n]))
      act.append(gt * jax.nn.sigmoid(gt) * _dot(x_sel, _as_bf16(wu_s[n])))
    act = _cat_cols(act)
    keep = jnp.zeros((8, _LANES), _F32)
    for c in range(_TOP_C):
      keep = jnp.where(sub == c, 1.0 - g_s[pl.ds(idx_s[c], 1)], keep)
    keep = keep * jax.nn.sigmoid(rsel_s[...])
    for n in range(kt):
      y = _dot(act, _as_bf16(wd_s[n])) * keep
      for c in range(_TOP_C):
        mix_s[n, pl.ds(idx_s[c], 1)] += y[c:c + 1]

  n_keys = -(-n_rows // 16) * 16
  qi = lax.broadcasted_iota(jnp.int32, (n_rows, n_keys), 0)
  ki = lax.broadcasted_iota(jnp.int32, (n_rows, n_keys), 1)
  visible = ((qi < n_mem) | (qi >= ki)) & (ki < n_rows)
  hidden = jnp.where(ki < n_rows, -1e9, -jnp.inf).astype(_F32)
  key_pad = jnp.zeros((n_keys - n_rows, _LANES), _F32)

  def step(s, mem):
    word0 = (ahead - n_mem) // 2 + s * (ride // 2)
    lhs = []
    for k in range(kt):
      xw = x_s[k, pl.ds(word0, seg // 2)]
      mw = pltpu.bitcast(
          jnp.concatenate([mem[k], jnp.zeros_like(mem[k])], axis=0
                          ).astype(_BF16), _U32)
      head = jnp.where(sub < n_mem // 2, mw, xw[0:8])
      lhs.append(_as_bf16(jnp.concatenate([head, xw[8:]], axis=0)))
    put = [pl.multiple_of(lax.rem(ahead + s * ride + 8 * i, ring_rows), 8)
           for i in range(ride // 8)]
    get = pl.multiple_of(lax.rem(s * seg, ring_rows), 8)

    qkv, probs, partial = {}, {}, {}

    def project_part(h, k0, k1):
      words = slice(k0 * _LANES // 2, k1 * _LANES // 2)
      w = _cat_cols([_as_bf16(wqkv_s[h, m, words]) for m in range(3)])
      return _dot(_cat_cols(lhs[k0:k1]), w)

    def project(h):
      if h in partial:
        r = partial[h] + project_part(h, kt // 2, kt)
      else:
        r = project_part(h, 0, kt)
      parts = [r[:, _block(m)] for m in range(3)]
      for m in range(3):
        for i in range(ride // 8):
          lo = n_mem + 8 * i
          ring[3 * h + m, pl.ds(put[i], 8)] = parts[m][lo:lo + 8]
      rows = [[parts[m][0:n_mem], ring[3 * h + m, pl.ds(get, seg)]]
              for m in range(3)]
      qkv[h] = (
          jnp.concatenate(rows[0], axis=0),
          jnp.concatenate(rows[1] + [key_pad], axis=0).astype(_BF16),
          jnp.concatenate(rows[2] + [key_pad], axis=0).astype(_BF16))

    def attend_scores(h):
      q, k, _ = qkv[h]
      sc = lax.dot_general(q, k, (((1,), (1,)), ((), ())),
                           preferred_element_type=_F32)
      sc = jnp.where(visible, sc * scale, hidden)
      p = jnp.exp(sc - jnp.max(sc, axis=-1, keepdims=True))
      probs[h] = (p, jnp.sum(p, axis=-1, keepdims=True))

    def attend_values(h):
      p, denom = probs[h]
      o_s[:, _block(h)] = _dot(p, qkv[h][2]) / denom

    k_part = heads * _LANES // o_split
    acc = [None]

    def out_project(i0, i1):
      w = _cat_cols([
          _as_bf16(wo_s[n, i0 * k_part // 2:i1 * k_part // 2])
          for n in range(kt)])
      r = _dot(o_s[:, i0 * k_part:i1 * k_part], w)
      acc[0] = r if acc[0] is None else acc[0] + r

    for h in range(k_first):
      partial[h] = project_part(h, 0, kt // 2)
    done = 0
    for h in range(heads + lag_pv):
      if h < heads:
        project(h)
      else:
        out_project(done, done + 1)
        done += 1
      if 0 <= h - lag_s < heads:
        attend_scores(h - lag_s)
      if 0 <= h - lag_pv < heads:
        attend_values(h - lag_pv)
    out_project(done, done + 1)
    out_project(done + 1, o_split)

    rows = pl.ds(pl.multiple_of(s * seg, seg), seg)
    g = g_s[rows]
    for k in range(kt):
      mixed = g * acc[0][n_mem:, _block(k)] + mix_s[k, rows]
      mix_s[k, rows] = mixed
      out_s[rows, _block(k)] = mixed.astype(_BF16)
    return [acc[0][0:n_mem, _block(k)] for k in range(kt)]

  span = unroll * seg

  def out_copy(i):
    rows = pl.ds(pl.multiple_of(i * span, span), span)
    return pltpu.make_async_copy(out_s.at[rows], out_hbm.at[rows], sem_out)

  def steps(i, carry):
    @pl.when(i == 1)
    def _():
      routed_ffn()
      for k in range(kt):
        out_s[0:span, _block(k)] = mix_s[k, 0:span].astype(_BF16)

    pl.when(i >= 1)(lambda: out_copy(i - 1).start())
    mem = [mem_s[:, _block(k)] for k in range(kt)]
    for u in range(unroll):
      mem = step(i * unroll + u, mem)
    mem_s[...] = _cat_cols(mem)
    return carry

  wait_all([wo_copy(n) for n in range(kt)])
  lax.fori_loop(0, n_seg // unroll, steps, 0)
  out_copy(n_seg // unroll - 1).start()
  pltpu.make_async_copy(out_s, out_hbm, sem_out).wait()


@functools.partial(jax.jit, static_argnames=("A_seg_len",))
def pallas_gated_mix__memory_aug_recurrent_mem_tr__moe_arch_mod__prompt_kernel(
    A_x: jax.Array,
    A_mem0: jax.Array,
    A_Wq: jax.Array,
    A_Wk: jax.Array,
    A_Wv: jax.Array,
    A_Wo: jax.Array,
    A_seg_len: int,
    B_x: jax.Array,
    B_w_r: jax.Array,
    B_w_gate: jax.Array,
    B_w_up: jax.Array,
    B_w_down: jax.Array,
    gate_w: jax.Array,
):
  del B_x
  batch, seq, dm = A_x.shape
  _, heads, dh = A_Wq.shape
  n_mem = A_mem0.shape[1]
  ffn = B_w_gate.shape[1]
  seg = int(A_seg_len)
  kt, ft = dm // _LANES, ffn // _LANES
  assert batch == 1 and dh == _LANES and (n_mem, seg) == (8, 32)
  assert heads == 4 * _TOP_C == 4 * kt
  ahead = seq - (seq // seg) * (seg - n_mem)
  ring_rows = -(-(ahead + seg) // seg) * seg

  hbm = pl.BlockSpec(memory_space=pl.ANY)
  vmem = pl.BlockSpec(memory_space=pltpu.VMEM)
  kernel = functools.partial(
      _kernel, seq=seq, dm=dm, heads=heads, n_mem=n_mem, seg=seg, ffn=ffn,
      lag_s=3, lag_pv=6, o_split=16, unroll=2, k_first=2)
  out = pl.pallas_call(
      kernel,
      out_shape=jax.ShapeDtypeStruct((seq, dm), A_x.dtype),
      in_specs=[hbm, vmem, hbm, hbm, hbm, hbm, vmem, hbm, hbm, hbm, vmem],
      out_specs=hbm,
      scratch_shapes=[
          pltpu.VMEM((kt, seq // 2, _LANES), _U32),
          pltpu.VMEM((heads, 3, dm // 2, _LANES), _U32),
          pltpu.VMEM((kt, heads * dh // 2, _LANES), _U32),
          pltpu.VMEM((ft, dm // 2, _LANES), _U32),
          pltpu.VMEM((ft, dm // 2, _LANES), _U32),
          pltpu.VMEM((kt, ffn // 2, _LANES), _U32),
          pltpu.VMEM((3 * heads, ring_rows, _LANES), _F32),
          pltpu.VMEM((n_mem + seg, heads * dh), _F32),
          pltpu.VMEM((n_mem, dm), _F32),
          pltpu.VMEM((seq, _LANES), _F32),
          pltpu.VMEM((kt, seq, _LANES), _F32),
          pltpu.VMEM((seq // _LANES, _LANES), _F32),
          pltpu.VMEM((seq // _LANES, _LANES), _F32),
          pltpu.VMEM((_TOP_C, _LANES), _F32),
          pltpu.VMEM((_TOP_C, dm), _F32),
          pltpu.SMEM((_TOP_C,), jnp.int32),
          pltpu.VMEM((seq, dm), _BF16),
          pltpu.SemaphoreType.DMA((2,)),
          pltpu.SemaphoreType.DMA((heads // 2,)),
          pltpu.SemaphoreType.DMA((3,)),
          pltpu.SemaphoreType.DMA,
      ],
      compiler_params=pltpu.CompilerParams(vmem_limit_bytes=120 * 2**20),
      name="gated_rmt_mod",
  )(
      A_x.reshape(seq, dm),
      A_mem0.reshape(n_mem, dm),
      A_Wq.reshape(dm // 2, 2, heads, dh),
      A_Wk.reshape(dm // 2, 2, heads, dh),
      A_Wv.reshape(dm // 2, 2, heads, dh),
      A_Wo.reshape(heads * dh, dm),
      B_w_r.reshape(kt, _LANES),
      B_w_gate,
      B_w_up,
      B_w_down,
      gate_w.reshape(kt, _LANES),
  )
  return out.reshape(batch, seq, dm)
```

```python
import functools

import jax
import jax.experimental.pallas as pl
import jax.experimental.pallas.tpu as pltpu
import jax.numpy as jnp
import numpy as np
from jax import lax

_BF16 = jnp.bfloat16
_F32 = jnp.float32
_U32 = jnp.uint32
_LANES = 128
_TOP_C = 8


def _as_bf16(words):
  return pltpu.bitcast(words, _BF16)


def _cat_cols(parts):
  return parts[0] if len(parts) == 1 else jnp.concatenate(parts, axis=1)


def _block(n):
  return slice(n * _LANES, (n + 1) * _LANES)


def _dot(a, b):
  return jnp.dot(a, b, preferred_element_type=_F32)


def _reduce_all(op, a):
  return op(op(a, axis=1, keepdims=True), axis=0, keepdims=True)


def _kernel(
    x_hbm, mem0_ref, wq_hbm, wk_hbm, wv_hbm, wo_hbm, wr_ref, wg_hbm, wu_hbm,
    wd_hbm, gw_ref,
    out_hbm,
    x_s, wqkv_s, wo_s, wg_s, wu_s, wd_s, ring, o_s, mem_s, g_s, mix_s, score_s,
    part_s, free_s, rsel_s, xsel_s, idx_s, out_s, sem_x, sem_w, sem_misc, sem_out,
    *, seq, dm, heads, n_mem, seg, ffn, lag_s, lag_pv, o_split, unroll, k_first,
    o_gap,
):
  kt = dm // _LANES
  ft = ffn // _LANES
  n_seg = seq // seg
  n_rows = n_mem + seg
  ride = seg - n_mem
  ahead = seq - n_seg * ride
  ring_rows = ring.shape[1]
  n_pairs = heads // 2
  half = n_pairs // 2
  scale = float(_LANES) ** -0.5
  w_hbms = (wq_hbm, wk_hbm, wv_hbm)
  sub = lax.broadcasted_iota(jnp.int32, (8, _LANES), 0)
  lane = lax.broadcasted_iota(jnp.int32, (8, _LANES), 1)

  def cols(n):
    return pl.ds(pl.multiple_of(n * _LANES, _LANES), _LANES)

  def x_copies(part):
    lo, n = (0, ahead) if part == 0 else (ahead, seq - ahead)
    return [
        pltpu.make_async_copy(
            x_hbm.at[pl.ds(lo, n), cols(k)],
            x_s.at[k, pl.ds(lo // 2, n // 2)].bitcast(_BF16),
            sem_x.at[part])
        for k in range(kt)]

  def pair_copies(j):
    return [
        pltpu.make_async_copy(
            w_hbms[m].bitcast(_U32).at[:, p, j], wqkv_s.at[2 * j + p, m],
            sem_w.at[j])
        for m in range(3) for p in range(2)]

  def col_copy(src, dst, n, sem):
    return pltpu.make_async_copy(
        src.at[:, cols(n)], dst.at[n].bitcast(_BF16), sem)

  wo_copy = lambda n: col_copy(wo_hbm, wo_s, n, sem_misc.at[0])
  wg_copy = lambda n: col_copy(wg_hbm, wg_s, n, sem_misc.at[1])
  wu_copy = lambda n: col_copy(wu_hbm, wu_s, n, sem_misc.at[1])
  wd_copy = lambda n: col_copy(wd_hbm, wd_s, n, sem_misc.at[2])

  def start_all(copies):
    for cp in copies:
      cp.start()

  def wait_all(copies):
    for cp in copies:
      cp.wait()

  start_all(x_copies(0) + pair_copies(0) + pair_copies(1) + x_copies(1)
            + pair_copies(2))

  def project_ahead(j):
    for m in range(3):
      even = wqkv_s[2 * j, m]
      odd = wqkv_s[2 * j + 1, m]
      wqkv_s[2 * j, m] = (even & np.uint32(0xFFFF)) | (odd << 16)
      wqkv_s[2 * j + 1, m] = (even >> 16) | (odd & np.uint32(0xFFFF0000))
    xa = _cat_cols([_as_bf16(x_s[k, 0:ahead // 2]) for k in range(kt)])
    for p in range(2):
      for m in range(3):
        ring[3 * (2 * j + p) + m, 0:ahead] = _dot(
            xa, _as_bf16(wqkv_s[2 * j + p, m]))

  def gate_and_score(j):
    n = seq // half
    gw = gw_ref[...].astype(_F32)
    wr = wr_ref[...].astype(_F32)
    page = pl.ds(pl.multiple_of((j * n) // (8 * _LANES) * 8, 8), 8)
    lane0 = lax.rem(j * (n // 8), _LANES)
    score = score_s[page]
    for i in range(n // 16):
      words = pl.ds(pl.multiple_of(j * (n // 2) + 8 * i, 8), 8)
      rows = pl.ds(pl.multiple_of(j * n + 16 * i, 16), 16)
      xs = [_as_bf16(x_s[k, words]).astype(_F32) for k in range(kt)]
      lg = functools.reduce(jnp.add, [xs[k] * gw[k:k + 1] for k in range(kt)])
      r = functools.reduce(jnp.add, [xs[k] * wr[k:k + 1] for k in range(kt)])
      g = jax.nn.sigmoid(jnp.sum(lg, axis=-1, keepdims=True))
      r = jnp.sum(r, axis=-1, keepdims=True)
      g_s[rows] = jnp.broadcast_to(g, (16, _LANES))
      for k in range(kt):
        mix_s[k, rows] = (1.0 - g) * xs[k]
      for u in range(2):
        score = jnp.where(lane == lane0 + 2 * i + u, r[8 * u:8 * u + 8], score)
    score_s[page] = score

  def pick_next(c):
    score = score_s[...].astype(_BF16).astype(_F32)
    row = lax.broadcasted_iota(jnp.int32, score.shape, 0)
    col = lax.broadcasted_iota(jnp.int32, score.shape, 1)
    tok = ((row >> 3) * (8 * _LANES) + col * 8 + (row & 7)).astype(_F32)
    free = free_s[...] > 0
    cand = jnp.where(free & (score == score), score, -jnp.inf)
    best = _reduce_all(jnp.max, cand)
    pick = _reduce_all(
        jnp.min, jnp.where(free & (cand == best), tok, float(seq)))
    chosen = tok == pick
    free_s[...] = jnp.where(chosen, 0.0, free_s[...])
    r_c = _reduce_all(jnp.sum, jnp.where(chosen, score, 0.0))
    rsel_s[...] = jnp.where(sub == c, r_c, rsel_s[...])
    t = jnp.clip(pick.astype(jnp.int32)[0, 0], 0, seq - 1)
    idx_s[c] = t
    words = pl.ds(pl.multiple_of((t >> 4) * 8, 8), 8)
    row16 = lax.broadcasted_iota(jnp.int32, (16, _LANES), 0)
    for k in range(kt):
      blk = _as_bf16(x_s[k, words]).astype(_F32)
      xt = jnp.sum(jnp.where(row16 == (t & 15), blk, 0.0), axis=0,
                   keepdims=True)
      xsel_s[:, _block(k)] = jnp.where(sub == c, xt, xsel_s[:, _block(k)])

  def first_half(j, carry):
    wait_all(pair_copies(j))
    pl.when(j == ahead // (seq // half))(lambda: wait_all(x_copies(1)))
    gate_and_score(j)
    project_ahead(j)
    start_all(pair_copies(j + 3) + [wo_copy(j)])
    return carry

  def second_half(i, carry):
    j = half + i
    wait_all(pair_copies(j))
    pick_next(i)
    project_ahead(j)
    pl.when(j + 3 < n_pairs)(lambda: start_all(pair_copies(j + 3)))
    per = -(-ft // half)

    @pl.when(i < ft // per)
    def _():
      start_all([wg_copy(per * i + n) for n in range(per)]
                + [wu_copy(per * i + n) for n in range(per)])

    return carry

  score_s[...] = jnp.zeros(score_s.shape, _F32)
  free_s[...] = jnp.ones(free_s.shape, _F32)
  rsel_s[...] = jnp.zeros(rsel_s.shape, _F32)
  xsel_s[...] = jnp.zeros(xsel_s.shape, _F32)
  mem_s[...] = mem0_ref[...].astype(_F32)
  wait_all(x_copies(0))
  lax.fori_loop(0, half, first_half, 0)
  lax.fori_loop(0, half, second_half, 0)
  start_all([wd_copy(n) for n in range(kt)])

  def routed_ffn():
    x_sel = xsel_s[...]
    wait_all([wg_copy(n) for n in range(ft)] + [wu_copy(n) for n in range(ft)]
             + [wd_copy(n) for n in range(kt)])
    act = []
    for n in range(ft):
      gt = _dot(x_sel, _as_bf16(wg_s[n]))
      act.append(gt * jax.nn.sigmoid(gt) * _dot(x_sel, _as_bf16(wu_s[n])))
    act = _cat_cols(act)
    keep = jnp.zeros((8, _LANES), _F32)
    for c in range(_TOP_C):
      keep = jnp.where(sub == c, 1.0 - g_s[pl.ds(idx_s[c], 1)], keep)
    keep = keep * jax.nn.sigmoid(rsel_s[...])
    for n in range(kt):
      y = _dot(act, _as_bf16(wd_s[n])) * keep
      for c in range(_TOP_C):
        mix_s[n, pl.ds(idx_s[c], 1)] += y[c:c + 1]

  n_keys = -(-n_rows // 16) * 16
  qi = lax.broadcasted_iota(jnp.int32, (n_rows, n_keys), 0)
  ki = lax.broadcasted_iota(jnp.int32, (n_rows, n_keys), 1)
  visible = ((qi < n_mem) | (qi >= ki)) & (ki < n_rows)
  hidden = jnp.where(ki < n_rows, -1e9, -jnp.inf).astype(_F32)
  key_pad = jnp.zeros((n_keys - n_rows, _LANES), _F32)

  def step(s, mem):
    word0 = (ahead - n_mem) // 2 + s * (ride // 2)
    lhs = []
    for k in range(kt):
      xw = x_s[k, pl.ds(word0, seg // 2)]
      mw = pltpu.bitcast(
          jnp.concatenate([mem[k], jnp.zeros_like(mem[k])], axis=0
                          ).astype(_BF16), _U32)
      head = jnp.where(sub < n_mem // 2, mw, xw[0:8])
      lhs.append(_as_bf16(jnp.concatenate([head, xw[8:]], axis=0)))
    put = [pl.multiple_of(lax.rem(ahead + s * ride + 8 * i, ring_rows), 8)
           for i in range(ride // 8)]
    get = pl.multiple_of(lax.rem(s * seg, ring_rows), 8)

    qkv, probs, partial = {}, {}, {}

    def project_part(h, k0, k1):
      words = slice(k0 * _LANES // 2, k1 * _LANES // 2)
      w = _cat_cols([_as_bf16(wqkv_s[h, m, words]) for m in range(3)])
      return _dot(_cat_cols(lhs[k0:k1]), w)

    def project(h):
      if h in partial:
        r = part_s[h] + project_part(h, kt // 2, kt)
      else:
        r = project_part(h, 0, kt)
      parts = [r[:, _block(m)] for m in range(3)]
      for m in range(3):
        for i in range(ride // 8):
          lo = n_mem + 8 * i
          ring[3 * h + m, pl.ds(put[i], 8)] = parts[m][lo:lo + 8]
      rows = [[parts[m][0:n_mem], ring[3 * h + m, pl.ds(get, seg)]]
              for m in range(3)]
      qkv[h] = (
          jnp.concatenate(rows[0], axis=0),
          jnp.concatenate(rows[1] + [key_pad], axis=0).astype(_BF16),
          jnp.concatenate(rows[2] + [key_pad], axis=0).astype(_BF16))

    def attend_scores(h):
      q, k, _ = qkv[h]
      sc = lax.dot_general(q, k, (((1,), (1,)), ((), ())),
                           preferred_element_type=_F32)
      sc = jnp.where(visible, sc * scale, hidden)
      p = jnp.exp(sc - jnp.max(sc, axis=-1, keepdims=True))
      probs[h] = (p, jnp.sum(p, axis=-1, keepdims=True))

    def attend_values(h):
      p, denom = probs[h]
      o_s[:, _block(h)] = _dot(p, qkv[h][2]) / denom

    k_part = heads * _LANES // o_split
    acc = [None]

    def out_project(i0, i1):
      w = _cat_cols([
          _as_bf16(wo_s[n, i0 * k_part // 2:i1 * k_part // 2])
          for n in range(kt)])
      r = _dot(o_s[:, i0 * k_part:i1 * k_part], w)
      acc[0] = r if acc[0] is None else acc[0] + r

    for h in range(k_first):
      partial[h] = True
      part_s[h] = project_part(h, 0, kt // 2)
    done = 0
    for h in range(heads + lag_pv):
      if h < heads:
        project(h)
      else:
        out_project(done, done + 1)
        done += 1
      if 0 <= h - lag_s < heads:
        attend_scores(h - lag_s)
      if 0 <= h - lag_pv < heads:
        attend_values(h - lag_pv)
    for _ in range(o_gap):
      out_project(done, done + 1)
      done += 1
    out_project(done, o_split)

    rows = pl.ds(pl.multiple_of(s * seg, seg), seg)
    g = g_s[rows]
    for k in range(kt):
      mixed = g * acc[0][n_mem:, _block(k)] + mix_s[k, rows]
      mix_s[k, rows] = mixed
      out_s[rows, _block(k)] = mixed.astype(_BF16)
    return [acc[0][0:n_mem, _block(k)] for k in range(kt)]

  span = unroll * seg

  def out_copy(i):
    rows = pl.ds(pl.multiple_of(i * span, span), span)
    return pltpu.make_async_copy(out_s.at[rows], out_hbm.at[rows], sem_out)

  def steps(i, carry):
    @pl.when(i == 1)
    def _():
      routed_ffn()
      for k in range(kt):
        out_s[0:span, _block(k)] = mix_s[k, 0:span].astype(_BF16)

    pl.when(i >= 1)(lambda: out_copy(i - 1).start())
    mem = [mem_s[:, _block(k)] for k in range(kt)]
    for u in range(unroll):
      mem = step(i * unroll + u, mem)
    mem_s[...] = _cat_cols(mem)
    return carry

  wait_all([wo_copy(n) for n in range(kt)])
  lax.fori_loop(0, n_seg // unroll, steps, 0)
  out_copy(n_seg // unroll - 1).start()
  pltpu.make_async_copy(out_s, out_hbm, sem_out).wait()


@functools.partial(jax.jit, static_argnames=("A_seg_len",))
def pallas_gated_mix__memory_aug_recurrent_mem_tr__moe_arch_mod__prompt_kernel(
    A_x: jax.Array,
    A_mem0: jax.Array,
    A_Wq: jax.Array,
    A_Wk: jax.Array,
    A_Wv: jax.Array,
    A_Wo: jax.Array,
    A_seg_len: int,
    B_x: jax.Array,
    B_w_r: jax.Array,
    B_w_gate: jax.Array,
    B_w_up: jax.Array,
    B_w_down: jax.Array,
    gate_w: jax.Array,
):
  del B_x
  batch, seq, dm = A_x.shape
  _, heads, dh = A_Wq.shape
  n_mem = A_mem0.shape[1]
  ffn = B_w_gate.shape[1]
  seg = int(A_seg_len)
  kt, ft = dm // _LANES, ffn // _LANES
  assert batch == 1 and dh == _LANES and (n_mem, seg) == (8, 32)
  assert heads == 4 * _TOP_C == 4 * kt
  ahead = seq - (seq // seg) * (seg - n_mem)
  ring_rows = -(-(ahead + seg) // seg) * seg

  hbm = pl.BlockSpec(memory_space=pl.ANY)
  vmem = pl.BlockSpec(memory_space=pltpu.VMEM)
  kernel = functools.partial(
      _kernel, seq=seq, dm=dm, heads=heads, n_mem=n_mem, seg=seg, ffn=ffn,
      lag_s=2, lag_pv=5, o_split=16, unroll=4, k_first=1, o_gap=2)
  out = pl.pallas_call(
      kernel,
      out_shape=jax.ShapeDtypeStruct((seq, dm), A_x.dtype),
      in_specs=[hbm, vmem, hbm, hbm, hbm, hbm, vmem, hbm, hbm, hbm, vmem],
      out_specs=hbm,
      scratch_shapes=[
          pltpu.VMEM((kt, seq // 2, _LANES), _U32),
          pltpu.VMEM((heads, 3, dm // 2, _LANES), _U32),
          pltpu.VMEM((kt, heads * dh // 2, _LANES), _U32),
          pltpu.VMEM((ft, dm // 2, _LANES), _U32),
          pltpu.VMEM((ft, dm // 2, _LANES), _U32),
          pltpu.VMEM((kt, ffn // 2, _LANES), _U32),
          pltpu.VMEM((3 * heads, ring_rows, _LANES), _F32),
          pltpu.VMEM((n_mem + seg, heads * dh), _F32),
          pltpu.VMEM((n_mem, dm), _F32),
          pltpu.VMEM((seq, _LANES), _F32),
          pltpu.VMEM((kt, seq, _LANES), _F32),
          pltpu.VMEM((seq // _LANES, _LANES), _F32),
          pltpu.VMEM((4, seg, 3 * _LANES), _F32),
          pltpu.VMEM((seq // _LANES, _LANES), _F32),
          pltpu.VMEM((_TOP_C, _LANES), _F32),
          pltpu.VMEM((_TOP_C, dm), _F32),
          pltpu.SMEM((_TOP_C,), jnp.int32),
          pltpu.VMEM((seq, dm), _BF16),
          pltpu.SemaphoreType.DMA((2,)),
          pltpu.SemaphoreType.DMA((heads // 2,)),
          pltpu.SemaphoreType.DMA((3,)),
          pltpu.SemaphoreType.DMA,
      ],
      compiler_params=pltpu.CompilerParams(vmem_limit_bytes=120 * 2**20),
      name="gated_rmt_mod",
  )(
      A_x.reshape(seq, dm),
      A_mem0.reshape(n_mem, dm),
      A_Wq.reshape(dm // 2, 2, heads, dh),
      A_Wk.reshape(dm // 2, 2, heads, dh),
      A_Wv.reshape(dm // 2, 2, heads, dh),
      A_Wo.reshape(heads * dh, dm),
      B_w_r.reshape(kt, _LANES),
      B_w_gate,
      B_w_up,
      B_w_down,
      gate_w.reshape(kt, _LANES),
  )
  return out.reshape(batch, seq, dm)
```

```python
import functools

import jax
import jax.experimental.pallas as pl
import jax.experimental.pallas.tpu as pltpu
import jax.numpy as jnp
import numpy as np
from jax import lax

_BF16 = jnp.bfloat16
_F32 = jnp.float32
_U32 = jnp.uint32
_LANES = 128
_TOP_C = 8


def _as_bf16(words):
  return pltpu.bitcast(words, _BF16)


def _cat_cols(parts):
  return parts[0] if len(parts) == 1 else jnp.concatenate(parts, axis=1)


def _block(n):
  return slice(n * _LANES, (n + 1) * _LANES)


def _dot(a, b):
  return jnp.dot(a, b, preferred_element_type=_F32)


def _reduce_all(op, a):
  return op(op(a, axis=1, keepdims=True), axis=0, keepdims=True)


def _work_layout(seq, kt, heads, ring_rows):
  sizes = (
      ("ring", 3 * heads * ring_rows),
      ("mix", kt * seq),
      ("gate", seq),
      ("score", seq // _LANES),
      ("taken", seq // _LANES),
      ("r_sel", _TOP_C),
      ("x_sel", kt * _TOP_C),
      ("end", 0),
  )
  starts = np.cumsum([0] + [n for _, n in sizes])
  return {name: int(start) for (name, _), start in zip(sizes, starts)}


def _kernel(
    x_hbm, mem0_ref, wq_hbm, wk_hbm, wv_hbm, wo_hbm, wr_ref, wg_hbm, wu_hbm,
    wd_hbm, gw_ref,
    out_hbm,
    x_s, wqkv_s, wo_s, wg_s, wu_s, wd_s, work, o_s, mem_s, part_s, pre_s, y_s, idx_s, out_s,
    sem_x, sem_w, sem_misc, sem_out,
    *, seq, dm, heads, n_mem, seg, ffn, ring_rows, lag_s, lag_pv, o_split, unroll, k_first,
    o_gap, p_rows,
):
  kt = dm // _LANES
  ft = ffn // _LANES
  n_seg = seq // seg
  n_rows = n_mem + seg
  ride = seg - n_mem
  ahead = seq - n_seg * ride
  n_pairs = heads // 2
  half = n_pairs // 2
  scale = float(_LANES) ** -0.5
  ffn_blocks = unroll // 2
  ffn_iters = ft // ffn_blocks
  w_hbms = (wq_hbm, wk_hbm, wv_hbm)
  sub = lax.broadcasted_iota(jnp.int32, (8, _LANES), 0)
  lane = lax.broadcasted_iota(jnp.int32, (8, _LANES), 1)

  layout = _work_layout(seq, kt, heads, ring_rows)

  def area(name, row, n, align=8):
    start = layout[name] + row
    return pl.ds(start if isinstance(start, int) or align == 1
                 else pl.multiple_of(start, align), n)

  def ring(h, m, row, n):
    return area("ring", (3 * h + m) * ring_rows + row, n)

  def cols(n):
    return pl.ds(pl.multiple_of(n * _LANES, _LANES), _LANES)

  def x_copies(part):
    lo, n = (0, ahead) if part == 0 else (ahead, seq - ahead)
    return [
        pltpu.make_async_copy(
            x_hbm.at[pl.ds(lo, n), cols(k)],
            x_s.at[k, pl.ds(lo // 2, n // 2)].bitcast(_BF16),
            sem_x.at[part])
        for k in range(kt)]

  def pair_copies(j):
    return [
        pltpu.make_async_copy(
            w_hbms[m].bitcast(_U32).at[:, p, j], wqkv_s.at[2 * j + p, m],
            sem_w.at[j])
        for m in range(3) for p in range(2)]

  def wo_copy(n):
    return pltpu.make_async_copy(
        wo_hbm.at[:, cols(n)], wo_s.at[n].bitcast(_BF16), sem_misc.at[0])

  def ffn_copies(part):
    cut = ffn_blocks * _LANES
    f = pl.ds(0, cut) if part == 0 else pl.ds(cut, ffn - cut)
    sem = sem_misc.at[1 + part]
    return [pltpu.make_async_copy(wg_hbm.at[:, f], wg_s.at[:, f], sem),
            pltpu.make_async_copy(wu_hbm.at[:, f], wu_s.at[:, f], sem),
            pltpu.make_async_copy(wd_hbm.at[f], wd_s.at[f], sem)]

  def start_all(copies):
    for cp in copies:
      cp.start()

  def wait_all(copies):
    for cp in copies:
      cp.wait()

  start_all(x_copies(0) + pair_copies(0) + pair_copies(1) + x_copies(1)
            + pair_copies(2))

  def project_ahead(j, side_work):
    def untangle(m):
      even = wqkv_s[2 * j, m]
      odd = wqkv_s[2 * j + 1, m]
      wqkv_s[2 * j, m] = (even & np.uint32(0xFFFF)) | (odd << 16)
      wqkv_s[2 * j + 1, m] = (even >> 16) | (odd & np.uint32(0xFFFF0000))

    chunks = ahead // p_rows
    untangle(0)
    for m in range(3):
      for p in range(2):
        for c in range(chunks):
          words = slice(c * p_rows // 2, (c + 1) * p_rows // 2)
          xa = _cat_cols([_as_bf16(x_s[k, words]) for k in range(kt)])
          w = _as_bf16(wqkv_s[2 * j + p, m])
          if p == 1 and m < 2 and c == 0:
            untangle(m + 1)
          side_work((2 * m + p) * chunks + c, 6 * chunks)
          work[ring(2 * j + p, m, c * p_rows, p_rows)] = _dot(xa, w)

  def gate_and_score(t0, n):
    gw = gw_ref[...].astype(_F32)
    wr = wr_ref[...].astype(_F32)
    page = area("score", t0 // (8 * _LANES) * 8, 8)
    lane0 = lax.rem(t0 // 8, _LANES)
    score = work[page]
    for i in range(n // 16):
      words = pl.ds(pl.multiple_of(t0 // 2 + 8 * i, 8), 8)
      xs = [_as_bf16(x_s[k, words]).astype(_F32) for k in range(kt)]
      lg = functools.reduce(jnp.add, [xs[k] * gw[k:k + 1] for k in range(kt)])
      r = functools.reduce(jnp.add, [xs[k] * wr[k:k + 1] for k in range(kt)])
      g = jax.nn.sigmoid(jnp.sum(lg, axis=-1, keepdims=True))
      r = jnp.sum(r, axis=-1, keepdims=True)
      work[area("gate", t0 + 16 * i, 16)] = jnp.broadcast_to(g, (16, _LANES))
      for k in range(kt):
        work[area("mix", k * seq + t0 + 16 * i, 16)] = (1.0 - g) * xs[k]
      for u in range(2):
        score = jnp.where(lane == lane0 + 2 * i + u, r[8 * u:8 * u + 8], score)
    work[page] = score

  def pick_next(c):
    n = seq // _LANES
    score = work[area("score", 0, n)].astype(_BF16).astype(_F32)
    row = lax.broadcasted_iota(jnp.int32, score.shape, 0)
    col = lax.broadcasted_iota(jnp.int32, score.shape, 1)
    tok = ((row >> 3) * (8 * _LANES) + col * 8 + (row & 7)).astype(_F32)
    taken = work[area("taken", 0, n)]
    free = taken == 0.0
    cand = jnp.where(free & (score == score), score, -jnp.inf)
    best = _reduce_all(jnp.max, cand)
    pick = _reduce_all(
        jnp.min, jnp.where(free & (cand == best), tok, float(seq)))
    chosen = tok == pick
    work[area("taken", 0, n)] = jnp.where(chosen, 1.0, taken)
    r_c = _reduce_all(jnp.sum, jnp.where(chosen, score, 0.0))
    r_sel = area("r_sel", 0, _TOP_C)
    work[r_sel] = jnp.where(sub == c, r_c, work[r_sel])
    t = jnp.clip(pick.astype(jnp.int32)[0, 0], 0, seq - 1)
    idx_s[c] = t
    words = pl.ds(pl.multiple_of((t >> 4) * 8, 8), 8)
    row16 = lax.broadcasted_iota(jnp.int32, (16, _LANES), 0)
    for k in range(kt):
      blk = _as_bf16(x_s[k, words]).astype(_F32)
      xt = jnp.sum(jnp.where(row16 == (t & 15), blk, 0.0), axis=0,
                   keepdims=True)
      x_sel = area("x_sel", k * _TOP_C, _TOP_C)
      work[x_sel] = jnp.where(sub == c, xt, work[x_sel])

  def first_half(j, carry):
    n = seq // half
    wait_all(pair_copies(j))
    pl.when(j == ahead // n)(lambda: wait_all(x_copies(1)))

    def side_work(i, slots):
      pieces = 2 * slots // 3
      if i < pieces:
        gate_and_score(j * n + i * (n // pieces), n // pieces)
      elif i == pieces:
        wo_copy(j).start()
        start_all(pair_copies(j + 3))

    project_ahead(j, side_work)
    return carry

  def second_half(c, carry):
    j = half + c
    wait_all(pair_copies(j))

    def side_work(i, slots):
      if i == slots // 3:
        pick_next(c)
      elif i == 2 * slots // 3:
        pl.when(j + 3 < n_pairs)(lambda: start_all(pair_copies(j + 3)))
        pl.when(j + 3 == n_pairs)(lambda: start_all(
            ffn_copies(0) + ffn_copies(1)))

    project_ahead(j, side_work)
    return carry

  n_small = layout["end"] - layout["score"]
  work[area("score", 0, n_small)] = jnp.zeros((n_small, _LANES), _F32)
  mem_s[...] = mem0_ref[...].astype(_F32)
  wait_all(x_copies(0))
  lax.fori_loop(0, half, first_half, 0)
  lax.fori_loop(0, half, second_half, 0)

  def ffn_groups(i):
    x_sel = [work[area("x_sel", k * _TOP_C, _TOP_C)] for k in range(kt)]
    first = jnp.minimum(i, ffn_iters - 1) * ffn_blocks
    act = {}

    def widen(b, which, part):
      ks = range(part * kt // 2, (part + 1) * kt // 2)
      w = (wg_s, wu_s)[which][ks[0] * _LANES:(ks[-1] + 1) * _LANES,
                              cols(first + b)]
      r = _dot(_cat_cols([x_sel[k] for k in ks]), w)
      pre_s[b, which, part] = r

    def narrow(b, part):
      if part == 0:
        gate, up = (pre_s[b, n, 0] + pre_s[b, n, 1] for n in range(2))
        act[b] = jnp.where(i < ffn_iters, gate * jax.nn.sigmoid(gate) * up, 0.0)
      span = slice(part * dm // 2, (part + 1) * dm // 2)
      y_s[:, span] += _dot(act[b], wd_s[cols(first + b), span])

    return (
        [functools.partial(widen, b, which, part) for b in range(ffn_blocks)
         for which in range(2) for part in range(2)]
        + [functools.partial(narrow, b, part) for b in range(ffn_blocks)
           for part in range(2)])

  def add_ffn():
    keep = jnp.zeros((8, _LANES), _F32)
    for c in range(_TOP_C):
      keep = jnp.where(sub == c, 1.0 - work[area("gate", idx_s[c], 1, 1)], keep)
    keep = keep * jax.nn.sigmoid(work[area("r_sel", 0, _TOP_C)])
    row16 = lax.broadcasted_iota(jnp.int32, (16, _LANES), 0)
    y = [y_s[:, _block(k)] * keep for k in range(kt)]
    for c in range(_TOP_C):
      t0 = pl.multiple_of((idx_s[c] >> 4) * 16, 16)
      hit = row16 == (idx_s[c] & 15)
      old = [work[area("mix", k * seq + t0, 16)] for k in range(kt)]
      for k in range(kt):
        new = jnp.where(hit, old[k] + y[k][c:c + 1], old[k])
        work[area("mix", k * seq + t0, 16)] = new
        out_s[pl.ds(t0, 16), _block(k)] = new.astype(_BF16)

  n_keys = -(-n_rows // 16) * 16
  qi = lax.broadcasted_iota(jnp.int32, (n_rows, n_keys), 0)
  ki = lax.broadcasted_iota(jnp.int32, (n_rows, n_keys), 1)
  visible = ((qi < n_mem) | (qi >= ki)) & (ki < n_rows)
  hidden = jnp.where(ki < n_rows, -1e9, -jnp.inf).astype(_F32)
  key_pad = jnp.zeros((n_keys - n_rows, _LANES), _F32)

  def step(s, mem, fillers):
    word0 = (ahead - n_mem) // 2 + s * (ride // 2)
    lhs = []
    for k in range(kt):
      xw = x_s[k, pl.ds(word0, seg // 2)]
      mw = pltpu.bitcast(
          jnp.concatenate([mem[k], jnp.zeros_like(mem[k])], axis=0
                          ).astype(_BF16), _U32)
      head = jnp.where(sub < n_mem // 2, mw, xw[0:8])
      lhs.append(_as_bf16(jnp.concatenate([head, xw[8:]], axis=0)))
    put = [lax.rem(ahead + s * ride + 8 * i, ring_rows)
           for i in range(ride // 8)]
    get = lax.rem(s * seg, ring_rows)

    qkv, probs, partial = {}, {}, {}

    def project_part(h, k0, k1):
      words = slice(k0 * _LANES // 2, k1 * _LANES // 2)
      w = _cat_cols([_as_bf16(wqkv_s[h, m, words]) for m in range(3)])
      return _dot(_cat_cols(lhs[k0:k1]), w)

    def project(h):
      if h in partial:
        r = part_s[h] + project_part(h, kt // 2, kt)
      else:
        r = project_part(h, 0, kt)
      parts = [r[:, _block(m)] for m in range(3)]
      for m in range(3):
        for i in range(ride // 8):
          lo = n_mem + 8 * i
          work[ring(h, m, put[i], 8)] = parts[m][lo:lo + 8]
      rows = [[parts[m][0:n_mem], work[ring(h, m, get, seg)]]
              for m in range(3)]
      qkv[h] = (
          jnp.concatenate(rows[0], axis=0),
          jnp.concatenate(rows[1] + [key_pad], axis=0).astype(_BF16),
          jnp.concatenate(rows[2] + [key_pad], axis=0).astype(_BF16))

    def attend_scores(h):
      q, k, _ = qkv[h]
      sc = lax.dot_general(q, k, (((1,), (1,)), ((), ())),
                           preferred_element_type=_F32)
      sc = jnp.where(visible, sc * scale, hidden)
      p = jnp.exp(sc - jnp.max(sc, axis=-1, keepdims=True))
      probs[h] = (p, jnp.sum(p, axis=-1, keepdims=True))

    def attend_values(h):
      p, denom = probs[h]
      o_s[:, _block(h)] = _dot(p, qkv[h][2]) / denom

    k_part = heads * _LANES // o_split
    acc = [None]

    def out_project(i0, i1):
      w = _cat_cols([
          _as_bf16(wo_s[n, i0 * k_part // 2:i1 * k_part // 2])
          for n in range(kt)])
      r = _dot(o_s[:, i0 * k_part:i1 * k_part], w)
      acc[0] = r if acc[0] is None else acc[0] + r

    for h in range(k_first):
      partial[h] = True
      part_s[h] = project_part(h, 0, kt // 2)
    done = 0
    for h in range(heads + lag_pv):
      if h < heads:
        project(h)
      else:
        out_project(done, done + 1)
        done += 1
      if 0 <= h - lag_s < heads:
        attend_scores(h - lag_s)
      if 0 <= h - lag_pv < heads:
        attend_values(h - lag_pv)
    for _ in range(o_gap):
      out_project(done, done + 1)
      done += 1
      if fillers:
        fillers.pop(0)()
    assert not fillers
    out_project(done, o_split)

    rows = pl.ds(pl.multiple_of(s * seg, seg), seg)
    g = work[area("gate", s * seg, seg)]
    for k in range(kt):
      mix = area("mix", k * seq + s * seg, seg)
      mixed = g * acc[0][n_mem:, _block(k)] + work[mix]
      work[mix] = mixed
      out_s[rows, _block(k)] = mixed.astype(_BF16)
    return [acc[0][0:n_mem, _block(k)] for k in range(kt)]

  span = unroll * seg

  def out_copy(first, n):
    rows = pl.ds(first * span, n * span)
    return pltpu.make_async_copy(out_s.at[rows], out_hbm.at[rows], sem_out)

  def steps(i, carry):
    pl.when(i == 1)(lambda: wait_all(ffn_copies(1)))

    @pl.when(i == ffn_iters)
    def _():
      add_ffn()
      out_copy(0, ffn_iters).start()

    groups = ffn_groups(i)
    per_step = len(groups) // unroll
    mem = [mem_s[:, _block(k)] for k in range(kt)]
    for u in range(unroll):
      mem = step(i * unroll + u, mem,
                 groups[u * per_step:(u + 1) * per_step])
    mem_s[...] = _cat_cols(mem)
    return carry

  y_s[...] = jnp.zeros(y_s.shape, _F32)
  wait_all([wo_copy(n) for n in range(kt)] + ffn_copies(0))
  lax.fori_loop(0, n_seg // unroll, steps, 0)
  out_copy(ffn_iters, n_seg // unroll - ffn_iters).start()
  pltpu.make_async_copy(out_s, out_hbm, sem_out).wait()


@functools.partial(jax.jit, static_argnames=("A_seg_len",))
def pallas_gated_mix__memory_aug_recurrent_mem_tr__moe_arch_mod__prompt_kernel(
    A_x: jax.Array,
    A_mem0: jax.Array,
    A_Wq: jax.Array,
    A_Wk: jax.Array,
    A_Wv: jax.Array,
    A_Wo: jax.Array,
    A_seg_len: int,
    B_x: jax.Array,
    B_w_r: jax.Array,
    B_w_gate: jax.Array,
    B_w_up: jax.Array,
    B_w_down: jax.Array,
    gate_w: jax.Array,
):
  del B_x
  batch, seq, dm = A_x.shape
  _, heads, dh = A_Wq.shape
  n_mem = A_mem0.shape[1]
  ffn = B_w_gate.shape[1]
  seg = int(A_seg_len)
  kt = dm // _LANES
  assert batch == 1 and dh == _LANES and (n_mem, seg) == (8, 32)
  assert heads == 4 * _TOP_C == 4 * kt
  ahead = seq - (seq // seg) * (seg - n_mem)
  ring_rows = -(-(ahead + seg) // seg) * seg
  work_rows = _work_layout(seq, kt, heads, ring_rows)["end"]

  hbm = pl.BlockSpec(memory_space=pl.ANY)
  vmem = pl.BlockSpec(memory_space=pltpu.VMEM)
  kernel = functools.partial(
      _kernel, seq=seq, dm=dm, heads=heads, n_mem=n_mem, seg=seg, ffn=ffn,
      ring_rows=ring_rows,
      lag_s=2, lag_pv=6, o_split=16, unroll=4, k_first=1, o_gap=4, p_rows=128)
  out = pl.pallas_call(
      kernel,
      out_shape=jax.ShapeDtypeStruct((seq, dm), A_x.dtype),
      in_specs=[hbm, vmem, hbm, hbm, hbm, hbm, vmem, hbm, hbm, hbm, vmem],
      out_specs=hbm,
      scratch_shapes=[
          pltpu.VMEM((kt, seq // 2, _LANES), _U32),
          pltpu.VMEM((heads, 3, dm // 2, _LANES), _U32),
          pltpu.VMEM((kt, heads * dh // 2, _LANES), _U32),
          pltpu.VMEM((dm, ffn), _BF16),
          pltpu.VMEM((dm, ffn), _BF16),
          pltpu.VMEM((ffn, dm), _BF16),
          pltpu.VMEM((work_rows, _LANES), _F32),
          pltpu.VMEM((n_mem + seg, heads * dh), _F32),
          pltpu.VMEM((n_mem, dm), _F32),
          pltpu.VMEM((4, seg, 3 * _LANES), _F32),
          pltpu.VMEM((2, 2, 2, _TOP_C, _LANES), _F32),
          pltpu.VMEM((_TOP_C, dm), _F32),
          pltpu.SMEM((_TOP_C,), jnp.int32),
          pltpu.VMEM((seq, dm), _BF16),
          pltpu.SemaphoreType.DMA((2,)),
          pltpu.SemaphoreType.DMA((heads // 2,)),
          pltpu.SemaphoreType.DMA((3,)),
          pltpu.SemaphoreType.DMA,
      ],
      compiler_params=pltpu.CompilerParams(vmem_limit_bytes=120 * 2**20),
      name="gated_rmt_mod",
  )(
      A_x.reshape(seq, dm),
      A_mem0.reshape(n_mem, dm),
      A_Wq.reshape(dm // 2, 2, heads, dh),
      A_Wk.reshape(dm // 2, 2, heads, dh),
      A_Wv.reshape(dm // 2, 2, heads, dh),
      A_Wo.reshape(heads * dh, dm),
      B_w_r.reshape(kt, _LANES),
      B_w_gate,
      B_w_up,
      B_w_down,
      gate_w.reshape(kt, _LANES),
  )
  return out.reshape(batch, seq, dm)
```

```python
import functools

import jax
import jax.experimental.pallas as pl
import jax.experimental.pallas.tpu as pltpu
import jax.numpy as jnp
import numpy as np
from jax import lax

_BF16 = jnp.bfloat16
_F32 = jnp.float32
_U32 = jnp.uint32
_LANES = 128
_TOP_C = 8


def _as_bf16(words):
  return pltpu.bitcast(words, _BF16)


def _cat_cols(parts):
  return parts[0] if len(parts) == 1 else jnp.concatenate(parts, axis=1)


def _block(n):
  return slice(n * _LANES, (n + 1) * _LANES)


def _dot(a, b):
  return jnp.dot(a, b, preferred_element_type=_F32)


def _reduce_all(op, a):
  return op(op(a, axis=1, keepdims=True), axis=0, keepdims=True)


def _work_layout(seq, kt, heads, ring_rows):
  sizes = (
      ("ring", 3 * heads * ring_rows),
      ("mix", kt * seq),
      ("gate", seq),
      ("score", seq // _LANES),
      ("taken", seq // _LANES),
      ("r_sel", _TOP_C),
      ("x_sel", kt * _TOP_C),
      ("end", 0),
  )
  starts = np.cumsum([0] + [n for _, n in sizes])
  return {name: int(start) for (name, _), start in zip(sizes, starts)}


def _kernel(
    x_hbm, mem0_ref, wq_hbm, wk_hbm, wv_hbm, wo_hbm, wr_ref, wg_hbm, wu_hbm,
    wd_hbm, gw_ref,
    out_hbm,
    x_s, wqkv_s, wo_s, wg_s, wu_s, wd_s, work, o_s, mem_s, part_s, pre_s, y_s, idx_s, out_s,
    sem_x, sem_w, sem_misc, sem_out,
    *, seq, dm, heads, n_mem, seg, ffn, ring_rows, lag_s, lag_pv, o_split, unroll, k_first,
    o_gap, p_rows,
):
  kt = dm // _LANES
  ft = ffn // _LANES
  n_seg = seq // seg
  n_rows = n_mem + seg
  ride = seg - n_mem
  ahead = seq - n_seg * ride
  n_pairs = heads // 2
  half = n_pairs // 2
  scale = float(_LANES) ** -0.5
  ffn_blocks = unroll // 2
  ffn_iters = ft // ffn_blocks
  w_hbms = (wq_hbm, wk_hbm, wv_hbm)
  sub = lax.broadcasted_iota(jnp.int32, (8, _LANES), 0)
  lane = lax.broadcasted_iota(jnp.int32, (8, _LANES), 1)

  layout = _work_layout(seq, kt, heads, ring_rows)

  def area(name, row, n, align=8):
    start = layout[name] + row
    return pl.ds(start if isinstance(start, int) or align == 1
                 else pl.multiple_of(start, align), n)

  def ring(h, m, row, n):
    return area("ring", (3 * h + m) * ring_rows + row, n)

  def cols(n):
    return pl.ds(pl.multiple_of(n * _LANES, _LANES), _LANES)

  def x_copies(part):
    lo, n = (0, ahead) if part == 0 else (ahead, seq - ahead)
    return [
        pltpu.make_async_copy(
            x_hbm.at[pl.ds(lo, n), cols(k)],
            x_s.at[k, pl.ds(lo // 2, n // 2)].bitcast(_BF16),
            sem_x.at[part])
        for k in range(kt)]

  def pair_copies(j):
    return [
        pltpu.make_async_copy(
            w_hbms[m].bitcast(_U32).at[:, p, j], wqkv_s.at[2 * j + p, m],
            sem_w.at[j])
        for m in range(3) for p in range(2)]

  def wo_copy(n):
    return pltpu.make_async_copy(
        wo_hbm.at[:, cols(n)], wo_s.at[n].bitcast(_BF16), sem_misc.at[0])

  def ffn_copies(part):
    cut = ffn_blocks * _LANES
    f = pl.ds(0, cut) if part == 0 else pl.ds(cut, ffn - cut)
    sem = sem_misc.at[1 + part]
    return [pltpu.make_async_copy(wg_hbm.at[:, f], wg_s.at[:, f], sem),
            pltpu.make_async_copy(wu_hbm.at[:, f], wu_s.at[:, f], sem),
            pltpu.make_async_copy(wd_hbm.at[f], wd_s.at[f], sem)]

  def start_all(copies):
    for cp in copies:
      cp.start()

  def wait_all(copies):
    for cp in copies:
      cp.wait()

  start_all(x_copies(0) + pair_copies(0) + pair_copies(1) + x_copies(1)
            + pair_copies(2))

  def project_ahead(j, side_work):
    def untangle(m):
      even = wqkv_s[2 * j, m]
      odd = wqkv_s[2 * j + 1, m]
      wqkv_s[2 * j, m] = (even & np.uint32(0xFFFF)) | (odd << 16)
      wqkv_s[2 * j + 1, m] = (even >> 16) | (odd & np.uint32(0xFFFF0000))

    chunks = ahead // p_rows
    untangle(0)
    for m in range(3):
      for p in range(2):
        for c in range(chunks):
          words = slice(c * p_rows // 2, (c + 1) * p_rows // 2)
          xa = _cat_cols([_as_bf16(x_s[k, words]) for k in range(kt)])
          w = _as_bf16(wqkv_s[2 * j + p, m])
          if p == 1 and m < 2 and c == 0:
            untangle(m + 1)
          side_work((2 * m + p) * chunks + c, 6 * chunks)
          work[ring(2 * j + p, m, c * p_rows, p_rows)] = _dot(xa, w)

  def gate_and_score(t0, n):
    gw = gw_ref[...].astype(_F32)
    wr = wr_ref[...].astype(_F32)
    page = area("score", t0 // (8 * _LANES) * 8, 8)
    lane0 = lax.rem(t0 // 8, _LANES)
    score = work[page]
    for i in range(n // 16):
      words = pl.ds(pl.multiple_of(t0 // 2 + 8 * i, 8), 8)
      xs = [_as_bf16(x_s[k, words]).astype(_F32) for k in range(kt)]
      lg = functools.reduce(jnp.add, [xs[k] * gw[k:k + 1] for k in range(kt)])
      r = functools.reduce(jnp.add, [xs[k] * wr[k:k + 1] for k in range(kt)])
      g = jax.nn.sigmoid(jnp.sum(lg, axis=-1, keepdims=True))
      r = jnp.sum(r, axis=-1, keepdims=True)
      work[area("gate", t0 + 16 * i, 16)] = jnp.broadcast_to(g, (16, _LANES))
      for k in range(kt):
        work[area("mix", k * seq + t0 + 16 * i, 16)] = (1.0 - g) * xs[k]
      for u in range(2):
        score = jnp.where(lane == lane0 + 2 * i + u, r[8 * u:8 * u + 8], score)
    work[page] = score

  def pick_next(c):
    n = seq // _LANES
    score = work[area("score", 0, n)].astype(_BF16).astype(_F32)
    row = lax.broadcasted_iota(jnp.int32, score.shape, 0)
    col = lax.broadcasted_iota(jnp.int32, score.shape, 1)
    tok = ((row >> 3) * (8 * _LANES) + col * 8 + (row & 7)).astype(_F32)
    taken = work[area("taken", 0, n)]
    free = taken == 0.0
    cand = jnp.where(free & (score == score), score, -jnp.inf)
    best = _reduce_all(jnp.max, cand)
    pick = _reduce_all(
        jnp.min, jnp.where(free & (cand == best), tok, float(seq)))
    chosen = tok == pick
    work[area("taken", 0, n)] = jnp.where(chosen, 1.0, taken)
    r_c = _reduce_all(jnp.sum, jnp.where(chosen, score, 0.0))
    r_sel = area("r_sel", 0, _TOP_C)
    work[r_sel] = jnp.where(sub == c, r_c, work[r_sel])
    t = jnp.clip(pick.astype(jnp.int32)[0, 0], 0, seq - 1)
    idx_s[c] = t
    words = pl.ds(pl.multiple_of((t >> 4) * 8, 8), 8)
    row16 = lax.broadcasted_iota(jnp.int32, (16, _LANES), 0)
    for k in range(kt):
      blk = _as_bf16(x_s[k, words]).astype(_F32)
      xt = jnp.sum(jnp.where(row16 == (t & 15), blk, 0.0), axis=0,
                   keepdims=True)
      x_sel = area("x_sel", k * _TOP_C, _TOP_C)
      work[x_sel] = jnp.where(sub == c, xt, work[x_sel])

  def first_half(j, carry):
    n = seq // half
    wait_all(pair_copies(j))
    pl.when(j == ahead // n)(lambda: wait_all(x_copies(1)))

    def side_work(i, slots):
      pieces = 2 * slots // 3
      if i < pieces:
        gate_and_score(j * n + i * (n // pieces), n // pieces)
      elif i == pieces:
        wo_copy(j).start()
        start_all(pair_copies(j + 3))

    project_ahead(j, side_work)
    return carry

  def second_half(c, carry):
    j = half + c
    wait_all(pair_copies(j))

    def side_work(i, slots):
      if i == slots // 3:
        pick_next(c)
      elif i == 2 * slots // 3:
        pl.when(j + 3 < n_pairs)(lambda: start_all(pair_copies(j + 3)))
        pl.when(j + 3 == n_pairs)(lambda: start_all(
            ffn_copies(0) + ffn_copies(1)))

    project_ahead(j, side_work)
    return carry

  n_small = layout["end"] - layout["score"]
  work[area("score", 0, n_small)] = jnp.zeros((n_small, _LANES), _F32)
  mem_s[...] = mem0_ref[...].astype(_F32)
  wait_all(x_copies(0))
  lax.fori_loop(0, half, first_half, 0)
  lax.fori_loop(0, half, second_half, 0)

  def ffn_groups(i):
    x_sel = [work[area("x_sel", k * _TOP_C, _TOP_C)] for k in range(kt)]
    first = jnp.minimum(i, ffn_iters - 1) * ffn_blocks
    act = {}

    def widen(b, which, part):
      ks = range(part * kt // 2, (part + 1) * kt // 2)
      w = (wg_s, wu_s)[which][ks[0] * _LANES:(ks[-1] + 1) * _LANES,
                              cols(first + b)]
      r = _dot(_cat_cols([x_sel[k] for k in ks]), w)
      pre_s[b, which, part] = r

    def narrow(b, part):
      if part == 0:
        gate, up = (pre_s[b, n, 0] + pre_s[b, n, 1] for n in range(2))
        act[b] = jnp.where(i < ffn_iters, gate * jax.nn.sigmoid(gate) * up, 0.0)
      span = slice(part * dm // 2, (part + 1) * dm // 2)
      y_s[:, span] += _dot(act[b], wd_s[cols(first + b), span])

    return (
        [functools.partial(widen, b, which, part) for b in range(ffn_blocks)
         for which in range(2) for part in range(2)]
        + [functools.partial(narrow, b, part) for b in range(ffn_blocks)
           for part in range(2)])

  def add_ffn():
    keep = jnp.zeros((8, _LANES), _F32)
    for c in range(_TOP_C):
      keep = jnp.where(sub == c, 1.0 - work[area("gate", idx_s[c], 1, 1)], keep)
    keep = keep * jax.nn.sigmoid(work[area("r_sel", 0, _TOP_C)])
    row16 = lax.broadcasted_iota(jnp.int32, (16, _LANES), 0)
    y = [y_s[:, _block(k)] * keep for k in range(kt)]
    for c in range(_TOP_C):
      t0 = pl.multiple_of((idx_s[c] >> 4) * 16, 16)
      hit = row16 == (idx_s[c] & 15)
      old = [work[area("mix", k * seq + t0, 16)] for k in range(kt)]
      for k in range(kt):
        new = jnp.where(hit, old[k] + y[k][c:c + 1], old[k])
        work[area("mix", k * seq + t0, 16)] = new
        out_s[pl.ds(t0, 16), _block(k)] = new.astype(_BF16)

  n_keys = -(-n_rows // 16) * 16
  qi = lax.broadcasted_iota(jnp.int32, (n_rows, n_keys), 0)
  ki = lax.broadcasted_iota(jnp.int32, (n_rows, n_keys), 1)
  visible = ((qi < n_mem) | (qi >= ki)) & (ki < n_rows)
  hidden = jnp.where(ki < n_rows, -1e9, -jnp.inf).astype(_F32)
  key_pad = jnp.zeros((n_keys - n_rows, _LANES), _F32)

  def step(s, parity, mem, fillers):
    mem_first = (ahead + parity * ride) % 16 != 0
    word0 = ((ahead // 2 + s * (ride // 2)) >> 3) << 3
    mem_row, tok_row = (0, n_mem) if mem_first else (ride, 0)
    word = word0 + lax.broadcasted_iota(jnp.int32, (seg // 2, _LANES), 0)
    first = ahead // 2 + s * (ride // 2)
    is_mem = (word < first) | (word >= first + ride // 2)
    lhs = []
    for k in range(kt):
      xw = x_s[k, pl.ds(pl.multiple_of(word0, 8), seg // 2)]
      mw = pltpu.bitcast(
          jnp.concatenate([mem[k], mem[k]], axis=0).astype(_BF16), _U32)
      lhs.append(_as_bf16(
          jnp.where(is_mem, jnp.concatenate([mw, mw], axis=0), xw)))
    put = [lax.rem(ahead + s * ride + 8 * i, ring_rows)
           for i in range(ride // 8)]
    get = lax.rem(s * seg, ring_rows)

    qkv, probs, partial = {}, {}, {}

    def project_part(h, k0, k1):
      words = slice(k0 * _LANES // 2, k1 * _LANES // 2)
      w = _cat_cols([_as_bf16(wqkv_s[h, m, words]) for m in range(3)])
      return _dot(_cat_cols(lhs[k0:k1]), w)

    def project(h):
      if h in partial:
        r = part_s[h] + project_part(h, kt // 2, kt)
      else:
        r = project_part(h, 0, kt)
      parts = [r[:, _block(m)] for m in range(3)]
      for m in range(3):
        for i in range(ride // 8):
          lo = tok_row + 8 * i
          work[ring(h, m, put[i], 8)] = parts[m][lo:lo + 8]
      rows = [[parts[m][mem_row:mem_row + n_mem], work[ring(h, m, get, seg)]]
              for m in range(3)]
      qkv[h] = (
          jnp.concatenate(rows[0], axis=0),
          jnp.concatenate(rows[1] + [key_pad], axis=0).astype(_BF16),
          jnp.concatenate(rows[2] + [key_pad], axis=0).astype(_BF16))

    def attend_scores(h):
      q, k, _ = qkv[h]
      sc = lax.dot_general(q, k, (((1,), (1,)), ((), ())),
                           preferred_element_type=_F32)
      sc = jnp.where(visible, sc * scale, hidden)
      p = jnp.exp(sc - jnp.max(sc, axis=-1, keepdims=True))
      probs[h] = (p, jnp.sum(p, axis=-1, keepdims=True))

    def attend_values(h):
      p, denom = probs[h]
      o_s[:, _block(h)] = _dot(p, qkv[h][2]) / denom

    k_part = heads * _LANES // o_split
    acc = [None]

    def out_project(i0, i1):
      w = _cat_cols([
          _as_bf16(wo_s[n, i0 * k_part // 2:i1 * k_part // 2])
          for n in range(kt)])
      r = _dot(o_s[:, i0 * k_part:i1 * k_part], w)
      acc[0] = r if acc[0] is None else acc[0] + r

    for h in range(k_first):
      partial[h] = True
      part_s[h] = project_part(h, 0, kt // 2)
    done = 0
    for h in range(heads + lag_pv):
      if h < heads:
        project(h)
      else:
        out_project(done, done + 1)
        done += 1
      if 0 <= h - lag_s < heads:
        attend_scores(h - lag_s)
      if 0 <= h - lag_pv < heads:
        attend_values(h - lag_pv)
    for _ in range(o_gap):
      out_project(done, done + 1)
      done += 1
      if fillers:
        fillers.pop(0)()
    assert not fillers
    out_project(done, o_split)

    rows = pl.ds(pl.multiple_of(s * seg, seg), seg)
    g = work[area("gate", s * seg, seg)]
    for k in range(kt):
      mix = area("mix", k * seq + s * seg, seg)
      mixed = g * acc[0][n_mem:, _block(k)] + work[mix]
      work[mix] = mixed
      out_s[rows, _block(k)] = mixed.astype(_BF16)
    return [acc[0][0:n_mem, _block(k)] for k in range(kt)]

  span = unroll * seg

  def out_copy(first, n):
    rows = pl.ds(first * span, n * span)
    return pltpu.make_async_copy(out_s.at[rows], out_hbm.at[rows], sem_out)

  def steps(i, carry):
    pl.when(i == 1)(lambda: wait_all(ffn_copies(1)))

    @pl.when(i == ffn_iters)
    def _():
      add_ffn()
      out_copy(0, ffn_iters).start()

    groups = ffn_groups(i)
    per_step = len(groups) // unroll
    mem = [mem_s[:, _block(k)] for k in range(kt)]
    for u in range(unroll):
      mem = step(i * unroll + u, u % 2, mem,
                 groups[u * per_step:(u + 1) * per_step])
    mem_s[...] = _cat_cols(mem)
    return carry

  y_s[...] = jnp.zeros(y_s.shape, _F32)
  wait_all([wo_copy(n) for n in range(kt)] + ffn_copies(0))
  lax.fori_loop(0, n_seg // unroll, steps, 0)
  out_copy(ffn_iters, n_seg // unroll - ffn_iters).start()
  pltpu.make_async_copy(out_s, out_hbm, sem_out).wait()


@functools.partial(jax.jit, static_argnames=("A_seg_len",))
def pallas_gated_mix__memory_aug_recurrent_mem_tr__moe_arch_mod__prompt_kernel(
    A_x: jax.Array,
    A_mem0: jax.Array,
    A_Wq: jax.Array,
    A_Wk: jax.Array,
    A_Wv: jax.Array,
    A_Wo: jax.Array,
    A_seg_len: int,
    B_x: jax.Array,
    B_w_r: jax.Array,
    B_w_gate: jax.Array,
    B_w_up: jax.Array,
    B_w_down: jax.Array,
    gate_w: jax.Array,
):
  del B_x
  batch, seq, dm = A_x.shape
  _, heads, dh = A_Wq.shape
  n_mem = A_mem0.shape[1]
  ffn = B_w_gate.shape[1]
  seg = int(A_seg_len)
  kt = dm // _LANES
  assert batch == 1 and dh == _LANES and (n_mem, seg) == (8, 32)
  assert heads == 4 * _TOP_C == 4 * kt
  ahead = seq - (seq // seg) * (seg - n_mem)
  ring_rows = -(-(ahead + seg) // seg) * seg
  work_rows = _work_layout(seq, kt, heads, ring_rows)["end"]

  hbm = pl.BlockSpec(memory_space=pl.ANY)
  vmem = pl.BlockSpec(memory_space=pltpu.VMEM)
  kernel = functools.partial(
      _kernel, seq=seq, dm=dm, heads=heads, n_mem=n_mem, seg=seg, ffn=ffn,
      ring_rows=ring_rows,
      lag_s=2, lag_pv=6, o_split=16, unroll=4, k_first=1, o_gap=4, p_rows=128)
  out = pl.pallas_call(
      kernel,
      out_shape=jax.ShapeDtypeStruct((seq, dm), A_x.dtype),
      in_specs=[hbm, vmem, hbm, hbm, hbm, hbm, vmem, hbm, hbm, hbm, vmem],
      out_specs=hbm,
      scratch_shapes=[
          pltpu.VMEM((kt, seq // 2, _LANES), _U32),
          pltpu.VMEM((heads, 3, dm // 2, _LANES), _U32),
          pltpu.VMEM((kt, heads * dh // 2, _LANES), _U32),
          pltpu.VMEM((dm, ffn), _BF16),
          pltpu.VMEM((dm, ffn), _BF16),
          pltpu.VMEM((ffn, dm), _BF16),
          pltpu.VMEM((work_rows, _LANES), _F32),
          pltpu.VMEM((n_mem + seg, heads * dh), _F32),
          pltpu.VMEM((n_mem, dm), _F32),
          pltpu.VMEM((4, seg, 3 * _LANES), _F32),
          pltpu.VMEM((2, 2, 2, _TOP_C, _LANES), _F32),
          pltpu.VMEM((_TOP_C, dm), _F32),
          pltpu.SMEM((_TOP_C,), jnp.int32),
          pltpu.VMEM((seq, dm), _BF16),
          pltpu.SemaphoreType.DMA((2,)),
          pltpu.SemaphoreType.DMA((heads // 2,)),
          pltpu.SemaphoreType.DMA((3,)),
          pltpu.SemaphoreType.DMA,
      ],
      compiler_params=pltpu.CompilerParams(vmem_limit_bytes=120 * 2**20),
      name="gated_rmt_mod",
  )(
      A_x.reshape(seq, dm),
      A_mem0.reshape(n_mem, dm),
      A_Wq.reshape(dm // 2, 2, heads, dh),
      A_Wk.reshape(dm // 2, 2, heads, dh),
      A_Wv.reshape(dm // 2, 2, heads, dh),
      A_Wo.reshape(heads * dh, dm),
      B_w_r.reshape(kt, _LANES),
      B_w_gate,
      B_w_up,
      B_w_down,
      gate_w.reshape(kt, _LANES),
  )
  return out.reshape(batch, seq, dm)
```

```python
import functools

import jax
import jax.experimental.pallas as pl
import jax.experimental.pallas.tpu as pltpu
import jax.numpy as jnp
import numpy as np
from jax import lax

_BF16 = jnp.bfloat16
_F32 = jnp.float32
_U32 = jnp.uint32
_LANES = 128
_TOP_C = 8


def _as_bf16(words):
  return pltpu.bitcast(words, _BF16)


def _cat_cols(parts):
  return parts[0] if len(parts) == 1 else jnp.concatenate(parts, axis=1)


def _block(n):
  return slice(n * _LANES, (n + 1) * _LANES)


def _dot(a, b):
  return jnp.dot(a, b, preferred_element_type=_F32)


def _reduce_all(op, a):
  return op(op(a, axis=1, keepdims=True), axis=0, keepdims=True)


def _work_layout(seq, kt, heads, ring_rows):
  sizes = (
      ("ring", 3 * heads * ring_rows),
      ("mix", kt * seq),
      ("gate", seq),
      ("score", seq // _LANES),
      ("taken", seq // _LANES),
      ("r_sel", _TOP_C),
      ("x_sel", kt * _TOP_C),
      ("end", 0),
  )
  starts = np.cumsum([0] + [n for _, n in sizes])
  return {name: int(start) for (name, _), start in zip(sizes, starts)}


def _kernel(
    x_hbm, mem0_hbm, wq_hbm, wk_hbm, wv_hbm, wo_hbm, wr_hbm, wg_hbm, wu_hbm,
    wd_hbm, gw_hbm,
    out_hbm,
    x_s, wqkv_s, wo_s, wg_s, wu_s, wd_s, work, o_s, mem_s, part_s, pre_s, y_s, idx_s, out_s,
    mem0_ref, wr_ref, gw_ref, sem_x, sem_w, sem_misc, sem_out,
    *, seq, dm, heads, n_mem, seg, ffn, ring_rows, lag_s, lag_pv, o_split, unroll, k_first,
    o_gap, p_rows,
):
  kt = dm // _LANES
  ft = ffn // _LANES
  n_seg = seq // seg
  n_rows = n_mem + seg
  ride = seg - n_mem
  ahead = seq - n_seg * ride
  n_pairs = heads // 2
  half = n_pairs // 2
  x_rows = seq // half
  scale = float(_LANES) ** -0.5
  ffn_blocks = unroll // 2
  ffn_iters = ft // ffn_blocks
  w_hbms = (wq_hbm, wk_hbm, wv_hbm)
  sub = lax.broadcasted_iota(jnp.int32, (8, _LANES), 0)
  lane = lax.broadcasted_iota(jnp.int32, (8, _LANES), 1)

  layout = _work_layout(seq, kt, heads, ring_rows)

  def area(name, row, n, align=8):
    start = layout[name] + row
    return pl.ds(start if isinstance(start, int) or align == 1
                 else pl.multiple_of(start, align), n)

  def ring(h, m, row, n):
    return area("ring", (3 * h + m) * ring_rows + row, n)

  def cols(n):
    return pl.ds(pl.multiple_of(n * _LANES, _LANES), _LANES)

  def x_copies(j):
    n = x_rows // 2
    parts = [pl.ds(pl.multiple_of(j * x_rows + i * n, n), n) for i in range(2)]
    return [pltpu.make_async_copy(x_hbm.at[rows], x_s.at[rows], sem_x.at[j])
            for rows in parts]

  def w_copies(j, m):
    return [
        pltpu.make_async_copy(
            w_hbms[m].bitcast(_U32).at[:, p, j], wqkv_s.at[2 * j + p, m],
            sem_w.at[3 * j + m])
        for p in range(2)]

  small_copies = [
      pltpu.make_async_copy(src, dst, sem_misc.at[3])
      for src, dst in ((mem0_hbm, mem0_ref), (wr_hbm, wr_ref), (gw_hbm, gw_ref))]

  def wo_copy(n):
    return pltpu.make_async_copy(
        wo_hbm.at[:, cols(n)], wo_s.at[n].bitcast(_BF16), sem_misc.at[0])

  def ffn_copies(part):
    cut = 2 * ffn_blocks * _LANES
    f = pl.ds(0, cut) if part == 0 else pl.ds(cut, ffn - cut)
    sem = sem_misc.at[1 + part]
    return [pltpu.make_async_copy(wg_hbm.at[:, f], wg_s.at[:, f], sem),
            pltpu.make_async_copy(wu_hbm.at[:, f], wu_s.at[:, f], sem),
            pltpu.make_async_copy(wd_hbm.at[f], wd_s.at[f], sem)]

  def start_all(copies):
    for cp in copies:
      cp.start()

  def wait_all(copies):
    for cp in copies:
      cp.wait()

  def pair_copies(j):
    return [cp for m in range(3) for cp in w_copies(j, m)]

  start_all(x_copies(0) + w_copies(0, 0) + x_copies(1) + w_copies(0, 1))

  chunks = ahead // p_rows

  def untangle(j, m):
    even = wqkv_s[2 * j, m]
    odd = wqkv_s[2 * j + 1, m]
    wqkv_s[2 * j, m] = (even & np.uint32(0xFFFF)) | (odd << 16)
    wqkv_s[2 * j + 1, m] = (even >> 16) | (odd & np.uint32(0xFFFF0000))

  def project_chunk(h, m, c, before_store=None):
    xa = x_s[c * p_rows:(c + 1) * p_rows]
    w = _as_bf16(wqkv_s[h, m])
    if before_store is not None:
      before_store()
    work[ring(h, m, c * p_rows, p_rows)] = _dot(xa, w)

  def project_pair(j, side_work):
    untangle(j, 0)
    for m in range(3):
      for p in range(2):
        for c in range(chunks):
          def before_store(m=m, p=p, c=c):
            if p == 1 and m < 2 and c == 0:
              untangle(j, m + 1)
            side_work((2 * m + p) * chunks + c)

          project_chunk(2 * j + p, m, c, before_store)

  def gate_and_score(t0, n):
    gw = gw_ref[...].astype(_F32)
    wr = wr_ref[...].astype(_F32)
    page = area("score", t0 // (8 * _LANES) * 8, 8)
    lane0 = lax.rem(t0 // 8, _LANES)
    score = work[page]
    for i in range(n // 16):
      rows = pl.ds(pl.multiple_of(t0 + 16 * i, 16), 16)
      xs = [x_s[rows, _block(k)].astype(_F32) for k in range(kt)]
      lg = functools.reduce(jnp.add, [xs[k] * gw[k:k + 1] for k in range(kt)])
      r = functools.reduce(jnp.add, [xs[k] * wr[k:k + 1] for k in range(kt)])
      g = jax.nn.sigmoid(jnp.sum(lg, axis=-1, keepdims=True))
      r = jnp.sum(r, axis=-1, keepdims=True)
      work[area("gate", t0 + 16 * i, 16)] = jnp.broadcast_to(g, (16, _LANES))
      for k in range(kt):
        work[area("mix", k * seq + t0 + 16 * i, 16)] = (1.0 - g) * xs[k]
      for u in range(2):
        score = jnp.where(lane == lane0 + 2 * i + u, r[8 * u:8 * u + 8], score)
    work[page] = score

  def pick_next(c):
    n = seq // _LANES
    score = work[area("score", 0, n)].astype(_BF16).astype(_F32)
    row = lax.broadcasted_iota(jnp.int32, score.shape, 0)
    col = lax.broadcasted_iota(jnp.int32, score.shape, 1)
    tok = ((row >> 3) * (8 * _LANES) + col * 8 + (row & 7)).astype(_F32)
    taken = work[area("taken", 0, n)]
    free = taken == 0.0
    cand = jnp.where(free & (score == score), score, -jnp.inf)
    best = _reduce_all(jnp.max, cand)
    pick = _reduce_all(
        jnp.min, jnp.where(free & (cand == best), tok, float(seq)))
    chosen = tok == pick
    work[area("taken", 0, n)] = jnp.where(chosen, 1.0, taken)
    r_c = _reduce_all(jnp.sum, jnp.where(chosen, score, 0.0))
    r_sel = area("r_sel", 0, _TOP_C)
    work[r_sel] = jnp.where(sub == c, r_c, work[r_sel])
    t = jnp.clip(pick.astype(jnp.int32)[0, 0], 0, seq - 1)
    idx_s[c] = t
    rows = pl.ds(pl.multiple_of((t >> 4) * 16, 16), 16)
    row16 = lax.broadcasted_iota(jnp.int32, (16, _LANES), 0)
    for k in range(kt):
      blk = x_s[rows, _block(k)].astype(_F32)
      xt = jnp.sum(jnp.where(row16 == (t & 15), blk, 0.0), axis=0,
                   keepdims=True)
      x_sel = area("x_sel", k * _TOP_C, _TOP_C)
      work[x_sel] = jnp.where(sub == c, xt, work[x_sel])

  def gate_piece(j, i, pieces):
    gate_and_score(j * x_rows + i * (x_rows // pieces), x_rows // pieces)

  def first_pair():
    wait_all(x_copies(0) + w_copies(0, 0))
    start_all(small_copies + w_copies(0, 2))
    untangle(0, 0)
    for c in range(chunks):
      if c * p_rows == x_rows:
        wait_all(x_copies(1))
        start_all(pair_copies(1))
      for p in range(2):
        project_chunk(p, 0, c)
    for m in (1, 2):
      wait_all(w_copies(0, m) + (small_copies if m == 2 else []))
      if m == 2:
        start_all(x_copies(2) + pair_copies(2))
      untangle(0, m)
      for p in range(2):
        for c in range(chunks):
          project_chunk(p, m, c, None if m == 1 else functools.partial(
              gate_piece, 0, p * chunks + c, 2 * chunks))

  def first_half(j, carry):
    wait_all(pair_copies(j))
    pl.when(j >= 2)(lambda: wait_all(x_copies(j)))

    def side_work(slot):
      if slot < 4 * chunks:
        gate_piece(j, slot, 4 * chunks)
      elif slot == 4 * chunks:
        pl.when(j + 2 < half)(lambda: start_all(x_copies(j + 2)))
        nxt = j + 2 + jnp.maximum(j + 2 - half, 0)
        start_all(pair_copies(nxt))
        pl.when(nxt >= half)(lambda: start_all(pair_copies(nxt + 1)))
        wo_copy(j).start()

    project_pair(j, side_work)
    return carry

  def second_half(i, carry):
    pairs = (half + 2 * i, half + 2 * i + 1)
    for j in pairs:
      wait_all(pair_copies(j))
    for u, j in enumerate(pairs):
      def side_work(slot, u=u, j=j):
        if slot == 2 * chunks:
          pick_next(j - half)
        elif slot == 4 * chunks:
          if u == 0:
            pl.when(j == half)(lambda: start_all([wo_copy(0)] + ffn_copies(0)))
            pl.when(j + 2 == n_pairs)(lambda: start_all(ffn_copies(1)))
          pl.when(j + 4 < n_pairs)(lambda: start_all(pair_copies(j + 4)))

      project_pair(j, side_work)
    return carry

  n_small = layout["end"] - layout["score"]
  work[area("score", 0, n_small)] = jnp.zeros((n_small, _LANES), _F32)
  first_pair()
  lax.fori_loop(1, half, first_half, 0)
  lax.fori_loop(0, half // 2, second_half, 0)
  mem_s[...] = mem0_ref[...].astype(_F32)

  def ffn_groups(i):
    x_sel = [work[area("x_sel", k * _TOP_C, _TOP_C)] for k in range(kt)]
    first = jnp.minimum(i, ffn_iters - 1) * ffn_blocks
    act = {}

    def widen(b, which, part):
      ks = range(part * kt // 2, (part + 1) * kt // 2)
      w = (wg_s, wu_s)[which][ks[0] * _LANES:(ks[-1] + 1) * _LANES,
                              cols(first + b)]
      r = _dot(_cat_cols([x_sel[k] for k in ks]), w)
      pre_s[b, which, part] = r

    def narrow(b, part):
      if part == 0:
        gate, up = (pre_s[b, n, 0] + pre_s[b, n, 1] for n in range(2))
        act[b] = jnp.where(i < ffn_iters, gate * jax.nn.sigmoid(gate) * up, 0.0)
      span = slice(part * dm // 2, (part + 1) * dm // 2)
      y_s[:, span] += _dot(act[b], wd_s[cols(first + b), span])

    return (
        [functools.partial(widen, b, which, part) for b in range(ffn_blocks)
         for which in range(2) for part in range(2)]
        + [functools.partial(narrow, b, part) for b in range(ffn_blocks)
           for part in range(2)])

  def add_ffn():
    keep = jnp.zeros((8, _LANES), _F32)
    for c in range(_TOP_C):
      keep = jnp.where(sub == c, 1.0 - work[area("gate", idx_s[c], 1, 1)], keep)
    keep = keep * jax.nn.sigmoid(work[area("r_sel", 0, _TOP_C)])
    row16 = lax.broadcasted_iota(jnp.int32, (16, _LANES), 0)
    y = [y_s[:, _block(k)] * keep for k in range(kt)]
    for c in range(_TOP_C):
      t0 = pl.multiple_of((idx_s[c] >> 4) * 16, 16)
      hit = row16 == (idx_s[c] & 15)
      old = [work[area("mix", k * seq + t0, 16)] for k in range(kt)]
      for k in range(kt):
        new = jnp.where(hit, old[k] + y[k][c:c + 1], old[k])
        work[area("mix", k * seq + t0, 16)] = new
        out_s[pl.ds(t0, 16), _block(k)] = new.astype(_BF16)

  n_keys = -(-n_rows // 16) * 16
  qi = lax.broadcasted_iota(jnp.int32, (n_rows, n_keys), 0)
  ki = lax.broadcasted_iota(jnp.int32, (n_rows, n_keys), 1)
  visible = ((qi < n_mem) | (qi >= ki)) & (ki < n_rows)
  hidden = jnp.where(ki < n_rows, -1e9, -jnp.inf).astype(_F32)
  key_pad = jnp.zeros((n_keys - n_rows, _LANES), _F32)

  def step(s, mem, fillers):
    tokens = pl.ds(pl.multiple_of(ahead + s * ride, 8), ride)
    lhs = [
        jnp.concatenate([mem[k], x_s[tokens, _block(k)].astype(_F32)], axis=0
                        ).astype(_BF16) for k in range(kt)]
    put = [lax.rem(ahead + s * ride + 8 * i, ring_rows)
           for i in range(ride // 8)]
    get = lax.rem(s * seg, ring_rows)

    qkv, probs, partial = {}, {}, {}

    def project_part(h, k0, k1):
      words = slice(k0 * _LANES // 2, k1 * _LANES // 2)
      w = _cat_cols([_as_bf16(wqkv_s[h, m, words]) for m in range(3)])
      return _dot(_cat_cols(lhs[k0:k1]), w)

    def project(h):
      if h in partial:
        r = part_s[h] + project_part(h, kt // 2, kt)
      else:
        r = project_part(h, 0, kt)
      parts = [r[:, _block(m)] for m in range(3)]
      for m in range(3):
        for i in range(ride // 8):
          lo = n_mem + 8 * i
          work[ring(h, m, put[i], 8)] = parts[m][lo:lo + 8]
      rows = [[parts[m][0:n_mem], work[ring(h, m, get, seg)]]
              for m in range(3)]
      qkv[h] = (
          jnp.concatenate(rows[0], axis=0),
          jnp.concatenate(rows[1] + [key_pad], axis=0).astype(_BF16),
          jnp.concatenate(rows[2] + [key_pad], axis=0).astype(_BF16))

    def attend_scores(h):
      q, k, _ = qkv[h]
      sc = lax.dot_general(q, k, (((1,), (1,)), ((), ())),
                           preferred_element_type=_F32)
      sc = jnp.where(visible, sc * scale, hidden)
      p = jnp.exp(sc - jnp.max(sc, axis=-1, keepdims=True))
      probs[h] = (p, jnp.sum(p, axis=-1, keepdims=True))

    def attend_values(h):
      p, denom = probs[h]
      o_s[:, _block(h)] = _dot(p, qkv[h][2]) / denom

    k_part = heads * _LANES // o_split
    acc = [None]

    def out_project(i0, i1):
      w = _cat_cols([
          _as_bf16(wo_s[n, i0 * k_part // 2:i1 * k_part // 2])
          for n in range(kt)])
      r = _dot(o_s[:, i0 * k_part:i1 * k_part], w)
      acc[0] = r if acc[0] is None else acc[0] + r

    for h in range(k_first):
      partial[h] = True
      part_s[h] = project_part(h, 0, kt // 2)
    done = 0
    for h in range(heads + lag_pv):
      if h < heads:
        project(h)
      else:
        out_project(done, done + 1)
        done += 1
      if 0 <= h - lag_s < heads:
        attend_scores(h - lag_s)
      if 0 <= h - lag_pv < heads:
        attend_values(h - lag_pv)
    for _ in range(o_gap):
      out_project(done, done + 1)
      done += 1
      if fillers:
        fillers.pop(0)()
    assert not fillers
    out_project(done, o_split)

    rows = pl.ds(pl.multiple_of(s * seg, seg), seg)
    g = work[area("gate", s * seg, seg)]
    for k in range(kt):
      mix = area("mix", k * seq + s * seg, seg)
      mixed = g * acc[0][n_mem:, _block(k)] + work[mix]
      work[mix] = mixed
      out_s[rows, _block(k)] = mixed.astype(_BF16)
    return [acc[0][0:n_mem, _block(k)] for k in range(kt)]

  def out_copy(first, n):
    rows = pl.ds(pl.multiple_of(first * seg, seg), n * seg)
    return pltpu.make_async_copy(out_s.at[rows], out_hbm.at[rows], sem_out)

  def steps(i, carry):
    pl.when(i == 2)(lambda: wait_all(ffn_copies(1)))

    @pl.when(i == ffn_iters)
    def _():
      add_ffn()
      out_copy(0, ffn_iters * unroll).start()

    pl.when(i > ffn_iters)(out_copy((i - 1) * unroll, unroll).start)
    groups = ffn_groups(i)
    per_step = len(groups) // unroll
    mem = [mem_s[:, _block(k)] for k in range(kt)]
    for u in range(unroll):
      s = i * unroll + u
      mem = step(s, mem, groups[u * per_step:(u + 1) * per_step])
    mem_s[...] = _cat_cols(mem)
    return carry

  y_s[...] = jnp.zeros(y_s.shape, _F32)
  wait_all([wo_copy(n) for n in range(kt)] + ffn_copies(0))
  lax.fori_loop(0, n_seg // unroll, steps, 0)
  out_copy(n_seg - unroll, unroll).start()
  pltpu.make_async_copy(out_s, out_hbm, sem_out).wait()


@functools.partial(jax.jit, static_argnames=("A_seg_len",))
def pallas_gated_mix__memory_aug_recurrent_mem_tr__moe_arch_mod__prompt_kernel(
    A_x: jax.Array,
    A_mem0: jax.Array,
    A_Wq: jax.Array,
    A_Wk: jax.Array,
    A_Wv: jax.Array,
    A_Wo: jax.Array,
    A_seg_len: int,
    B_x: jax.Array,
    B_w_r: jax.Array,
    B_w_gate: jax.Array,
    B_w_up: jax.Array,
    B_w_down: jax.Array,
    gate_w: jax.Array,
):
  del B_x
  batch, seq, dm = A_x.shape
  _, heads, dh = A_Wq.shape
  n_mem = A_mem0.shape[1]
  ffn = B_w_gate.shape[1]
  seg = int(A_seg_len)
  kt = dm // _LANES
  assert batch == 1 and dh == _LANES and (n_mem, seg) == (8, 32)
  assert heads == 4 * _TOP_C == 4 * kt
  ahead = seq - (seq // seg) * (seg - n_mem)
  assert ahead == seq // 4
  ring_rows = -(-(ahead + seg) // seg) * seg
  work_rows = _work_layout(seq, kt, heads, ring_rows)["end"]

  hbm = pl.BlockSpec(memory_space=pl.ANY)
  kernel = functools.partial(
      _kernel, seq=seq, dm=dm, heads=heads, n_mem=n_mem, seg=seg, ffn=ffn,
      ring_rows=ring_rows,
      lag_s=2, lag_pv=6, o_split=16, unroll=4, k_first=1, o_gap=4, p_rows=128)
  out = pl.pallas_call(
      kernel,
      out_shape=jax.ShapeDtypeStruct((seq, dm), A_x.dtype),
      in_specs=[hbm] * 11,
      out_specs=hbm,
      scratch_shapes=[
          pltpu.VMEM((seq, dm), _BF16),
          pltpu.VMEM((heads, 3, dm // 2, _LANES), _U32),
          pltpu.VMEM((kt, heads * dh // 2, _LANES), _U32),
          pltpu.VMEM((dm, ffn), _BF16),
          pltpu.VMEM((dm, ffn), _BF16),
          pltpu.VMEM((ffn, dm), _BF16),
          pltpu.VMEM((work_rows, _LANES), _F32),
          pltpu.VMEM((n_mem + seg, heads * dh), _F32),
          pltpu.VMEM((n_mem, dm), _F32),
          pltpu.VMEM((4, seg, 3 * _LANES), _F32),
          pltpu.VMEM((2, 2, 2, _TOP_C, _LANES), _F32),
          pltpu.VMEM((_TOP_C, dm), _F32),
          pltpu.SMEM((_TOP_C,), jnp.int32),
          pltpu.VMEM((seq, dm), _BF16),
          pltpu.VMEM((n_mem, dm), _BF16),
          pltpu.VMEM((kt, _LANES), _BF16),
          pltpu.VMEM((kt, _LANES), _BF16),
          pltpu.SemaphoreType.DMA((heads // 4,)),
          pltpu.SemaphoreType.DMA((3 * heads // 2,)),
          pltpu.SemaphoreType.DMA((4,)),
          pltpu.SemaphoreType.DMA,
      ],
      compiler_params=pltpu.CompilerParams(vmem_limit_bytes=120 * 2**20),
      name="gated_rmt_mod",
  )(
      A_x.reshape(seq, dm),
      A_mem0.reshape(n_mem, dm),
      A_Wq.reshape(dm // 2, 2, heads, dh),
      A_Wk.reshape(dm // 2, 2, heads, dh),
      A_Wv.reshape(dm // 2, 2, heads, dh),
      A_Wo.reshape(heads * dh, dm),
      B_w_r.reshape(kt, _LANES),
      B_w_gate,
      B_w_up,
      B_w_down,
      gate_w.reshape(kt, _LANES),
  )
  return out.reshape(batch, seq, dm)
```

```python
import functools

import jax
import jax.experimental.pallas as pl
import jax.experimental.pallas.tpu as pltpu
import jax.numpy as jnp
import numpy as np
from jax import lax

_BF16 = jnp.bfloat16
_F32 = jnp.float32
_U32 = jnp.uint32
_LANES = 128
_TOP_C = 8


def _as_bf16(words):
  return pltpu.bitcast(words, _BF16)


def _cat_cols(parts):
  return parts[0] if len(parts) == 1 else jnp.concatenate(parts, axis=1)


def _block(n):
  return slice(n * _LANES, (n + 1) * _LANES)


def _dot(a, b):
  return jnp.dot(a, b, preferred_element_type=_F32)


def _reduce_all(op, a):
  return op(op(a, axis=1, keepdims=True), axis=0, keepdims=True)


def _work_layout(seq, kt, heads, ring_rows):
  sizes = (
      ("ring", 3 * heads * ring_rows),
      ("mix", kt * seq),
      ("gate", seq),
      ("score", seq // _LANES),
      ("taken", seq // _LANES),
      ("r_sel", _TOP_C),
      ("x_sel", kt * _TOP_C),
      ("end", 0),
  )
  starts = np.cumsum([0] + [n for _, n in sizes])
  return {name: int(start) for (name, _), start in zip(sizes, starts)}


def _kernel(
    x_hbm, mem0_hbm, wq_hbm, wk_hbm, wv_hbm, wo_hbm, wr_hbm, wg_hbm, wu_hbm,
    wd_hbm, gw_hbm,
    out_hbm,
    x_s, wqkv_s, wo_s, wg_s, wu_s, wd_s, work, o_s, mem_s, part_s, pre_s, y_s, idx_s, out_s,
    mem0_ref, wr_ref, gw_ref, sem_x, sem_w, sem_misc, sem_out,
    *, seq, dm, heads, n_mem, seg, ffn, ring_rows, lag_s, lag_pv, o_split, unroll, k_first,
    o_gap, p_rows, newton, get_s, get_pv,
):
  kt = dm // _LANES
  ft = ffn // _LANES
  n_seg = seq // seg
  n_rows = n_mem + seg
  ride = seg - n_mem
  ahead = seq - n_seg * ride
  n_pairs = heads // 2
  half = n_pairs // 2
  x_rows = seq // half
  scale = float(_LANES) ** -0.5
  ffn_blocks = unroll // 2
  ffn_iters = ft // ffn_blocks
  w_hbms = (wq_hbm, wk_hbm, wv_hbm)
  sub = lax.broadcasted_iota(jnp.int32, (8, _LANES), 0)
  lane = lax.broadcasted_iota(jnp.int32, (8, _LANES), 1)

  layout = _work_layout(seq, kt, heads, ring_rows)

  def area(name, row, n, align=8):
    start = layout[name] + row
    return pl.ds(start if isinstance(start, int) or align == 1
                 else pl.multiple_of(start, align), n)

  def ring(h, m, row, n):
    return area("ring", (3 * h + m) * ring_rows + row, n)

  def cols(n):
    return pl.ds(pl.multiple_of(n * _LANES, _LANES), _LANES)

  def x_copies(j):
    n = x_rows // 2
    parts = [pl.ds(pl.multiple_of(j * x_rows + i * n, n), n) for i in range(2)]
    return [pltpu.make_async_copy(x_hbm.at[rows], x_s.at[rows], sem_x.at[j & 3])
            for rows in parts]

  def w_copies(j, m, sem=None):
    return [
        pltpu.make_async_copy(
            w_hbms[m].bitcast(_U32).at[:, p, j], wqkv_s.at[2 * j + p, m],
            sem_w.at[lax.rem(j, 6) if sem is None else sem])
        for p in range(2)]

  small_copies = [
      pltpu.make_async_copy(src, dst, sem_misc.at[1])
      for src, dst in ((mem0_hbm, mem0_ref), (wr_hbm, wr_ref), (gw_hbm, gw_ref))]

  def wo_copy(n):
    return pltpu.make_async_copy(
        wo_hbm.at[:, cols(n)], wo_s.at[n].bitcast(_BF16), sem_misc.at[0])

  def ffn_copies(i):
    width = ffn_blocks * _LANES
    f = pl.ds(pl.multiple_of(i * width, width), width)
    sem = sem_misc.at[2 + (i & 1)]
    return [pltpu.make_async_copy(wg_hbm.at[:, f], wg_s.at[i & 1], sem),
            pltpu.make_async_copy(wu_hbm.at[:, f], wu_s.at[i & 1], sem),
            pltpu.make_async_copy(wd_hbm.at[f], wd_s.at[i & 1], sem)]

  def start_all(copies):
    for cp in copies:
      cp.start()

  def wait_all(copies):
    for cp in copies:
      cp.wait()

  def pair_copies(j):
    return [cp for m in range(3) for cp in w_copies(j, m)]

  start_all(x_copies(0) + w_copies(0, 0) + x_copies(1) + w_copies(0, 1, 4))

  chunks = ahead // p_rows

  def untangle(j, m):
    even = wqkv_s[2 * j, m]
    odd = wqkv_s[2 * j + 1, m]
    wqkv_s[2 * j, m] = (even & np.uint32(0xFFFF)) | (odd << 16)
    wqkv_s[2 * j + 1, m] = (even >> 16) | (odd & np.uint32(0xFFFF0000))

  def project_chunk(h, m, c, before_store=None):
    xa = x_s[c * p_rows:(c + 1) * p_rows]
    w = _as_bf16(wqkv_s[h, m])
    if before_store is not None:
      before_store()
    work[ring(h, m, c * p_rows, p_rows)] = _dot(xa, w)

  def project_pair(j, side_work):
    untangle(j, 0)
    for m in range(3):
      for p in range(2):
        for c in range(chunks):
          def before_store(m=m, p=p, c=c):
            if p == 1 and m < 2 and c == 0:
              untangle(j, m + 1)
            side_work((2 * m + p) * chunks + c)

          project_chunk(2 * j + p, m, c, before_store)

  def gate_and_score(t0, score):
    gw = gw_ref[...].astype(_F32)
    wr = wr_ref[...].astype(_F32)
    rows = pl.ds(pl.multiple_of(t0, 16), 16)
    xs = [x_s[rows, _block(k)].astype(_F32) for k in range(kt)]
    lg = functools.reduce(jnp.add, [xs[k] * gw[k:k + 1] for k in range(kt)])
    r = functools.reduce(jnp.add, [xs[k] * wr[k:k + 1] for k in range(kt)])
    g = jax.nn.sigmoid(jnp.sum(lg, axis=-1, keepdims=True))
    r = jnp.sum(r, axis=-1, keepdims=True)
    work[area("gate", t0, 16)] = jnp.broadcast_to(g, (16, _LANES))
    for k in range(kt):
      work[area("mix", k * seq + t0, 16)] = (1.0 - g) * xs[k]
    for u in range(2):
      for n in range(len(score)):
        here = (n * _LANES + lane) * 8 == t0 + 8 * u
        score[n] = jnp.where(here, r[8 * u:8 * u + 8], score[n])

  def pick_next(c):
    n = seq // _LANES
    score = work[area("score", 0, n)].astype(_BF16).astype(_F32)
    row = lax.broadcasted_iota(jnp.int32, score.shape, 0)
    col = lax.broadcasted_iota(jnp.int32, score.shape, 1)
    tok = ((row >> 3) * (8 * _LANES) + col * 8 + (row & 7)).astype(_F32)
    taken = work[area("taken", 0, n)]
    free = taken == 0.0
    cand = jnp.where(free & (score == score), score, -jnp.inf)
    best = _reduce_all(jnp.max, cand)
    pick = _reduce_all(
        jnp.min, jnp.where(free & (cand == best), tok, float(seq)))
    chosen = tok == pick
    work[area("taken", 0, n)] = jnp.where(chosen, 1.0, taken)
    r_c = _reduce_all(jnp.sum, jnp.where(chosen, score, 0.0))
    r_sel = area("r_sel", 0, _TOP_C)
    work[r_sel] = jnp.where(sub == c, r_c, work[r_sel])
    t = jnp.clip(pick.astype(jnp.int32)[0, 0], 0, seq - 1)
    idx_s[c] = t
    rows = pl.ds(pl.multiple_of((t >> 4) * 16, 16), 16)
    row16 = lax.broadcasted_iota(jnp.int32, (16, _LANES), 0)
    for k in range(kt):
      blk = x_s[rows, _block(k)].astype(_F32)
      xt = jnp.sum(jnp.where(row16 == (t & 15), blk, 0.0), axis=0,
                   keepdims=True)
      x_sel = area("x_sel", k * _TOP_C, _TOP_C)
      work[x_sel] = jnp.where(sub == c, xt, work[x_sel])

  def first_pair():
    wait_all(x_copies(0) + w_copies(0, 0))
    start_all(small_copies + w_copies(0, 2, 5))
    untangle(0, 0)
    for c in range(chunks):
      if c * p_rows == x_rows:
        wait_all(x_copies(1))
        start_all(pair_copies(1) + x_copies(2))
      for p in range(2):
        project_chunk(p, 0, c)
    for m in (1, 2):
      wait_all(w_copies(0, m, 3 + m))
      if m == 2:
        start_all(pair_copies(2) + x_copies(3))
      untangle(0, m)
      for p in range(2):
        for c in range(chunks):
          project_chunk(p, m, c)
    start_all(pair_copies(3))
    wait_all(small_copies)

  def first_half(j, carry):
    wait_all(pair_copies(j))
    pl.when(j + 1 < half)(lambda: wait_all(x_copies(j + 1)))
    pieces = -(-seq // (16 * (half - 1)))

    pages = [area("score", 8 * n, 8) for n in range(seq // (8 * _LANES))]
    score = [work[page] for page in pages]

    def side_work(slot):
      if slot < pieces:
        first = jnp.minimum((j - 1) * pieces * 16, seq - pieces * 16)
        gate_and_score(first + 16 * slot, score)
      elif slot == pieces:
        for page, value in zip(pages, score):
          work[page] = value
      elif slot == 6 * chunks - 1:
        start_all(pair_copies(j + 3))
        pl.when(j + 1 == half)(lambda: start_all(pair_copies(j + 4)))
        pl.when(j + 3 < half)(lambda: start_all(x_copies(j + 3)))
        pl.when((j + 3 >= half) & (j + 1 < half))(
            lambda: wo_copy(j + 3 - half).start())

    project_pair(j, side_work)
    return carry

  def second_half(i, carry):
    pairs = (half + 2 * i, half + 2 * i + 1)
    for j in pairs:
      wait_all(pair_copies(j))
    for u, j in enumerate(pairs):
      def side_work(slot, u=u, j=j):
        if slot == 2 * chunks:
          pick_next(j - half)
        elif u == 1 and slot == 6 * chunks - 1:
          pl.when(j + 4 < n_pairs)(
              lambda: start_all(pair_copies(j + 3) + pair_copies(j + 4)))
          pl.when(2 * i + 2 < kt)(
              lambda: start_all([wo_copy(2 * i + 2), wo_copy(2 * i + 3)]))
          pl.when(2 * i + 4 == kt)(lambda: start_all(ffn_copies(0)))

      project_pair(j, side_work)
    return carry

  n_small = layout["end"] - layout["score"]
  work[area("score", 0, n_small)] = jnp.zeros((n_small, _LANES), _F32)
  first_pair()
  lax.fori_loop(1, half, first_half, 0)
  lax.fori_loop(0, half // 2, second_half, 0)
  mem_s[...] = mem0_ref[...].astype(_F32)

  def ffn_groups(i):
    x_sel = [work[area("x_sel", k * _TOP_C, _TOP_C)] for k in range(kt)]
    act = {}

    def widen(b, which, part):
      ks = range(part * kt // 2, (part + 1) * kt // 2)
      w = (wg_s, wu_s)[which][
          i & 1, ks[0] * _LANES:(ks[-1] + 1) * _LANES, _block(b)]
      r = _dot(_cat_cols([x_sel[k] for k in ks]), w)
      pre_s[b, which, part] = r

    def narrow(b, part):
      if part == 0:
        gate, up = (pre_s[b, n, 0] + pre_s[b, n, 1] for n in range(2))
        act[b] = jnp.where(i < ffn_iters, gate * jax.nn.sigmoid(gate) * up, 0.0)
      span = slice(part * dm // 2, (part + 1) * dm // 2)
      y_s[:, span] += _dot(act[b], wd_s[i & 1, _block(b), span])

    return (
        [functools.partial(widen, b, which, part) for b in range(ffn_blocks)
         for which in range(2) for part in range(2)]
        + [functools.partial(narrow, b, part) for b in range(ffn_blocks)
           for part in range(2)])

  def add_ffn():
    keep = jnp.zeros((8, _LANES), _F32)
    for c in range(_TOP_C):
      keep = jnp.where(sub == c, 1.0 - work[area("gate", idx_s[c], 1, 1)], keep)
    keep = keep * jax.nn.sigmoid(work[area("r_sel", 0, _TOP_C)])
    row16 = lax.broadcasted_iota(jnp.int32, (16, _LANES), 0)
    y = [y_s[:, _block(k)] * keep for k in range(kt)]
    for c in range(_TOP_C):
      t0 = pl.multiple_of((idx_s[c] >> 4) * 16, 16)
      hit = row16 == (idx_s[c] & 15)
      old = [work[area("mix", k * seq + t0, 16)] for k in range(kt)]
      for k in range(kt):
        new = jnp.where(hit, old[k] + y[k][c:c + 1], old[k])
        work[area("mix", k * seq + t0, 16)] = new
        out_s[pl.ds(t0, 16), _block(k)] = new.astype(_BF16)

  n_keys = -(-n_rows // 16) * 16
  qi = lax.broadcasted_iota(jnp.int32, (n_rows, n_keys), 0)
  ki = lax.broadcasted_iota(jnp.int32, (n_rows, n_keys), 1)
  visible = ((qi < n_mem) | (qi >= ki)) & (ki < n_rows)
  hidden = jnp.where(ki < n_rows, -1e9, -jnp.inf).astype(_F32)
  key_pad = jnp.zeros((n_keys - n_rows, _LANES), _F32)

  def step(s, mem, fillers):
    tokens = pl.ds(pl.multiple_of(ahead + s * ride, 8), ride)
    lhs = [
        jnp.concatenate([mem[k], x_s[tokens, _block(k)].astype(_F32)], axis=0
                        ).astype(_BF16) for k in range(kt)]
    put = [lax.rem(ahead + s * ride + 8 * i, ring_rows)
           for i in range(ride // 8)]
    get = lax.rem(s * seg, ring_rows)

    qkv, probs, partial = {}, {}, {}

    def project_part(h, k0, k1):
      words = slice(k0 * _LANES // 2, k1 * _LANES // 2)
      w = _cat_cols([_as_bf16(wqkv_s[h, m, words]) for m in range(3)])
      return _dot(_cat_cols(lhs[k0:k1]), w)

    def gather(h, m):
      if 0 <= h < heads:
        rows = [qkv[h][m], work[ring(h, m, get, seg)]]
        qkv[h][m] = (
            jnp.concatenate(rows, axis=0) if m == 0 else
            jnp.concatenate(rows + [key_pad], axis=0).astype(_BF16))

    def gather_for(h):
      gather(h - get_s, 0)
      gather(h - get_s, 1)
      gather(h - get_pv, 2)

    def project(h):
      if h in partial:
        r = part_s[h] + project_part(h, kt // 2, kt)
      else:
        r = project_part(h, 0, kt)
      parts = [r[:, _block(m)] for m in range(3)]
      for m in range(3):
        for i in range(ride // 8):
          lo = n_mem + 8 * i
          work[ring(h, m, put[i], 8)] = parts[m][lo:lo + 8]
      qkv[h] = [p[0:n_mem] for p in parts]
      gather_for(h)

    def attend_scores(h):
      q, k, _ = qkv[h]
      sc = lax.dot_general(q, k, (((1,), (1,)), ((), ())),
                           preferred_element_type=_F32)
      sc = jnp.where(visible, sc * scale, hidden)
      p = jnp.exp(sc - jnp.max(sc, axis=-1, keepdims=True))
      probs[h] = (p, jnp.sum(p, axis=-1, keepdims=True))

    def attend_values(h):
      p, denom = probs[h]
      if newton:
        inv = pltpu.reciprocal(denom, approx=True)
        inv = inv * (2.0 - denom * inv)
        o_s[:, _block(h)] = _dot(p, qkv[h][2]) * inv
      else:
        o_s[:, _block(h)] = _dot(p, qkv[h][2]) / denom

    k_part = heads * _LANES // o_split
    acc = [None]

    def out_project(i0, i1):
      w = _cat_cols([
          _as_bf16(wo_s[n, i0 * k_part // 2:i1 * k_part // 2])
          for n in range(kt)])
      r = _dot(o_s[:, i0 * k_part:i1 * k_part], w)
      acc[0] = r if acc[0] is None else acc[0] + r

    for h in range(k_first):
      partial[h] = True
      part_s[h] = project_part(h, 0, kt // 2)
    done = 0
    for h in range(heads + lag_pv):
      if h < heads:
        project(h)
      else:
        gather_for(h)
        out_project(done, done + 1)
        done += 1
      if 0 <= h - lag_s < heads:
        attend_scores(h - lag_s)
      if 0 <= h - lag_pv < heads:
        attend_values(h - lag_pv)
    for _ in range(o_gap):
      out_project(done, done + 1)
      done += 1
      if fillers:
        fillers.pop(0)()
    assert not fillers
    out_project(done, o_split)

    rows = pl.ds(pl.multiple_of(s * seg, seg), seg)
    g = work[area("gate", s * seg, seg)]
    for k in range(kt):
      mix = area("mix", k * seq + s * seg, seg)
      mixed = g * acc[0][n_mem:, _block(k)] + work[mix]
      work[mix] = mixed
      out_s[rows, _block(k)] = mixed.astype(_BF16)
    return [acc[0][0:n_mem, _block(k)] for k in range(kt)]

  def out_copy(first, n):
    rows = pl.ds(pl.multiple_of(first * seg, seg), n * seg)
    return pltpu.make_async_copy(out_s.at[rows], out_hbm.at[rows], sem_out)

  def steps(i, carry):
    pl.when(i < ffn_iters)(lambda: wait_all(ffn_copies(i)))
    pl.when(i + 1 < ffn_iters)(lambda: start_all(ffn_copies(i + 1)))

    @pl.when(i == ffn_iters)
    def _():
      add_ffn()
      out_copy(0, ffn_iters * unroll).start()

    pl.when(i > ffn_iters)(out_copy((i - 1) * unroll, unroll).start)
    groups = ffn_groups(i)
    per_step = len(groups) // unroll
    mem = [mem_s[:, _block(k)] for k in range(kt)]
    for u in range(unroll):
      s = i * unroll + u
      mem = step(s, mem, groups[u * per_step:(u + 1) * per_step])
    mem_s[...] = _cat_cols(mem)
    return carry

  y_s[...] = jnp.zeros(y_s.shape, _F32)
  wait_all([wo_copy(n) for n in range(kt)])
  lax.fori_loop(0, n_seg // unroll, steps, 0)
  out_copy(n_seg - unroll, unroll).start()
  pltpu.make_async_copy(out_s, out_hbm, sem_out).wait()


@functools.partial(jax.jit, static_argnames=("A_seg_len",))
def pallas_gated_mix__memory_aug_recurrent_mem_tr__moe_arch_mod__prompt_kernel(
    A_x: jax.Array,
    A_mem0: jax.Array,
    A_Wq: jax.Array,
    A_Wk: jax.Array,
    A_Wv: jax.Array,
    A_Wo: jax.Array,
    A_seg_len: int,
    B_x: jax.Array,
    B_w_r: jax.Array,
    B_w_gate: jax.Array,
    B_w_up: jax.Array,
    B_w_down: jax.Array,
    gate_w: jax.Array,
):
  del B_x
  batch, seq, dm = A_x.shape
  _, heads, dh = A_Wq.shape
  n_mem = A_mem0.shape[1]
  ffn = B_w_gate.shape[1]
  seg = int(A_seg_len)
  kt = dm // _LANES
  assert batch == 1 and dh == _LANES and (n_mem, seg) == (8, 32)
  assert heads == 4 * _TOP_C == 4 * kt
  ahead = seq - (seq // seg) * (seg - n_mem)
  assert ahead == seq // 4
  ring_rows = -(-(ahead + seg) // seg) * seg
  work_rows = _work_layout(seq, kt, heads, ring_rows)["end"]

  hbm = pl.BlockSpec(memory_space=pl.ANY)
  kernel = functools.partial(
      _kernel, seq=seq, dm=dm, heads=heads, n_mem=n_mem, seg=seg, ffn=ffn,
      ring_rows=ring_rows,
      lag_s=2, lag_pv=5, o_split=16, unroll=4, k_first=1, o_gap=4, p_rows=128, newton=1, get_s=0, get_pv=2)
  out = pl.pallas_call(
      kernel,
      out_shape=jax.ShapeDtypeStruct((seq, dm), A_x.dtype),
      in_specs=[hbm] * 11,
      out_specs=hbm,
      scratch_shapes=[
          pltpu.VMEM((seq, dm), _BF16),
          pltpu.VMEM((heads, 3, dm // 2, _LANES), _U32),
          pltpu.VMEM((kt, heads * dh // 2, _LANES), _U32),
          pltpu.VMEM((2, dm, 256), _BF16),
          pltpu.VMEM((2, dm, 256), _BF16),
          pltpu.VMEM((2, 256, dm), _BF16),
          pltpu.VMEM((work_rows, _LANES), _F32),
          pltpu.VMEM((n_mem + seg, heads * dh), _F32),
          pltpu.VMEM((n_mem, dm), _F32),
          pltpu.VMEM((4, seg, 3 * _LANES), _F32),
          pltpu.VMEM((2, 2, 2, _TOP_C, _LANES), _F32),
          pltpu.VMEM((_TOP_C, dm), _F32),
          pltpu.SMEM((_TOP_C,), jnp.int32),
          pltpu.VMEM((seq, dm), _BF16),
          pltpu.VMEM((n_mem, dm), _BF16),
          pltpu.VMEM((kt, _LANES), _BF16),
          pltpu.VMEM((kt, _LANES), _BF16),
          pltpu.SemaphoreType.DMA((4,)),
          pltpu.SemaphoreType.DMA((6,)),
          pltpu.SemaphoreType.DMA((4,)),
          pltpu.SemaphoreType.DMA,
      ],
      compiler_params=pltpu.CompilerParams(
          vmem_limit_bytes=120 * 2**20, disable_bounds_checks=True),
      name="gated_rmt_mod",
  )(
      A_x.reshape(seq, dm),
      A_mem0.reshape(n_mem, dm),
      A_Wq.reshape(dm // 2, 2, heads, dh),
      A_Wk.reshape(dm // 2, 2, heads, dh),
      A_Wv.reshape(dm // 2, 2, heads, dh),
      A_Wo.reshape(heads * dh, dm),
      B_w_r.reshape(kt, _LANES),
      B_w_gate,
      B_w_up,
      B_w_down,
      gate_w.reshape(kt, _LANES),
  )
  return out.reshape(batch, seq, dm)
```

```python
import functools

import jax
import jax.experimental.pallas as pl
import jax.experimental.pallas.tpu as pltpu
import jax.numpy as jnp
import numpy as np
from jax import lax

_BF16 = jnp.bfloat16
_F32 = jnp.float32
_U32 = jnp.uint32
_LANES = 128
_TOP_C = 8


def _as_bf16(words):
  return pltpu.bitcast(words, _BF16)


def _cat_cols(parts):
  return parts[0] if len(parts) == 1 else jnp.concatenate(parts, axis=1)


def _block(n):
  return slice(n * _LANES, (n + 1) * _LANES)


def _dot(a, b):
  return jnp.dot(a, b, preferred_element_type=_F32)


def _reduce_all(op, a):
  return op(op(a, axis=1, keepdims=True), axis=0, keepdims=True)


def _work_layout(seq, kt, heads, ring_rows):
  sizes = (
      ("ring", 3 * heads * ring_rows),
      ("mix", kt * seq),
      ("gate", seq),
      ("score", seq // _LANES),
      ("taken", seq // _LANES),
      ("r_sel", _TOP_C),
      ("x_sel", kt * _TOP_C),
      ("end", 0),
  )
  starts = np.cumsum([0] + [n for _, n in sizes])
  return {name: int(start) for (name, _), start in zip(sizes, starts)}


def _kernel(
    x_hbm, mem0_hbm, wq_hbm, wk_hbm, wv_hbm, wo_hbm, wr_hbm, wg_hbm, wu_hbm,
    wd_hbm, gw_hbm,
    out_hbm,
    x_s, wqkv_s, wo_s, wg_s, wu_s, wd_s, work, o_s, mem_s, part_s, pre_s, y_s, idx_s, out_s,
    mem0_ref, wr_ref, gw_ref, sem_x, sem_w, sem_misc, sem_out,
    *, seq, dm, heads, n_mem, seg, ffn, ring_rows, lag_s, lag_pv, o_split, unroll, k_first,
    o_gap, p_rows, newton, get_s, get_pv,
    g_slots, p_gap,
):
  kt = dm // _LANES
  ft = ffn // _LANES
  n_seg = seq // seg
  n_rows = n_mem + seg
  ride = seg - n_mem
  ahead = seq - n_seg * ride
  n_pairs = heads // 2
  half = n_pairs // 2
  x_rows = seq // half
  scale = float(_LANES) ** -0.5
  ffn_blocks = unroll // 2
  ffn_iters = ft // ffn_blocks
  w_hbms = (wq_hbm, wk_hbm, wv_hbm)
  sub = lax.broadcasted_iota(jnp.int32, (8, _LANES), 0)
  lane = lax.broadcasted_iota(jnp.int32, (8, _LANES), 1)

  layout = _work_layout(seq, kt, heads, ring_rows)

  def area(name, row, n, align=8):
    start = layout[name] + row
    return pl.ds(start if isinstance(start, int) or align == 1
                 else pl.multiple_of(start, align), n)

  def ring(h, m, row, n):
    return area("ring", (3 * h + m) * ring_rows + row, n)

  def cols(n):
    return pl.ds(pl.multiple_of(n * _LANES, _LANES), _LANES)

  def x_copies(j):
    n = x_rows // 2
    parts = [pl.ds(pl.multiple_of(j * x_rows + i * n, n), n) for i in range(2)]
    return [pltpu.make_async_copy(x_hbm.at[rows], x_s.at[rows], sem_x.at[j])
            for rows in parts]

  def w_copies(j, m, sem=None):
    return [
        pltpu.make_async_copy(
            w_hbms[m].bitcast(_U32).at[:, p, j], wqkv_s.at[2 * j + p, m],
            sem_w.at[lax.rem(j, 6) if sem is None else sem])
        for p in range(2)]

  small_copies = [
      pltpu.make_async_copy(src, dst, sem_misc.at[1])
      for src, dst in ((mem0_hbm, mem0_ref), (wr_hbm, wr_ref), (gw_hbm, gw_ref))]

  def wo_copy(n):
    return pltpu.make_async_copy(
        wo_hbm.at[:, cols(n)], wo_s.at[n].bitcast(_BF16), sem_misc.at[0])

  def ffn_copies(i):
    width = ffn_blocks * _LANES
    f = pl.ds(pl.multiple_of(i * width, width), width)
    sem = sem_misc.at[2 + (i & 1)]
    return [pltpu.make_async_copy(wg_hbm.at[:, f], wg_s.at[i & 1], sem),
            pltpu.make_async_copy(wu_hbm.at[:, f], wu_s.at[i & 1], sem),
            pltpu.make_async_copy(wd_hbm.at[f], wd_s.at[i & 1], sem)]

  def start_all(copies):
    for cp in copies:
      cp.start()

  def wait_all(copies):
    for cp in copies:
      cp.wait()

  def pair_copies(j):
    return [cp for m in range(3) for cp in w_copies(j, m)]

  start_all(x_copies(0) + w_copies(0, 0) + x_copies(1) + w_copies(0, 1, 4))

  chunks = ahead // p_rows

  def untangle(j, m):
    even = wqkv_s[2 * j, m]
    odd = wqkv_s[2 * j + 1, m]
    wqkv_s[2 * j, m] = (even & np.uint32(0xFFFF)) | (odd << 16)
    wqkv_s[2 * j + 1, m] = (even >> 16) | (odd & np.uint32(0xFFFF0000))

  def project_chunk(h, m, c, before_store=None):
    xa = x_s[c * p_rows:(c + 1) * p_rows]
    w = _as_bf16(wqkv_s[h, m])
    if before_store is not None:
      before_store()
    work[ring(h, m, c * p_rows, p_rows)] = _dot(xa, w)

  def project_pair(j, side_work):
    untangle(j, 0)
    for m in range(3):
      for p in range(2):
        for c in range(chunks):
          def before_store(m=m, p=p, c=c):
            if p == 1 and m < 2 and c == 0:
              untangle(j, m + 1)
            side_work((2 * m + p) * chunks + c)

          project_chunk(2 * j + p, m, c, before_store)

  def gate_and_score(t0, score):
    gw = gw_ref[...].astype(_F32)
    wr = wr_ref[...].astype(_F32)
    rows = pl.ds(pl.multiple_of(t0, 16), 16)
    xs = [x_s[rows, _block(k)].astype(_F32) for k in range(kt)]
    lg = functools.reduce(jnp.add, [xs[k] * gw[k:k + 1] for k in range(kt)])
    r = functools.reduce(jnp.add, [xs[k] * wr[k:k + 1] for k in range(kt)])
    g = jax.nn.sigmoid(jnp.sum(lg, axis=-1, keepdims=True))
    r = jnp.sum(r, axis=-1, keepdims=True)
    work[area("gate", t0, 16)] = jnp.broadcast_to(g, (16, _LANES))
    for k in range(kt):
      work[area("mix", k * seq + t0, 16)] = (1.0 - g) * xs[k]
    for u in range(2):
      for n in range(len(score)):
        here = (n * _LANES + lane) * 8 == t0 + 8 * u
        score[n] = jnp.where(here, r[8 * u:8 * u + 8], score[n])

  def pick_next(c):
    n = seq // _LANES
    score = work[area("score", 0, n)].astype(_BF16).astype(_F32)
    row = lax.broadcasted_iota(jnp.int32, score.shape, 0)
    col = lax.broadcasted_iota(jnp.int32, score.shape, 1)
    tok = ((row >> 3) * (8 * _LANES) + col * 8 + (row & 7)).astype(_F32)
    taken = work[area("taken", 0, n)]
    free = taken == 0.0
    cand = jnp.where(free & (score == score), score, -jnp.inf)
    best = _reduce_all(jnp.max, cand)
    pick = _reduce_all(
        jnp.min, jnp.where(free & (cand == best), tok, float(seq)))
    chosen = tok == pick
    work[area("taken", 0, n)] = jnp.where(
        chosen, jnp.where(c >= 0, 1.0, 0.0), taken)
    r_c = _reduce_all(jnp.sum, jnp.where(chosen, score, 0.0))
    r_sel = area("r_sel", 0, _TOP_C)
    work[r_sel] = jnp.where(sub == c, r_c, work[r_sel])
    t = jnp.clip(pick.astype(jnp.int32)[0, 0], 0, seq - 1)
    idx_s[jnp.maximum(c, 0)] = t
    rows = pl.ds(pl.multiple_of(jnp.where(c >= 0, (t >> 4) * 16, 0), 16), 16)
    row16 = lax.broadcasted_iota(jnp.int32, (16, _LANES), 0)
    for k in range(kt):
      blk = x_s[rows, _block(k)].astype(_F32)
      xt = jnp.sum(jnp.where(row16 == (t & 15), blk, 0.0), axis=0,
                   keepdims=True)
      x_sel = area("x_sel", k * _TOP_C, _TOP_C)
      work[x_sel] = jnp.where(sub == c, xt, work[x_sel])

  def first_pairs():
    wait_all(x_copies(0) + w_copies(0, 0))
    start_all(small_copies + w_copies(0, 2, 5))
    untangle(0, 0)
    for c in range(chunks):
      if c * p_rows == x_rows:
        wait_all(x_copies(1))
        start_all(pair_copies(1))
      for p in range(2):
        project_chunk(p, 0, c)
    for m in (1, 2):
      wait_all(w_copies(0, m, 3 + m))
      start_all(pair_copies(2) if m == 1 else pair_copies(3) + x_copies(2))
      untangle(0, m)
      for p in range(2):
        for c in range(chunks):
          project_chunk(p, m, c)
    wait_all(small_copies + pair_copies(1))

    def side_work(slot):
      if slot == 6 * chunks - 1:
        start_all(pair_copies(4) + pair_copies(5) + x_copies(3) + x_copies(4)
                  + x_copies(5))

    project_pair(1, side_work)

  rounds = n_pairs // 2 - 1
  scoring = rounds - _TOP_C // 2
  pieces = -(-seq // (16 * scoring))

  def other_pairs(i, carry):
    wait_all(pair_copies(2 * i + 2) + pair_copies(2 * i + 3))
    for n in range(3):
      j = 3 * i + n
      pl.when((j >= 2) & (j < half))(lambda j=j: wait_all(x_copies(j)))
    first = jnp.minimum(i * pieces * 16, seq - pieces * 16)
    pages = [area("score", 8 * n, 8) for n in range(seq // (8 * _LANES))]
    score = [work[page] for page in pages]
    for u in range(2):
      def side_work(slot, u=u):
        piece = u * 6 * chunks + slot
        for n in range(pieces):
          if n * g_slots // pieces == piece:
            gate_and_score(first + 16 * n, score)
        if piece == g_slots:
          for page, value in zip(pages, score):
            work[page] = value
        for v in range(2):
          if piece == g_slots + (v + 1) * p_gap:
            pick_next(2 * (i - scoring) + v)
        if piece == 12 * chunks - 1:
          pl.when(i + 2 < rounds)(lambda: start_all(
              pair_copies(2 * i + 6) + pair_copies(2 * i + 7)))
          pl.when(i == 0)(lambda: start_all(x_copies(6) + x_copies(7)))
          pl.when((i >= 1) & (i <= kt // 2))(
              lambda: start_all([wo_copy(2 * i - 2), wo_copy(2 * i - 1)]))
          pl.when(i + 2 == rounds)(lambda: start_all(ffn_copies(0)))

      project_pair(2 * i + 2 + u, side_work)
    return carry

  n_small = layout["end"] - layout["score"]
  work[area("score", 0, n_small)] = jnp.zeros((n_small, _LANES), _F32)
  first_pairs()
  lax.fori_loop(0, rounds, other_pairs, 0)
  mem_s[...] = mem0_ref[...].astype(_F32)

  def ffn_groups(i):
    x_sel = [work[area("x_sel", k * _TOP_C, _TOP_C)] for k in range(kt)]
    act = {}

    def widen(b, which, part):
      ks = range(part * kt // 2, (part + 1) * kt // 2)
      w = (wg_s, wu_s)[which][
          i & 1, ks[0] * _LANES:(ks[-1] + 1) * _LANES, _block(b)]
      r = _dot(_cat_cols([x_sel[k] for k in ks]), w)
      pre_s[b, which, part] = r

    def narrow(b, part):
      if part == 0:
        gate, up = (pre_s[b, n, 0] + pre_s[b, n, 1] for n in range(2))
        act[b] = gate * jax.nn.sigmoid(gate) * up
      span = slice(part * dm // 2, (part + 1) * dm // 2)
      y_s[:, span] += _dot(act[b], wd_s[i & 1, _block(b), span])

    return (
        [functools.partial(widen, b, which, part) for b in range(ffn_blocks)
         for which in range(2) for part in range(2)]
        + [functools.partial(narrow, b, part) for b in range(ffn_blocks)
           for part in range(2)])

  def add_ffn():
    keep = jnp.zeros((8, _LANES), _F32)
    for c in range(_TOP_C):
      keep = jnp.where(sub == c, 1.0 - work[area("gate", idx_s[c], 1, 1)], keep)
    keep = keep * jax.nn.sigmoid(work[area("r_sel", 0, _TOP_C)])
    row16 = lax.broadcasted_iota(jnp.int32, (16, _LANES), 0)
    y = [y_s[:, _block(k)] * keep for k in range(kt)]
    for c in range(_TOP_C):
      t0 = pl.multiple_of((idx_s[c] >> 4) * 16, 16)
      hit = row16 == (idx_s[c] & 15)
      old = [work[area("mix", k * seq + t0, 16)] for k in range(kt)]
      for k in range(kt):
        new = jnp.where(hit, old[k] + y[k][c:c + 1], old[k])
        work[area("mix", k * seq + t0, 16)] = new
        out_s[pl.ds(t0, 16), _block(k)] = new.astype(_BF16)

  n_keys = -(-n_rows // 16) * 16
  qi = lax.broadcasted_iota(jnp.int32, (n_rows, n_keys), 0)
  ki = lax.broadcasted_iota(jnp.int32, (n_rows, n_keys), 1)
  visible = ((qi < n_mem) | (qi >= ki)) & (ki < n_rows)
  hidden = jnp.where(ki < n_rows, -1e9, -jnp.inf).astype(_F32)
  key_pad = jnp.zeros((n_keys - n_rows, _LANES), _F32)

  def step(s, mem, fillers):
    tokens = pl.ds(pl.multiple_of(ahead + s * ride, 8), ride)
    lhs = [
        jnp.concatenate([mem[k], x_s[tokens, _block(k)].astype(_F32)], axis=0
                        ).astype(_BF16) for k in range(kt)]
    put = [lax.rem(ahead + s * ride + 8 * i, ring_rows)
           for i in range(ride // 8)]
    get = lax.rem(s * seg, ring_rows)

    qkv, probs, partial = {}, {}, {}

    def project_part(h, k0, k1):
      words = slice(k0 * _LANES // 2, k1 * _LANES // 2)
      w = _cat_cols([_as_bf16(wqkv_s[h, m, words]) for m in range(3)])
      return _dot(_cat_cols(lhs[k0:k1]), w)

    def gather(h, m):
      if 0 <= h < heads:
        rows = [qkv[h][m], work[ring(h, m, get, seg)]]
        qkv[h][m] = (
            jnp.concatenate(rows, axis=0) if m == 0 else
            jnp.concatenate(rows + [key_pad], axis=0).astype(_BF16))

    def gather_for(h):
      gather(h - get_s, 0)
      gather(h - get_s, 1)
      gather(h - get_pv, 2)

    def project(h):
      if h in partial:
        r = part_s[h] + project_part(h, kt // 2, kt)
      else:
        r = project_part(h, 0, kt)
      parts = [r[:, _block(m)] for m in range(3)]
      for m in range(3):
        for i in range(ride // 8):
          lo = n_mem + 8 * i
          work[ring(h, m, put[i], 8)] = parts[m][lo:lo + 8]
      qkv[h] = [p[0:n_mem] for p in parts]
      gather_for(h)

    def attend_scores(h):
      q, k, _ = qkv[h]
      sc = lax.dot_general(q, k, (((1,), (1,)), ((), ())),
                           preferred_element_type=_F32)
      sc = jnp.where(visible, sc * scale, hidden)
      p = jnp.exp(sc - jnp.max(sc, axis=-1, keepdims=True))
      probs[h] = (p, jnp.sum(p, axis=-1, keepdims=True))

    def attend_values(h):
      p, denom = probs[h]
      if newton:
        inv = pltpu.reciprocal(denom, approx=True)
        inv = inv * (2.0 - denom * inv)
        o_s[:, _block(h)] = _dot(p, qkv[h][2]) * inv
      else:
        o_s[:, _block(h)] = _dot(p, qkv[h][2]) / denom

    k_part = heads * _LANES // o_split
    acc = [None]

    def out_project(i0, i1):
      w = _cat_cols([
          _as_bf16(wo_s[n, i0 * k_part // 2:i1 * k_part // 2])
          for n in range(kt)])
      r = _dot(o_s[:, i0 * k_part:i1 * k_part], w)
      acc[0] = r if acc[0] is None else acc[0] + r

    for h in range(k_first):
      partial[h] = True
      part_s[h] = project_part(h, 0, kt // 2)
    done = 0
    for h in range(heads + lag_pv):
      if h < heads:
        project(h)
      else:
        gather_for(h)
        out_project(done, done + 1)
        done += 1
      if 0 <= h - lag_s < heads:
        attend_scores(h - lag_s)
      if 0 <= h - lag_pv < heads:
        attend_values(h - lag_pv)
    for _ in range(o_gap):
      out_project(done, done + 1)
      done += 1
      if fillers:
        fillers.pop(0)()
    assert not fillers
    out_project(done, o_split)

    rows = pl.ds(pl.multiple_of(s * seg, seg), seg)
    g = work[area("gate", s * seg, seg)]
    for k in range(kt):
      mix = area("mix", k * seq + s * seg, seg)
      mixed = g * acc[0][n_mem:, _block(k)] + work[mix]
      work[mix] = mixed
      out_s[rows, _block(k)] = mixed.astype(_BF16)
    return [acc[0][0:n_mem, _block(k)] for k in range(kt)]

  def out_copy(first, n):
    rows = pl.ds(pl.multiple_of(first * seg, seg), n * seg)
    return pltpu.make_async_copy(out_s.at[rows], out_hbm.at[rows], sem_out)

  def steps(i, carry):
    pl.when(i < ffn_iters)(lambda: wait_all(ffn_copies(i)))
    pl.when(i + 1 < ffn_iters)(lambda: start_all(ffn_copies(i + 1)))

    @pl.when(i == ffn_iters)
    def _():
      add_ffn()
      out_copy(0, ffn_iters * unroll).start()

    pl.when(i > ffn_iters)(lambda: out_copy((i - 1) * unroll, unroll).start())
    groups = ffn_groups(i)
    per_step = len(groups) // unroll
    mem = [mem_s[:, _block(k)] for k in range(kt)]
    for u in range(unroll):
      s = i * unroll + u
      mem = step(s, mem, groups[u * per_step:(u + 1) * per_step])
    mem_s[...] = _cat_cols(mem)
    return carry

  y_s[...] = jnp.zeros(y_s.shape, _F32)
  wait_all([wo_copy(n) for n in range(kt)])
  lax.fori_loop(0, n_seg // unroll, steps, 0)
  out_copy(n_seg - unroll, unroll).start()
  pltpu.make_async_copy(out_s, out_hbm, sem_out).wait()


@functools.partial(jax.jit, static_argnames=("A_seg_len",))
def pallas_gated_mix__memory_aug_recurrent_mem_tr__moe_arch_mod__prompt_kernel(
    A_x: jax.Array,
    A_mem0: jax.Array,
    A_Wq: jax.Array,
    A_Wk: jax.Array,
    A_Wv: jax.Array,
    A_Wo: jax.Array,
    A_seg_len: int,
    B_x: jax.Array,
    B_w_r: jax.Array,
    B_w_gate: jax.Array,
    B_w_up: jax.Array,
    B_w_down: jax.Array,
    gate_w: jax.Array,
):
  del B_x
  batch, seq, dm = A_x.shape
  _, heads, dh = A_Wq.shape
  n_mem = A_mem0.shape[1]
  ffn = B_w_gate.shape[1]
  seg = int(A_seg_len)
  kt = dm // _LANES
  assert batch == 1 and dh == _LANES and (n_mem, seg) == (8, 32)
  assert heads == 4 * _TOP_C == 4 * kt
  ahead = seq - (seq // seg) * (seg - n_mem)
  assert ahead == seq // 4
  ring_rows = -(-(ahead + seg) // seg) * seg
  work_rows = _work_layout(seq, kt, heads, ring_rows)["end"]

  hbm = pl.BlockSpec(memory_space=pl.ANY)
  kernel = functools.partial(
      _kernel, seq=seq, dm=dm, heads=heads, n_mem=n_mem, seg=seg, ffn=ffn,
      ring_rows=ring_rows,
      lag_s=2, lag_pv=5, o_split=16, unroll=4, k_first=1, o_gap=4, p_rows=128, newton=1, get_s=0, get_pv=2, g_slots=38, p_gap=4)
  out = pl.pallas_call(
      kernel,
      out_shape=jax.ShapeDtypeStruct((seq, dm), A_x.dtype),
      in_specs=[hbm] * 11,
      out_specs=hbm,
      scratch_shapes=[
          pltpu.VMEM((seq, dm), _BF16),
          pltpu.VMEM((heads, 3, dm // 2, _LANES), _U32),
          pltpu.VMEM((kt, heads * dh // 2, _LANES), _U32),
          pltpu.VMEM((2, dm, 256), _BF16),
          pltpu.VMEM((2, dm, 256), _BF16),
          pltpu.VMEM((2, 256, dm), _BF16),
          pltpu.VMEM((work_rows, _LANES), _F32),
          pltpu.VMEM((n_mem + seg, heads * dh), _F32),
          pltpu.VMEM((n_mem, dm), _F32),
          pltpu.VMEM((4, seg, 3 * _LANES), _F32),
          pltpu.VMEM((2, 2, 2, _TOP_C, _LANES), _F32),
          pltpu.VMEM((_TOP_C, dm), _F32),
          pltpu.SMEM((_TOP_C,), jnp.int32),
          pltpu.VMEM((seq, dm), _BF16),
          pltpu.VMEM((n_mem, dm), _BF16),
          pltpu.VMEM((kt, _LANES), _BF16),
          pltpu.VMEM((kt, _LANES), _BF16),
          pltpu.SemaphoreType.DMA((heads // 4,)),
          pltpu.SemaphoreType.DMA((6,)),
          pltpu.SemaphoreType.DMA((4,)),
          pltpu.SemaphoreType.DMA,
      ],
      compiler_params=pltpu.CompilerParams(
          vmem_limit_bytes=120 * 2**20, disable_bounds_checks=True,
          disable_semaphore_checks=True),
      name="gated_rmt_mod",
  )(
      A_x.reshape(seq, dm),
      A_mem0.reshape(n_mem, dm),
      A_Wq.reshape(dm // 2, 2, heads, dh),
      A_Wk.reshape(dm // 2, 2, heads, dh),
      A_Wv.reshape(dm // 2, 2, heads, dh),
      A_Wo.reshape(heads * dh, dm),
      B_w_r.reshape(kt, _LANES),
      B_w_gate,
      B_w_up,
      B_w_down,
      gate_w.reshape(kt, _LANES),
  )
  return out.reshape(batch, seq, dm)
```

```python
import functools

import jax
import jax.experimental.pallas as pl
import jax.experimental.pallas.tpu as pltpu
import jax.numpy as jnp
import numpy as np
from jax import lax

_BF16 = jnp.bfloat16
_F32 = jnp.float32
_U32 = jnp.uint32
_LANES = 128
_TOP_C = 8

_UNROLL = 4
_FFN_BLOCKS = 2
_CHUNK = 128
_LAG_SCORES = 2
_LAG_VALUES = 5
_LAG_FETCH_V = 2
_OUT_HEADS = 2
_OUT_EXTRA = 4


def _as_bf16(words):
  return pltpu.bitcast(words, _BF16)


def _cat_cols(parts):
  return parts[0] if len(parts) == 1 else jnp.concatenate(parts, axis=1)


def _block(n):
  return slice(n * _LANES, (n + 1) * _LANES)


def _dot(a, b):
  return jnp.dot(a, b, preferred_element_type=_F32)


def _reduce_all(op, a):
  return op(op(a, axis=1, keepdims=True), axis=0, keepdims=True)


def _start(copies):
  for copy in copies:
    copy.start()


def _wait(copies):
  for copy in copies:
    copy.wait()


def _work_layout(seq, kt, heads, ring_rows):
  sizes = (
      ("ring", 3 * heads * ring_rows),
      ("mix", kt * seq),
      ("gate", seq),
      ("score", seq // _LANES),
      ("taken", seq // _LANES),
      ("r_sel", _TOP_C),
      ("x_sel", kt * _TOP_C),
      ("end", 0),
  )
  starts = np.cumsum([0] + [n for _, n in sizes])
  return {name: int(start) for (name, _), start in zip(sizes, starts)}


def _kernel(
    x_hbm, mem0_hbm, wq_hbm, wk_hbm, wv_hbm, wo_hbm, wr_hbm, wg_hbm, wu_hbm,
    wd_hbm, gw_hbm,
    out_hbm,
    x_s, wqkv_s, wo_s, wg_s, wu_s, wd_s, out_s, work, o_s, mem_s, part_s, pre_s,
    y_s, mem0_s, wr_s, gw_s, idx_s, sem_x, sem_w, sem_misc, sem_out,
    *, heads, seg, ring_rows,
):
  seq, dm = x_hbm.shape
  n_mem = mem0_hbm.shape[0]
  kt = dm // _LANES
  n_seg = seq // seg
  n_rows = n_mem + seg
  ride = seg - n_mem
  ahead = seq - n_seg * ride
  x_rows = ahead // 2
  ffn_iters = wd_hbm.shape[0] // (_FFN_BLOCKS * _LANES)
  sub = lax.broadcasted_iota(jnp.int32, (8, _LANES), 0)
  lane = lax.broadcasted_iota(jnp.int32, (8, _LANES), 1)

  layout = _work_layout(seq, kt, heads, ring_rows)

  def area(name, row, n):
    start = layout[name] + row
    if n % 8 == 0 and not isinstance(start, int):
      start = pl.multiple_of(start, 8)
    return pl.ds(start, n)

  def ring(h, m, row, n):
    return area("ring", (3 * h + m) * ring_rows + row, n)

  def x_copies(j):
    n = x_rows // 2
    parts = [pl.ds(pl.multiple_of(j * x_rows + i * n, n), n) for i in range(2)]
    return [pltpu.make_async_copy(x_hbm.at[rows], x_s.at[rows], sem_x.at[j])
            for rows in parts]

  def w_copies(j, m, sem):
    words = (wq_hbm, wk_hbm, wv_hbm)[m].bitcast(_U32)
    return [pltpu.make_async_copy(
        words.at[:, p, j], wqkv_s.at[2 * j + p, m], sem_w.at[sem])
            for p in range(2)]

  def pair_copies(j):
    sem = j % 6 if isinstance(j, int) else lax.rem(j, 6)
    return [copy for m in range(3) for copy in w_copies(j, m, sem)]

  def wo_copy(n):
    cols = pl.ds(pl.multiple_of(n * _LANES, _LANES), _LANES)
    return pltpu.make_async_copy(
        wo_hbm.at[:, cols], wo_s.at[n].bitcast(_BF16), sem_misc.at[0])

  def ffn_copies(i):
    width = _FFN_BLOCKS * _LANES
    f = pl.ds(pl.multiple_of(i * width, width), width)
    sem = sem_misc.at[2 + (i & 1)]
    return [pltpu.make_async_copy(wg_hbm.at[:, f], wg_s.at[i & 1], sem),
            pltpu.make_async_copy(wu_hbm.at[:, f], wu_s.at[i & 1], sem),
            pltpu.make_async_copy(wd_hbm.at[f], wd_s.at[i & 1], sem)]

  small_copies = [
      pltpu.make_async_copy(src, dst, sem_misc.at[1])
      for src, dst in ((mem0_hbm, mem0_s), (wr_hbm, wr_s), (gw_hbm, gw_s))]

  def out_copy(first, n):
    rows = pl.ds(pl.multiple_of(first * seg, seg), n * seg)
    return pltpu.make_async_copy(out_s.at[rows], out_hbm.at[rows], sem_out)

  first_w = [w_copies(0, m, sem) for m, sem in enumerate((0, 4, 5))]
  _start(x_copies(0) + first_w[0] + x_copies(1) + first_w[1])

  def gate_and_score(t0, score):
    gw = gw_s[...].astype(_F32)
    wr = wr_s[...].astype(_F32)
    rows = pl.ds(pl.multiple_of(t0, 16), 16)
    xs = [x_s[rows, _block(k)].astype(_F32) for k in range(kt)]
    logit = functools.reduce(jnp.add, [xs[k] * gw[k:k + 1] for k in range(kt)])
    r = functools.reduce(jnp.add, [xs[k] * wr[k:k + 1] for k in range(kt)])
    g = jax.nn.sigmoid(jnp.sum(logit, axis=-1, keepdims=True))
    r = jnp.sum(r, axis=-1, keepdims=True)
    work[area("gate", t0, 16)] = jnp.broadcast_to(g, (16, _LANES))
    for k in range(kt):
      work[area("mix", k * seq + t0, 16)] = (1.0 - g) * xs[k]
    for u in range(2):
      for n in range(len(score)):
        here = (n * _LANES + lane) * 8 == t0 + 8 * u
        score[n] = jnp.where(here, r[8 * u:8 * u + 8], score[n])

  def route_next(c):
    n = seq // _LANES
    score = work[area("score", 0, n)].astype(_BF16).astype(_F32)
    row = lax.broadcasted_iota(jnp.int32, score.shape, 0)
    col = lax.broadcasted_iota(jnp.int32, score.shape, 1)
    tok = ((row >> 3) * (8 * _LANES) + col * 8 + (row & 7)).astype(_F32)
    taken = work[area("taken", 0, n)]
    free = taken == 0.0
    cand = jnp.where(free & (score == score), score, -jnp.inf)
    best = _reduce_all(jnp.max, cand)
    pick = _reduce_all(
        jnp.min, jnp.where(free & (cand == best), tok, float(seq)))
    chosen = tok == pick
    work[area("taken", 0, n)] = jnp.where(
        chosen, jnp.where(c >= 0, 1.0, 0.0), taken)
    r_c = _reduce_all(jnp.sum, jnp.where(chosen, score, 0.0))
    r_sel = area("r_sel", 0, _TOP_C)
    work[r_sel] = jnp.where(sub == c, r_c, work[r_sel])
    t = jnp.clip(pick.astype(jnp.int32)[0, 0], 0, seq - 1)
    idx_s[jnp.maximum(c, 0)] = t
    rows = pl.ds(pl.multiple_of(jnp.where(c >= 0, (t >> 4) * 16, 0), 16), 16)
    row16 = lax.broadcasted_iota(jnp.int32, (16, _LANES), 0)
    for k in range(kt):
      blk = x_s[rows, _block(k)].astype(_F32)
      xt = jnp.sum(jnp.where(row16 == (t & 15), blk, 0.0), axis=0,
                   keepdims=True)
      x_sel = area("x_sel", k * _TOP_C, _TOP_C)
      work[x_sel] = jnp.where(sub == c, xt, work[x_sel])

  chunks = ahead // _CHUNK
  slots = 6 * chunks

  def untangle(j, m):
    even = wqkv_s[2 * j, m]
    odd = wqkv_s[2 * j + 1, m]
    wqkv_s[2 * j, m] = (even & np.uint32(0xFFFF)) | (odd << 16)
    wqkv_s[2 * j + 1, m] = (even >> 16) | (odd & np.uint32(0xFFFF0000))

  def project_chunk(h, m, c, side_work=None):
    xa = x_s[c * _CHUNK:(c + 1) * _CHUNK]
    w = _as_bf16(wqkv_s[h, m])
    if side_work is not None:
      side_work()
    work[ring(h, m, c * _CHUNK, _CHUNK)] = _dot(xa, w)

  def project_pair(j, side_work):
    untangle(j, 0)
    for m in range(3):
      for p in range(2):
        for c in range(chunks):
          def between(m=m, p=p, c=c):
            if p == 1 and m < 2 and c == 0:
              untangle(j, m + 1)
            side_work((2 * m + p) * chunks + c)

          project_chunk(2 * j + p, m, c, between)

  def first_pairs():
    _wait(x_copies(0) + first_w[0])
    _start(small_copies + first_w[2])
    untangle(0, 0)
    for c in range(chunks):
      if c * _CHUNK == x_rows:
        _wait(x_copies(1))
        _start(pair_copies(1))
      for p in range(2):
        project_chunk(p, 0, c)
    for m in (1, 2):
      _wait(first_w[m])
      _start(pair_copies(2) if m == 1 else pair_copies(3) + x_copies(2))
      untangle(0, m)
      for p in range(2):
        for c in range(chunks):
          project_chunk(p, m, c)
    _wait(small_copies + pair_copies(1))

    def side_work(slot):
      if slot == slots - 1:
        _start(pair_copies(4) + pair_copies(5) + x_copies(3) + x_copies(4)
               + x_copies(5))

    project_pair(1, side_work)

  rounds = heads // 4 - 1
  scoring = rounds - _TOP_C // 2
  pieces = -(-seq // (16 * scoring))
  gate_slots = 2 * slots - 10

  def other_pairs(i, carry):
    _wait(pair_copies(2 * i + 2) + pair_copies(2 * i + 3))
    for n in range(3):
      j = 3 * i + n
      pl.when((j >= 2) & (j < seq // x_rows))(lambda j=j: _wait(x_copies(j)))
    first = jnp.minimum(i * pieces * 16, seq - pieces * 16)
    pages = [area("score", 8 * n, 8) for n in range(seq // (8 * _LANES))]
    score = [work[page] for page in pages]

    def side_work(slot):
      for n in range(pieces):
        if n * gate_slots // pieces == slot:
          gate_and_score(first + 16 * n, score)
      if slot == gate_slots:
        for page, value in zip(pages, score):
          work[page] = value
      for v in range(2):
        if slot == gate_slots + 4 * (v + 1):
          route_next(2 * (i - scoring) + v)
      if slot == 2 * slots - 1:
        pl.when(i + 2 < rounds)(lambda: _start(
            pair_copies(2 * i + 6) + pair_copies(2 * i + 7)))
        pl.when(i == 0)(lambda: _start(x_copies(6) + x_copies(7)))
        pl.when((i >= 1) & (i <= kt // 2))(
            lambda: _start([wo_copy(2 * i - 2), wo_copy(2 * i - 1)]))
        pl.when(i + 2 == rounds)(lambda: _start(ffn_copies(0) + ffn_copies(1)))

    for u in range(2):
      project_pair(2 * i + 2 + u, lambda slot, u=u: side_work(u * slots + slot))
    return carry

  n_small = layout["end"] - layout["score"]
  work[area("score", 0, n_small)] = jnp.zeros((n_small, _LANES), _F32)
  y_s[...] = jnp.zeros(y_s.shape, _F32)
  first_pairs()
  lax.fori_loop(0, rounds, other_pairs, 0)

  def ffn_groups(i):
    x_sel = [work[area("x_sel", k * _TOP_C, _TOP_C)] for k in range(kt)]
    act = {}

    def widen(b, which, part):
      ks = slice(part * kt // 2, (part + 1) * kt // 2)
      w = (wg_s, wu_s)[which][
          i & 1, ks.start * _LANES:ks.stop * _LANES, _block(b)]
      pre_s[b, which, part] = _dot(_cat_cols(x_sel[ks]), w)

    def narrow(b, part):
      if part == 0:
        gate, up = (pre_s[b, n, 0] + pre_s[b, n, 1] for n in range(2))
        act[b] = gate * jax.nn.sigmoid(gate) * up
      cols = slice(part * dm // 2, (part + 1) * dm // 2)
      y_s[:, cols] += _dot(act[b], wd_s[i & 1, _block(b), cols])

    return (
        [functools.partial(widen, b, which, part) for b in range(_FFN_BLOCKS)
         for which in range(2) for part in range(2)]
        + [functools.partial(narrow, b, part) for b in range(_FFN_BLOCKS)
           for part in range(2)])

  def add_ffn():
    keep = jnp.zeros((8, _LANES), _F32)
    for c in range(_TOP_C):
      keep = jnp.where(sub == c, 1.0 - work[area("gate", idx_s[c], 1)], keep)
    keep = keep * jax.nn.sigmoid(work[area("r_sel", 0, _TOP_C)])
    y = [y_s[:, _block(k)] * keep for k in range(kt)]
    for c in range(_TOP_C):
      t0 = pl.multiple_of((idx_s[c] >> 3) * 8, 8)
      hit = sub == (idx_s[c] & 7)
      old = [work[area("mix", k * seq + t0, 8)] for k in range(kt)]
      for k in range(kt):
        new = jnp.where(hit, old[k] + y[k][c:c + 1], old[k])
        work[area("mix", k * seq + t0, 8)] = new
        out_s[pl.ds(t0, 8), _block(k)] = new.astype(_BF16)

  scale = float(_LANES) ** -0.5
  n_keys = -(-n_rows // 16) * 16
  qi = lax.broadcasted_iota(jnp.int32, (n_rows, n_keys), 0)
  ki = lax.broadcasted_iota(jnp.int32, (n_rows, n_keys), 1)
  visible = ((qi < n_mem) | (qi >= ki)) & (ki < n_rows)
  hidden = jnp.where(ki < n_rows, -1e9, -jnp.inf).astype(_F32)
  key_pad = jnp.zeros((n_keys - n_rows, _LANES), _F32)

  def step(s, mem, fillers):
    tokens = pl.ds(pl.multiple_of(ahead + s * ride, 8), ride)
    lhs = [
        jnp.concatenate([mem[k], x_s[tokens, _block(k)].astype(_F32)], axis=0
                        ).astype(_BF16) for k in range(kt)]
    put = [lax.rem(ahead + s * ride + 8 * i, ring_rows)
           for i in range(ride // 8)]
    get = lax.rem(s * seg, ring_rows)
    qkv, probs = {}, {}

    def project_part(h, k0, k1):
      words = slice(k0 * _LANES // 2, k1 * _LANES // 2)
      w = _cat_cols([_as_bf16(wqkv_s[h, m, words]) for m in range(3)])
      return _dot(_cat_cols(lhs[k0:k1]), w)

    def project(h):
      if h == 0:
        part_s[...] = project_part(h, 0, kt // 2)
        r = part_s[...] + project_part(h, kt // 2, kt)
      else:
        r = project_part(h, 0, kt)
      for m in range(3):
        for i in range(ride // 8):
          work[ring(h, m, put[i], 8)] = r[
              n_mem + 8 * i:n_mem + 8 * i + 8, _block(m)]
      qkv[h] = [r[0:n_mem, _block(m)] for m in range(3)]

    def fetch(h, m):
      if 0 <= h < heads:
        rows = [qkv[h][m], work[ring(h, m, get, seg)]]
        qkv[h][m] = (
            jnp.concatenate(rows, axis=0) if m == 0 else
            jnp.concatenate(rows + [key_pad], axis=0).astype(_BF16))

    def attend_scores(h):
      q, k, _ = qkv[h]
      sc = lax.dot_general(q, k, (((1,), (1,)), ((), ())),
                           preferred_element_type=_F32)
      sc = jnp.where(visible, sc * scale, hidden)
      p = jnp.exp(sc - jnp.max(sc, axis=-1, keepdims=True))
      probs[h] = (p, jnp.sum(p, axis=-1, keepdims=True))

    def attend_values(h):
      p, denom = probs[h]
      inv = pltpu.reciprocal(denom, approx=True)
      inv = inv * (2.0 - denom * inv)
      o_s[:, _block(h)] = _dot(p, qkv[h][2]) * inv

    acc, done = None, 0

    def out_project(n):
      nonlocal acc, done
      lo, hi = done * _LANES, (done + n) * _LANES
      w = _cat_cols([_as_bf16(wo_s[k, lo // 2:hi // 2]) for k in range(kt)])
      r = _dot(o_s[:, lo:hi], w)
      acc = r if acc is None else acc + r
      done += n

    for h in range(heads + _LAG_VALUES):
      if h < heads:
        project(h)
      fetch(h, 0)
      fetch(h, 1)
      fetch(h - _LAG_FETCH_V, 2)
      if h >= heads:
        out_project(_OUT_HEADS)
      if 0 <= h - _LAG_SCORES < heads:
        attend_scores(h - _LAG_SCORES)
      if 0 <= h - _LAG_VALUES < heads:
        attend_values(h - _LAG_VALUES)
    assert len(fillers) <= _OUT_EXTRA
    for n in range(_OUT_EXTRA):
      out_project(_OUT_HEADS)
      if n < len(fillers):
        fillers[n]()
    out_project(heads - done)

    g = work[area("gate", s * seg, seg)]
    rows = pl.ds(pl.multiple_of(s * seg, seg), seg)
    for k in range(kt):
      mix = area("mix", k * seq + s * seg, seg)
      mixed = g * acc[n_mem:, _block(k)] + work[mix]
      work[mix] = mixed
      out_s[rows, _block(k)] = mixed.astype(_BF16)
    return [acc[0:n_mem, _block(k)] for k in range(kt)]

  def steps(i, carry):
    pl.when(i < ffn_iters)(lambda: _wait(ffn_copies(i)))

    @pl.when(i == ffn_iters)
    def _():
      add_ffn()
      out_copy(0, ffn_iters * _UNROLL).start()

    groups = ffn_groups(i)
    per_step = len(groups) // _UNROLL
    mem = [mem_s[:, _block(k)] for k in range(kt)]
    for u in range(_UNROLL):
      mem = step(i * _UNROLL + u, mem, groups[u * per_step:(u + 1) * per_step])
    mem_s[...] = _cat_cols(mem)
    pl.when(i + 2 < ffn_iters)(lambda: _start(ffn_copies(i + 2)))
    pl.when(i >= ffn_iters)(lambda: out_copy(i * _UNROLL, _UNROLL).start())
    return carry

  mem_s[...] = mem0_s[...].astype(_F32)
  _wait([wo_copy(n) for n in range(kt)])
  lax.fori_loop(0, n_seg // _UNROLL, steps, 0)
  pltpu.make_async_copy(out_s, out_hbm, sem_out).wait()


@functools.partial(jax.jit, static_argnames=("A_seg_len",))
def pallas_gated_mix__memory_aug_recurrent_mem_tr__moe_arch_mod__prompt_kernel(
    A_x: jax.Array,
    A_mem0: jax.Array,
    A_Wq: jax.Array,
    A_Wk: jax.Array,
    A_Wv: jax.Array,
    A_Wo: jax.Array,
    A_seg_len: int,
    B_x: jax.Array,
    B_w_r: jax.Array,
    B_w_gate: jax.Array,
    B_w_up: jax.Array,
    B_w_down: jax.Array,
    gate_w: jax.Array,
):
  del B_x
  batch, seq, dm = A_x.shape
  _, heads, dh = A_Wq.shape
  n_mem = A_mem0.shape[1]
  seg = int(A_seg_len)
  assert (batch, seq, dm, heads, dh) == (1, 2048, 1024, 32, _LANES)
  assert (n_mem, seg, B_w_down.shape[0]) == (8, 32, 3584)
  kt = dm // _LANES
  ring_rows = seq // 4 + seg
  width = _FFN_BLOCKS * _LANES

  hbm = pl.BlockSpec(memory_space=pl.ANY)
  out = pl.pallas_call(
      functools.partial(_kernel, heads=heads, seg=seg, ring_rows=ring_rows),
      out_shape=jax.ShapeDtypeStruct((seq, dm), A_x.dtype),
      in_specs=[hbm] * 11,
      out_specs=hbm,
      scratch_shapes=[
          pltpu.VMEM((seq, dm), _BF16),
          pltpu.VMEM((heads, 3, dm // 2, _LANES), _U32),
          pltpu.VMEM((kt, heads * dh // 2, _LANES), _U32),
          pltpu.VMEM((2, dm, width), _BF16),
          pltpu.VMEM((2, dm, width), _BF16),
          pltpu.VMEM((2, width, dm), _BF16),
          pltpu.VMEM((seq, dm), _BF16),
          pltpu.VMEM(
              (_work_layout(seq, kt, heads, ring_rows)["end"], _LANES), _F32),
          pltpu.VMEM((n_mem + seg, heads * dh), _F32),
          pltpu.VMEM((n_mem, dm), _F32),
          pltpu.VMEM((seg, 3 * _LANES), _F32),
          pltpu.VMEM((_FFN_BLOCKS, 2, 2, _TOP_C, _LANES), _F32),
          pltpu.VMEM((_TOP_C, dm), _F32),
          pltpu.VMEM((n_mem, dm), _BF16),
          pltpu.VMEM((kt, _LANES), _BF16),
          pltpu.VMEM((kt, _LANES), _BF16),
          pltpu.SMEM((_TOP_C,), jnp.int32),
          pltpu.SemaphoreType.DMA((8,)),
          pltpu.SemaphoreType.DMA((6,)),
          pltpu.SemaphoreType.DMA((4,)),
          pltpu.SemaphoreType.DMA,
      ],
      compiler_params=pltpu.CompilerParams(
          vmem_limit_bytes=100 * 2**20,
          disable_bounds_checks=True,
          disable_semaphore_checks=True,
      ),
      name="gated_rmt_mod",
  )(
      A_x.reshape(seq, dm),
      A_mem0.reshape(n_mem, dm),
      A_Wq.reshape(dm // 2, 2, heads, dh),
      A_Wk.reshape(dm // 2, 2, heads, dh),
      A_Wv.reshape(dm // 2, 2, heads, dh),
      A_Wo.reshape(heads * dh, dm),
      B_w_r.reshape(kt, _LANES),
      B_w_gate,
      B_w_up,
      B_w_down,
      gate_w.reshape(kt, _LANES),
  )
  return out.reshape(batch, seq, dm)
```

```python
import functools

import jax
import jax.experimental.pallas as pl
import jax.experimental.pallas.tpu as pltpu
import jax.numpy as jnp
import numpy as np
from jax import lax

_BF16 = jnp.bfloat16
_F32 = jnp.float32
_U32 = jnp.uint32
_LANES = 128
_TOP_C = 8

_UNROLL = 4
_FFN_BLOCKS = 2
_CHUNK = 128
_T32 = 1
_UNSHARE = -1
_SPLIT = 0
_LAG_TAILS = 4
_LAG_ATTEND = 4
_LAG_FETCH_V = 4
_OUT_HEADS = 2
_OUT_EXTRA = 3


def _as_bf16(words):
  return pltpu.bitcast(words, _BF16)


def _cat_cols(parts):
  return parts[0] if len(parts) == 1 else jnp.concatenate(parts, axis=1)


def _block(n):
  return slice(n * _LANES, (n + 1) * _LANES)


def _dot(a, b):
  return jnp.dot(a, b, preferred_element_type=_F32)


def _reduce_all(op, a):
  return op(op(a, axis=1, keepdims=True), axis=0, keepdims=True)


def _start(copies):
  for copy in copies:
    copy.start()


def _wait(copies):
  for copy in copies:
    copy.wait()


def _work_layout(seq, kt, heads, ring_rows):
  sizes = (
      ("ring", 3 * heads * ring_rows),
      ("mix", kt * seq),
      ("gate", seq),
      ("score", seq // _LANES),
      ("taken", seq // _LANES),
      ("r_sel", _TOP_C),
      ("x_sel", kt * _TOP_C),
      ("end", 0),
  )
  starts = np.cumsum([0] + [n for _, n in sizes])
  return {name: int(start) for (name, _), start in zip(sizes, starts)}


def _kernel(
    x_hbm, mem0_hbm, wq_hbm, wk_hbm, wv_hbm, wo_hbm, wr_hbm, wg_hbm, wu_hbm,
    wd_hbm, gw_hbm,
    out_hbm,
    x_s, wqkv_s, wo_s, wg_s, wu_s, wd_s, out_s, work, o_s, mem_s, part_s, pre_s,
    y_s, mem0_s, wr_s, gw_s, idx_s, sem_x, sem_w, sem_misc, sem_out,
    *, heads, seg, ring_rows,
):
  seq, dm = x_hbm.shape
  n_mem = mem0_hbm.shape[0]
  kt = dm // _LANES
  n_seg = seq // seg
  n_rows = n_mem + seg
  ride = seg - n_mem
  ahead = seq - n_seg * ride
  x_rows = ahead // 2
  ffn_iters = wd_hbm.shape[0] // (_FFN_BLOCKS * _LANES)
  sub = lax.broadcasted_iota(jnp.int32, (8, _LANES), 0)
  lane = lax.broadcasted_iota(jnp.int32, (8, _LANES), 1)

  layout = _work_layout(seq, kt, heads, ring_rows)

  def area(name, row, n):
    start = layout[name] + row
    if n % 8 == 0 and not isinstance(start, int):
      start = pl.multiple_of(start, 8)
    return pl.ds(start, n)

  def ring(h, m, row, n):
    return area("ring", (3 * h + m) * ring_rows + row, n)

  def x_copies(j):
    n = x_rows // 2
    parts = [pl.ds(pl.multiple_of(j * x_rows + i * n, n), n) for i in range(2)]
    return [pltpu.make_async_copy(x_hbm.at[rows], x_s.at[rows], sem_x.at[j])
            for rows in parts]

  def w_copies(j, m, sem):
    words = (wq_hbm, wk_hbm, wv_hbm)[m].bitcast(_U32)
    return [pltpu.make_async_copy(
        words.at[:, p, j], wqkv_s.at[2 * j + p, m], sem_w.at[sem])
            for p in range(2)]

  def pair_copies(j):
    sem = j % 6 if isinstance(j, int) else lax.rem(j, 6)
    return [copy for m in range(3) for copy in w_copies(j, m, sem)]

  def wo_copy(n):
    cols = pl.ds(pl.multiple_of(n * _LANES, _LANES), _LANES)
    return pltpu.make_async_copy(
        wo_hbm.at[:, cols], wo_s.at[n].bitcast(_BF16), sem_misc.at[0])

  def ffn_copies(i):
    width = _FFN_BLOCKS * _LANES
    f = pl.ds(pl.multiple_of(i * width, width), width)
    sem = sem_misc.at[2 + (i & 1)]
    return [pltpu.make_async_copy(wg_hbm.at[:, f], wg_s.at[i & 1], sem),
            pltpu.make_async_copy(wu_hbm.at[:, f], wu_s.at[i & 1], sem),
            pltpu.make_async_copy(wd_hbm.at[f], wd_s.at[i & 1], sem)]

  small_copies = [
      pltpu.make_async_copy(src, dst, sem_misc.at[1])
      for src, dst in ((mem0_hbm, mem0_s), (wr_hbm, wr_s), (gw_hbm, gw_s))]

  def out_copy(first, n):
    rows = pl.ds(pl.multiple_of(first * seg, seg), n * seg)
    return pltpu.make_async_copy(out_s.at[rows], out_hbm.at[rows], sem_out)

  first_w = [w_copies(0, m, sem) for m, sem in enumerate((0, 4, 5))]
  _start(x_copies(0) + first_w[0] + x_copies(1) + first_w[1])

  def gate_and_score(t0, score):
    gw = gw_s[...].astype(_F32)
    wr = wr_s[...].astype(_F32)
    rows = pl.ds(pl.multiple_of(t0, 16), 16)
    xs = [x_s[rows, _block(k)].astype(_F32) for k in range(kt)]
    logit = functools.reduce(jnp.add, [xs[k] * gw[k:k + 1] for k in range(kt)])
    r = functools.reduce(jnp.add, [xs[k] * wr[k:k + 1] for k in range(kt)])
    g = jax.nn.sigmoid(jnp.sum(logit, axis=-1, keepdims=True))
    r = jnp.sum(r, axis=-1, keepdims=True)
    work[area("gate", t0, 16)] = jnp.broadcast_to(g, (16, _LANES))
    for k in range(kt):
      work[area("mix", k * seq + t0, 16)] = (1.0 - g) * xs[k]
    for u in range(2):
      for n in range(len(score)):
        here = (n * _LANES + lane) * 8 == t0 + 8 * u
        score[n] = jnp.where(here, r[8 * u:8 * u + 8], score[n])

  def route_next(c):
    n = seq // _LANES
    score = work[area("score", 0, n)].astype(_BF16).astype(_F32)
    row = lax.broadcasted_iota(jnp.int32, score.shape, 0)
    col = lax.broadcasted_iota(jnp.int32, score.shape, 1)
    tok = ((row >> 3) * (8 * _LANES) + col * 8 + (row & 7)).astype(_F32)
    taken = work[area("taken", 0, n)]
    free = taken == 0.0
    cand = jnp.where(free & (score == score), score, -jnp.inf)
    best = _reduce_all(jnp.max, cand)
    pick = _reduce_all(
        jnp.min, jnp.where(free & (cand == best), tok, float(seq)))
    chosen = tok == pick
    work[area("taken", 0, n)] = jnp.where(
        chosen, jnp.where(c >= 0, 1.0, 0.0), taken)
    r_c = _reduce_all(jnp.sum, jnp.where(chosen, score, 0.0))
    r_sel = area("r_sel", 0, _TOP_C)
    work[r_sel] = jnp.where(sub == c, r_c, work[r_sel])
    t = jnp.clip(pick.astype(jnp.int32)[0, 0], 0, seq - 1)
    idx_s[jnp.maximum(c, 0)] = t
    rows = pl.ds(pl.multiple_of(jnp.where(c >= 0, (t >> 4) * 16, 0), 16), 16)
    row16 = lax.broadcasted_iota(jnp.int32, (16, _LANES), 0)
    for k in range(kt):
      blk = x_s[rows, _block(k)].astype(_F32)
      xt = jnp.sum(jnp.where(row16 == (t & 15), blk, 0.0), axis=0,
                   keepdims=True)
      x_sel = area("x_sel", k * _TOP_C, _TOP_C)
      work[x_sel] = jnp.where(sub == c, xt, work[x_sel])

  chunks = ahead // _CHUNK
  slots = 6 * chunks

  def untangle(j, m):
    even = wqkv_s[2 * j, m]
    odd = wqkv_s[2 * j + 1, m]
    wqkv_s[2 * j, m] = (even & np.uint32(0xFFFF)) | (odd << 16)
    wqkv_s[2 * j + 1, m] = (even >> 16) | (odd & np.uint32(0xFFFF0000))

  def project_chunk(h, m, c, side_work=None):
    xa = x_s[c * _CHUNK:(c + 1) * _CHUNK]
    w = _as_bf16(wqkv_s[h, m])
    if side_work is not None:
      side_work()
    work[ring(h, m, c * _CHUNK, _CHUNK)] = _dot(xa, w)

  def project_pair(j, side_work):
    untangle(j, 0)
    for m in range(3):
      for p in range(2):
        for c in range(chunks):
          def between(m=m, p=p, c=c):
            if p == 1 and m < 2 and c == 0:
              untangle(j, m + 1)
            side_work((2 * m + p) * chunks + c)

          project_chunk(2 * j + p, m, c, between)

  def first_pairs():
    _wait(x_copies(0) + first_w[0])
    _start(small_copies + first_w[2])
    untangle(0, 0)
    for c in range(chunks):
      if c * _CHUNK == x_rows:
        _wait(x_copies(1))
        _start(pair_copies(1))
      for p in range(2):
        project_chunk(p, 0, c)
    for m in (1, 2):
      _wait(first_w[m])
      _start(pair_copies(2) if m == 1 else pair_copies(3) + x_copies(2))
      untangle(0, m)
      for p in range(2):
        for c in range(chunks):
          project_chunk(p, m, c)
    _wait(small_copies + pair_copies(1))

    def side_work(slot):
      if slot == slots - 1:
        _start(pair_copies(4) + pair_copies(5) + x_copies(3) + x_copies(4)
               + x_copies(5))

    project_pair(1, side_work)

  rounds = heads // 4 - 1
  scoring = rounds - _TOP_C // 2
  pieces = -(-seq // (16 * scoring))
  gate_slots = 2 * slots - 10

  def other_pairs(i, carry):
    _wait(pair_copies(2 * i + 2) + pair_copies(2 * i + 3))
    for n in range(3):
      j = 3 * i + n
      pl.when((j >= 2) & (j < seq // x_rows))(lambda j=j: _wait(x_copies(j)))
    first = jnp.minimum(i * pieces * 16, seq - pieces * 16)
    pages = [area("score", 8 * n, 8) for n in range(seq // (8 * _LANES))]
    score = [work[page] for page in pages]

    def side_work(slot):
      for n in range(pieces):
        if n * gate_slots // pieces == slot:
          gate_and_score(first + 16 * n, score)
      if slot == gate_slots:
        for page, value in zip(pages, score):
          work[page] = value
      for v in range(2):
        if slot == gate_slots + 4 * (v + 1):
          route_next(2 * (i - scoring) + v)
      if slot == 2 * slots - 1:
        pl.when(i + 2 < rounds)(lambda: _start(
            pair_copies(2 * i + 6) + pair_copies(2 * i + 7)))
        pl.when(i == 0)(lambda: _start(x_copies(6) + x_copies(7)))
        pl.when((i >= 1) & (i <= kt // 2))(
            lambda: _start([wo_copy(2 * i - 2), wo_copy(2 * i - 1)]))
        pl.when(i + 2 == rounds)(lambda: _start(ffn_copies(0) + ffn_copies(1)))

    for u in range(2):
      project_pair(2 * i + 2 + u, lambda slot, u=u: side_work(u * slots + slot))
    return carry

  n_small = layout["end"] - layout["score"]
  work[area("score", 0, n_small)] = jnp.zeros((n_small, _LANES), _F32)
  y_s[...] = jnp.zeros(y_s.shape, _F32)
  first_pairs()
  lax.fori_loop(0, rounds, other_pairs, 0)

  def ffn_groups(i):
    x_sel = [work[area("x_sel", k * _TOP_C, _TOP_C)] for k in range(kt)]
    act = {}

    def widen(b, which, part):
      ks = slice(part * kt // 2, (part + 1) * kt // 2)
      w = (wg_s, wu_s)[which][
          i & 1, ks.start * _LANES:ks.stop * _LANES, _block(b)]
      pre_s[b, which, part] = _dot(_cat_cols(x_sel[ks]), w)

    def narrow(b, part):
      if part == 0:
        gate, up = (pre_s[b, n, 0] + pre_s[b, n, 1] for n in range(2))
        act[b] = gate * jax.nn.sigmoid(gate) * up
      cols = slice(part * dm // 2, (part + 1) * dm // 2)
      y_s[:, cols] += _dot(act[b], wd_s[i & 1, _block(b), cols])

    return (
        [functools.partial(widen, b, which, part) for b in range(_FFN_BLOCKS)
         for which in range(2) for part in range(2)]
        + [functools.partial(narrow, b, part) for b in range(_FFN_BLOCKS)
           for part in range(2)])

  def add_ffn():
    keep = jnp.zeros((8, _LANES), _F32)
    for c in range(_TOP_C):
      keep = jnp.where(sub == c, 1.0 - work[area("gate", idx_s[c], 1)], keep)
    keep = keep * jax.nn.sigmoid(work[area("r_sel", 0, _TOP_C)])
    y = [y_s[:, _block(k)] * keep for k in range(kt)]
    for c in range(_TOP_C):
      t0 = pl.multiple_of((idx_s[c] >> 3) * 8, 8)
      hit = sub == (idx_s[c] & 7)
      old = [work[area("mix", k * seq + t0, 8)] for k in range(kt)]
      for k in range(kt):
        new = jnp.where(hit, old[k] + y[k][c:c + 1], old[k])
        work[area("mix", k * seq + t0, 8)] = new
        out_s[pl.ds(t0, 8), _block(k)] = new.astype(_BF16)

  scale = float(_LANES) ** -0.5
  team = _LANES // n_rows
  qi = lax.broadcasted_iota(jnp.int32, (n_rows, _LANES), 0)
  col = lax.broadcasted_iota(jnp.int32, (1, _LANES), 1)
  window = [(col >= c * n_rows) & (col < (c + 1) * n_rows) for c in range(team)]
  ki = col - sum(jnp.where(window[c], c * n_rows, 0) for c in range(team))
  visible = ((qi < n_mem) | (qi >= ki)) & (col < team * n_rows)
  hidden = jnp.where(col < team * n_rows, -1e9, -jnp.inf).astype(_F32)
  teams = ([tuple(range(heads % team))] if heads % team else []) + [
      tuple(range(h, h + team)) for h in range(heads % team, heads, team)]

  def by_window(parts):
    out = parts[-1]
    for c in range(len(parts) - 1):
      out = jnp.where(window[c], parts[c], out)
    return out

  def word_rows(c):
    word = lax.broadcasted_iota(jnp.int32, (_LANES // 2, 1), 0)
    return (word >= c * n_rows // 2) & (word < (c + 1) * n_rows // 2)

  def step(s, mem, fillers):
    tokens = pl.ds(pl.multiple_of(ahead + s * ride, 8), ride)
    lhs = [
        jnp.concatenate([mem[k], x_s[tokens, _block(k)].astype(_F32)], axis=0
                        ).astype(_BF16) for k in range(kt)]
    put = [lax.rem(ahead + s * ride + 8 * i, ring_rows)
           for i in range(ride // 8)]
    get = lax.rem(s * seg, ring_rows)
    qkv, probs = {}, {}

    def project_part(h, k0, k1):
      words = slice(k0 * _LANES // 2, k1 * _LANES // 2)
      w = _cat_cols([_as_bf16(wqkv_s[h, m, words]) for m in range(3)])
      return _dot(_cat_cols(lhs[k0:k1]), w)

    def project(h):
      if h == 0:
        part_s[...] = project_part(h, 0, kt // 2)
        r = part_s[...] + project_part(h, kt // 2, kt)
      else:
        r = project_part(h, 0, kt)
      for m in range(3):
        for i in range(ride // 8):
          work[ring(h, m, put[i], 8)] = r[
              n_mem + 8 * i:n_mem + 8 * i + 8, _block(m)]
      qkv[h] = [r[0:n_mem, _block(m)] for m in range(3)]

    def fetch(h, m):
      return jnp.concatenate([qkv[h][m], work[ring(h, m, get, seg)]], axis=0)

    def stack(t, m):
      rows = [fetch(h, m) for h in teams[t]]
      pad = jnp.zeros((_LANES - len(rows) * n_rows, _LANES), _F32)
      return jnp.concatenate(rows + [pad], axis=0)

    queries, keys_t, values, tails = {}, {}, {}, {}

    def fetch_keys(t):
      queries[t] = [fetch(h, 0) for h in teams[t]]
      if _T32:
        keys_t[t] = stack(t, 1).T.astype(_BF16)
      else:
        keys_t[t] = stack(t, 1).astype(_BF16).T

    def fetch_values(t):
      values[t] = stack(t, 2).astype(_BF16)

    def softmax(t, sc):
      sc = jnp.where(visible, sc * scale, hidden)
      n = len(teams[t])
      top = [jnp.max(jnp.where(window[c], sc, -jnp.inf), axis=-1, keepdims=True)
             for c in range(n)]
      p = jnp.exp(sc - by_window(top))
      probs[t] = (p, [
          jnp.sum(jnp.where(window[c], p, 0.0), axis=-1, keepdims=True)
          for c in range(n)])

    def emit(t, outs):
      for h, o, denom in zip(teams[t], outs, probs[t][1]):
        inv = pltpu.reciprocal(denom, approx=True)
        o_s[:, _block(h)] = o * (inv * (2.0 - denom * inv))

    def diagonal(tile):
      words = pltpu.bitcast(tile, _U32)
      keep = functools.reduce(
          jnp.logical_or, [word_rows(c) & window[c] for c in range(team)])
      return _as_bf16(jnp.where(keep, words, np.uint32(0)))

    def shared(t):
      return (1 <= t < len(teams)
              and len(teams[t]) == len(teams[t - 1]) == team and t != _UNSHARE)

    def score_tails(t):
      if shared(t):
        tails[t] = _dot(by_window(queries[t]), diagonal(keys_t[t]))

    pending = {}

    def value_tails(t):
      if shared(t):
        rest = _dot(probs[t - 1][0], diagonal(values[t - 1]))
        emit(t - 1, [jnp.where(window[c], rest, pending[t][c])
                     for c in range(team)])

    def attend(t):
      if shared(t):
        p = probs[t - 1][0]
        kw = pltpu.bitcast(keys_t[t], _U32)
        vw = pltpu.bitcast(values[t - 1], _U32)
        both = []
        for c in range(team):
          tile = jnp.where(word_rows(c) == window[c], np.uint32(0),
                           jnp.where(word_rows(c), vw, kw))
          both.append(
              _dot(jnp.where(window[c], p, queries[t][c]), _as_bf16(tile)))
        softmax(t, by_window(both) + tails[t])
        pending[t] = both
        if not _SPLIT:
          value_tails(t)
        return
      if t < len(teams):
        softmax(t, by_window([_dot(q, keys_t[t]) for q in queries[t]]))
      if t >= 1:
        p = probs[t - 1][0]
        emit(t - 1, [_dot(jnp.where(window[c], p, 0.0), values[t - 1])
                     for c in range(len(teams[t - 1]))])

    acc, done = None, 0

    def out_project(n):
      nonlocal acc, done
      lo, hi = done * _LANES, (done + n) * _LANES
      w = _cat_cols([_as_bf16(wo_s[k, lo // 2:hi // 2]) for k in range(kt)])
      r = _dot(o_s[:, lo:hi], w)
      acc = r if acc is None else acc + r
      done += n

    last = {tm[-1]: t for t, tm in enumerate(teams)}
    last[heads - 1 + team] = len(teams)
    for h in range(heads + team + _LAG_ATTEND):
      if h < heads:
        project(h)
      if h in last and last[h] < len(teams):
        fetch_keys(last[h])
      if h - _LAG_FETCH_V in last and last[h - _LAG_FETCH_V] < len(teams):
        fetch_values(last[h - _LAG_FETCH_V])
      if h >= heads:
        out_project(_OUT_HEADS)
      if h - _LAG_TAILS in last:
        score_tails(last[h - _LAG_TAILS])
      if h - _LAG_ATTEND in last:
        attend(last[h - _LAG_ATTEND])
      if _SPLIT and h - _LAG_ATTEND - 1 in last:
        value_tails(last[h - _LAG_ATTEND - 1])
    assert len(fillers) <= _OUT_EXTRA
    for n in range(_OUT_EXTRA):
      out_project(_OUT_HEADS)
      if n < len(fillers):
        fillers[n]()
    out_project(heads - done)

    g = work[area("gate", s * seg, seg)]
    rows = pl.ds(pl.multiple_of(s * seg, seg), seg)
    for k in range(kt):
      mix = area("mix", k * seq + s * seg, seg)
      mixed = g * acc[n_mem:, _block(k)] + work[mix]
      work[mix] = mixed
      out_s[rows, _block(k)] = mixed.astype(_BF16)
    return [acc[0:n_mem, _block(k)] for k in range(kt)]

  def steps(i, carry):
    pl.when(i < ffn_iters)(lambda: _wait(ffn_copies(i)))

    @pl.when(i == ffn_iters)
    def _():
      add_ffn()
      out_copy(0, ffn_iters * _UNROLL).start()

    groups = ffn_groups(i)
    per_step = len(groups) // _UNROLL
    mem = [mem_s[:, _block(k)] for k in range(kt)]
    for u in range(_UNROLL):
      mem = step(i * _UNROLL + u, mem, groups[u * per_step:(u + 1) * per_step])
    mem_s[...] = _cat_cols(mem)
    pl.when(i + 2 < ffn_iters)(lambda: _start(ffn_copies(i + 2)))
    pl.when(i >= ffn_iters)(lambda: out_copy(i * _UNROLL, _UNROLL).start())
    return carry

  mem_s[...] = mem0_s[...].astype(_F32)
  _wait([wo_copy(n) for n in range(kt)])
  lax.fori_loop(0, n_seg // _UNROLL, steps, 0)
  pltpu.make_async_copy(out_s, out_hbm, sem_out).wait()


@functools.partial(jax.jit, static_argnames=("A_seg_len",))
def pallas_gated_mix__memory_aug_recurrent_mem_tr__moe_arch_mod__prompt_kernel(
    A_x: jax.Array,
    A_mem0: jax.Array,
    A_Wq: jax.Array,
    A_Wk: jax.Array,
    A_Wv: jax.Array,
    A_Wo: jax.Array,
    A_seg_len: int,
    B_x: jax.Array,
    B_w_r: jax.Array,
    B_w_gate: jax.Array,
    B_w_up: jax.Array,
    B_w_down: jax.Array,
    gate_w: jax.Array,
):
  del B_x
  batch, seq, dm = A_x.shape
  _, heads, dh = A_Wq.shape
  n_mem = A_mem0.shape[1]
  seg = int(A_seg_len)
  assert (batch, seq, dm, heads, dh) == (1, 2048, 1024, 32, _LANES)
  assert (n_mem, seg, B_w_down.shape[0]) == (8, 32, 3584)
  kt = dm // _LANES
  ring_rows = seq // 4 + seg
  width = _FFN_BLOCKS * _LANES

  hbm = pl.BlockSpec(memory_space=pl.ANY)
  out = pl.pallas_call(
      functools.partial(_kernel, heads=heads, seg=seg, ring_rows=ring_rows),
      out_shape=jax.ShapeDtypeStruct((seq, dm), A_x.dtype),
      in_specs=[hbm] * 11,
      out_specs=hbm,
      scratch_shapes=[
          pltpu.VMEM((seq, dm), _BF16),
          pltpu.VMEM((heads, 3, dm // 2, _LANES), _U32),
          pltpu.VMEM((kt, heads * dh // 2, _LANES), _U32),
          pltpu.VMEM((2, dm, width), _BF16),
          pltpu.VMEM((2, dm, width), _BF16),
          pltpu.VMEM((2, width, dm), _BF16),
          pltpu.VMEM((seq, dm), _BF16),
          pltpu.VMEM(
              (_work_layout(seq, kt, heads, ring_rows)["end"], _LANES), _F32),
          pltpu.VMEM((n_mem + seg, heads * dh), _F32),
          pltpu.VMEM((n_mem, dm), _F32),
          pltpu.VMEM((seg, 3 * _LANES), _F32),
          pltpu.VMEM((_FFN_BLOCKS, 2, 2, _TOP_C, _LANES), _F32),
          pltpu.VMEM((_TOP_C, dm), _F32),
          pltpu.VMEM((n_mem, dm), _BF16),
          pltpu.VMEM((kt, _LANES), _BF16),
          pltpu.VMEM((kt, _LANES), _BF16),
          pltpu.SMEM((_TOP_C,), jnp.int32),
          pltpu.SemaphoreType.DMA((8,)),
          pltpu.SemaphoreType.DMA((6,)),
          pltpu.SemaphoreType.DMA((4,)),
          pltpu.SemaphoreType.DMA,
      ],
      compiler_params=pltpu.CompilerParams(
          vmem_limit_bytes=100 * 2**20,
          disable_bounds_checks=True,
          disable_semaphore_checks=True,
      ),
      name="gated_rmt_mod",
  )(
      A_x.reshape(seq, dm),
      A_mem0.reshape(n_mem, dm),
      A_Wq.reshape(dm // 2, 2, heads, dh),
      A_Wk.reshape(dm // 2, 2, heads, dh),
      A_Wv.reshape(dm // 2, 2, heads, dh),
      A_Wo.reshape(heads * dh, dm),
      B_w_r.reshape(kt, _LANES),
      B_w_gate,
      B_w_up,
      B_w_down,
      gate_w.reshape(kt, _LANES),
  )
  return out.reshape(batch, seq, dm)
```

```python
import functools

import jax
import jax.experimental.pallas as pl
import jax.experimental.pallas.tpu as pltpu
import jax.numpy as jnp
import numpy as np
from jax import lax

_BF16 = jnp.bfloat16
_F32 = jnp.float32
_U32 = jnp.uint32
_LANES = 128
_TOP_C = 8

_UNROLL = 4
_FFN_BLOCKS = 2
_CHUNK = 128
_LAG_ATTEND = 4
_LAG_FETCH_V = 5
_OUT_HEADS = 2
_OUT_EXTRA = 4


def _as_bf16(words):
  return pltpu.bitcast(words, _BF16)


def _cat_cols(parts):
  return parts[0] if len(parts) == 1 else jnp.concatenate(parts, axis=1)


def _block(n):
  return slice(n * _LANES, (n + 1) * _LANES)


def _dot(a, b):
  return jnp.dot(a, b, preferred_element_type=_F32)


def _reduce_all(op, a):
  return op(op(a, axis=1, keepdims=True), axis=0, keepdims=True)


def _start(copies):
  for copy in copies:
    copy.start()


def _wait(copies):
  for copy in copies:
    copy.wait()


def _work_layout(seq, kt, heads, ring_rows):
  sizes = (
      ("ring", 3 * heads * ring_rows),
      ("mix", kt * seq),
      ("gate", seq),
      ("score", seq // _LANES),
      ("taken", seq // _LANES),
      ("r_sel", _TOP_C),
      ("x_sel", kt * _TOP_C),
      ("end", 0),
  )
  starts = np.cumsum([0] + [n for _, n in sizes])
  return {name: int(start) for (name, _), start in zip(sizes, starts)}


def _kernel(
    x_hbm, mem0_hbm, wq_hbm, wk_hbm, wv_hbm, wo_hbm, wr_hbm, wg_hbm, wu_hbm,
    wd_hbm, gw_hbm,
    out_hbm,
    x_s, wqkv_s, wo_s, wg_s, wu_s, wd_s, out_s, work, o_s, mem_s, part_s, pre_s,
    y_s, mem0_s, wr_s, gw_s, idx_s, sem_x, sem_w, sem_misc, sem_out,
    *, heads, seg, ring_rows,
):
  seq, dm = x_hbm.shape
  n_mem = mem0_hbm.shape[0]
  kt = dm // _LANES
  n_seg = seq // seg
  n_rows = n_mem + seg
  ride = seg - n_mem
  ahead = seq - n_seg * ride
  x_rows = ahead // 2
  ffn_iters = wd_hbm.shape[0] // (_FFN_BLOCKS * _LANES)
  sub = lax.broadcasted_iota(jnp.int32, (8, _LANES), 0)
  lane = lax.broadcasted_iota(jnp.int32, (8, _LANES), 1)

  layout = _work_layout(seq, kt, heads, ring_rows)

  def area(name, row, n):
    start = layout[name] + row
    if n % 8 == 0 and not isinstance(start, int):
      start = pl.multiple_of(start, 8)
    return pl.ds(start, n)

  def ring(h, m, row, n):
    return area("ring", (3 * h + m) * ring_rows + row, n)

  def x_copies(j):
    n = x_rows // 2
    parts = [pl.ds(pl.multiple_of(j * x_rows + i * n, n), n) for i in range(2)]
    return [pltpu.make_async_copy(x_hbm.at[rows], x_s.at[rows], sem_x.at[j])
            for rows in parts]

  def w_copies(j, m, sem):
    words = (wq_hbm, wk_hbm, wv_hbm)[m].bitcast(_U32)
    return [pltpu.make_async_copy(
        words.at[:, p, j], wqkv_s.at[2 * j + p, m], sem_w.at[sem])
            for p in range(2)]

  def pair_copies(j):
    sem = j % 6 if isinstance(j, int) else lax.rem(j, 6)
    return [copy for m in range(3) for copy in w_copies(j, m, sem)]

  def wo_copy(n):
    cols = pl.ds(pl.multiple_of(n * _LANES, _LANES), _LANES)
    return pltpu.make_async_copy(
        wo_hbm.at[:, cols], wo_s.at[n].bitcast(_BF16), sem_misc.at[0])

  def ffn_copies(i):
    width = _FFN_BLOCKS * _LANES
    f = pl.ds(pl.multiple_of(i * width, width), width)
    sem = sem_misc.at[2 + (i & 1)]
    return [pltpu.make_async_copy(wg_hbm.at[:, f], wg_s.at[i & 1], sem),
            pltpu.make_async_copy(wu_hbm.at[:, f], wu_s.at[i & 1], sem),
            pltpu.make_async_copy(wd_hbm.at[f], wd_s.at[i & 1], sem)]

  small_copies = [
      pltpu.make_async_copy(src, dst, sem_misc.at[1])
      for src, dst in ((mem0_hbm, mem0_s), (wr_hbm, wr_s), (gw_hbm, gw_s))]

  def out_copy(first, n):
    rows = pl.ds(pl.multiple_of(first * seg, seg), n * seg)
    return pltpu.make_async_copy(out_s.at[rows], out_hbm.at[rows], sem_out)

  first_w = [w_copies(0, m, sem) for m, sem in enumerate((0, 4, 5))]
  _start(x_copies(0) + first_w[0] + x_copies(1) + first_w[1])

  def gate_and_score(t0, score):
    gw = gw_s[...].astype(_F32)
    wr = wr_s[...].astype(_F32)
    rows = pl.ds(pl.multiple_of(t0, 16), 16)
    xs = [x_s[rows, _block(k)].astype(_F32) for k in range(kt)]
    logit = functools.reduce(jnp.add, [xs[k] * gw[k:k + 1] for k in range(kt)])
    r = functools.reduce(jnp.add, [xs[k] * wr[k:k + 1] for k in range(kt)])
    g = jax.nn.sigmoid(jnp.sum(logit, axis=-1, keepdims=True))
    r = jnp.sum(r, axis=-1, keepdims=True)
    work[area("gate", t0, 16)] = jnp.broadcast_to(g, (16, _LANES))
    for k in range(kt):
      work[area("mix", k * seq + t0, 16)] = (1.0 - g) * xs[k]
    for u in range(2):
      for n in range(len(score)):
        here = (n * _LANES + lane) * 8 == t0 + 8 * u
        score[n] = jnp.where(here, r[8 * u:8 * u + 8], score[n])

  def route_next(c):
    n = seq // _LANES
    score = work[area("score", 0, n)].astype(_BF16).astype(_F32)
    row = lax.broadcasted_iota(jnp.int32, score.shape, 0)
    col = lax.broadcasted_iota(jnp.int32, score.shape, 1)
    tok = ((row >> 3) * (8 * _LANES) + col * 8 + (row & 7)).astype(_F32)
    taken = work[area("taken", 0, n)]
    free = taken == 0.0
    cand = jnp.where(free & (score == score), score, -jnp.inf)
    best = _reduce_all(jnp.max, cand)
    pick = _reduce_all(
        jnp.min, jnp.where(free & (cand == best), tok, float(seq)))
    chosen = tok == pick
    work[area("taken", 0, n)] = jnp.where(
        chosen, jnp.where(c >= 0, 1.0, 0.0), taken)
    r_c = _reduce_all(jnp.sum, jnp.where(chosen, score, 0.0))
    r_sel = area("r_sel", 0, _TOP_C)
    work[r_sel] = jnp.where(sub == c, r_c, work[r_sel])
    t = jnp.clip(pick.astype(jnp.int32)[0, 0], 0, seq - 1)
    idx_s[jnp.maximum(c, 0)] = t
    rows = pl.ds(pl.multiple_of(jnp.where(c >= 0, (t >> 4) * 16, 0), 16), 16)
    row16 = lax.broadcasted_iota(jnp.int32, (16, _LANES), 0)
    for k in range(kt):
      blk = x_s[rows, _block(k)].astype(_F32)
      xt = jnp.sum(jnp.where(row16 == (t & 15), blk, 0.0), axis=0,
                   keepdims=True)
      x_sel = area("x_sel", k * _TOP_C, _TOP_C)
      work[x_sel] = jnp.where(sub == c, xt, work[x_sel])

  chunks = ahead // _CHUNK
  slots = 6 * chunks

  def untangle(j, m):
    even = wqkv_s[2 * j, m]
    odd = wqkv_s[2 * j + 1, m]
    wqkv_s[2 * j, m] = (even & np.uint32(0xFFFF)) | (odd << 16)
    wqkv_s[2 * j + 1, m] = (even >> 16) | (odd & np.uint32(0xFFFF0000))

  def project_chunk(h, m, c, side_work=None):
    xa = x_s[c * _CHUNK:(c + 1) * _CHUNK]
    w = _as_bf16(wqkv_s[h, m])
    if side_work is not None:
      side_work()
    work[ring(h, m, c * _CHUNK, _CHUNK)] = _dot(xa, w)

  def project_pair(j, side_work):
    untangle(j, 0)
    for m in range(3):
      for p in range(2):
        for c in range(chunks):
          def between(m=m, p=p, c=c):
            if p == 1 and m < 2 and c == 0:
              untangle(j, m + 1)
            side_work((2 * m + p) * chunks + c)

          project_chunk(2 * j + p, m, c, between)

  def first_pairs():
    _wait(x_copies(0) + first_w[0])
    _start(small_copies + first_w[2])
    untangle(0, 0)
    for c in range(chunks):
      if c * _CHUNK == x_rows:
        _wait(x_copies(1))
        _start(pair_copies(1))
      for p in range(2):
        project_chunk(p, 0, c)
    for m in (1, 2):
      _wait(first_w[m])
      _start(pair_copies(2) if m == 1 else pair_copies(3) + x_copies(2))
      untangle(0, m)
      for p in range(2):
        for c in range(chunks):
          project_chunk(p, m, c)
    _wait(small_copies + pair_copies(1))

    def side_work(slot):
      if slot == slots - 1:
        _start(pair_copies(4) + pair_copies(5) + x_copies(3) + x_copies(4)
               + x_copies(5))

    project_pair(1, side_work)

  rounds = heads // 4 - 1
  scoring = rounds - _TOP_C // 2
  pieces = -(-seq // (16 * scoring))
  gate_slots = 2 * slots - 10

  def other_pairs(i, carry):
    _wait(pair_copies(2 * i + 2) + pair_copies(2 * i + 3))
    for n in range(3):
      j = 3 * i + n
      pl.when((j >= 2) & (j < seq // x_rows))(lambda j=j: _wait(x_copies(j)))
    first = jnp.minimum(i * pieces * 16, seq - pieces * 16)
    pages = [area("score", 8 * n, 8) for n in range(seq // (8 * _LANES))]
    score = [work[page] for page in pages]

    def side_work(slot):
      for n in range(pieces):
        if n * gate_slots // pieces == slot:
          gate_and_score(first + 16 * n, score)
      if slot == gate_slots:
        for page, value in zip(pages, score):
          work[page] = value
      for v in range(2):
        if slot == gate_slots + 4 * (v + 1):
          route_next(2 * (i - scoring) + v)
      if slot == 2 * slots - 1:
        pl.when(i + 2 < rounds)(lambda: _start(
            pair_copies(2 * i + 6) + pair_copies(2 * i + 7)))
        pl.when(i == 0)(lambda: _start(x_copies(6) + x_copies(7)))
        pl.when((i >= 1) & (i <= kt // 2))(
            lambda: _start([wo_copy(2 * i - 2), wo_copy(2 * i - 1)]))
        pl.when(i + 2 == rounds)(lambda: _start(ffn_copies(0) + ffn_copies(1)))

    for u in range(2):
      project_pair(2 * i + 2 + u, lambda slot, u=u: side_work(u * slots + slot))
    return carry

  n_small = layout["end"] - layout["score"]
  work[area("score", 0, n_small)] = jnp.zeros((n_small, _LANES), _F32)
  y_s[...] = jnp.zeros(y_s.shape, _F32)
  first_pairs()
  lax.fori_loop(0, rounds, other_pairs, 0)

  def ffn_groups(i):
    x_sel = [work[area("x_sel", k * _TOP_C, _TOP_C)] for k in range(kt)]
    act = {}

    def widen(b, which, part):
      ks = slice(part * kt // 2, (part + 1) * kt // 2)
      w = (wg_s, wu_s)[which][
          i & 1, ks.start * _LANES:ks.stop * _LANES, _block(b)]
      pre_s[b, which, part] = _dot(_cat_cols(x_sel[ks]), w)

    def narrow(b, part):
      if part == 0:
        gate, up = (pre_s[b, n, 0] + pre_s[b, n, 1] for n in range(2))
        act[b] = gate * jax.nn.sigmoid(gate) * up
      cols = slice(part * dm // 2, (part + 1) * dm // 2)
      y_s[:, cols] += _dot(act[b], wd_s[i & 1, _block(b), cols])

    return (
        [functools.partial(widen, b, which, part) for b in range(_FFN_BLOCKS)
         for which in range(2) for part in range(2)]
        + [functools.partial(narrow, b, part) for b in range(_FFN_BLOCKS)
           for part in range(2)])

  def add_ffn():
    keep = jnp.zeros((8, _LANES), _F32)
    for c in range(_TOP_C):
      keep = jnp.where(sub == c, 1.0 - work[area("gate", idx_s[c], 1)], keep)
    keep = keep * jax.nn.sigmoid(work[area("r_sel", 0, _TOP_C)])
    y = [y_s[:, _block(k)] * keep for k in range(kt)]
    for c in range(_TOP_C):
      t0 = pl.multiple_of((idx_s[c] >> 3) * 8, 8)
      hit = sub == (idx_s[c] & 7)
      old = [work[area("mix", k * seq + t0, 8)] for k in range(kt)]
      for k in range(kt):
        new = jnp.where(hit, old[k] + y[k][c:c + 1], old[k])
        work[area("mix", k * seq + t0, 8)] = new
        out_s[pl.ds(t0, 8), _block(k)] = new.astype(_BF16)

  scale = float(_LANES) ** -0.5

  team = _LANES // n_rows
  qi = lax.broadcasted_iota(jnp.int32, (n_rows, _LANES), 0)
  col = lax.broadcasted_iota(jnp.int32, (1, _LANES), 1)
  window = [(col >= c * n_rows) & (col < (c + 1) * n_rows) for c in range(team)]
  ki = col - sum(jnp.where(window[c], c * n_rows, 0) for c in range(team))
  visible = ((qi < n_mem) | (qi >= ki)) & (col < team * n_rows)
  hidden = jnp.where(col < team * n_rows, -1e9, -jnp.inf).astype(_F32)
  teams = ([tuple(range(heads % team))] if heads % team else []) + [
      tuple(range(h, h + team)) for h in range(heads % team, heads, team)]

  def by_window(parts):
    out = parts[-1]
    for c in range(len(parts) - 1):
      out = jnp.where(window[c], parts[c], out)
    return out

  def stack_rows(rows):
    pad = _LANES - sum(r.shape[0] for r in rows)
    return jnp.concatenate(rows + [jnp.zeros((pad, _LANES), _F32)], axis=0)

  def diagonal(tile):
    return stack_rows(
        [jnp.where(window[c], tile[c * n_rows:(c + 1) * n_rows], 0.0)
         for c in range(team)]).astype(_BF16)

  def off_diagonal(keys_t, values, c):
    lo, hi = c * n_rows, (c + 1) * n_rows
    rows = [jnp.where(window[c], keys_t[:lo], 0.0)] if lo else []
    rows += [jnp.where(window[c], 0.0, values[lo:hi]),
             jnp.where(window[c], keys_t[hi:], 0.0)]
    return jnp.concatenate(rows, axis=0).astype(_BF16)

  def step(s, mem, fillers):
    tokens = pl.ds(pl.multiple_of(ahead + s * ride, 8), ride)
    lhs = [
        jnp.concatenate([mem[k], x_s[tokens, _block(k)].astype(_F32)], axis=0
                        ).astype(_BF16) for k in range(kt)]
    put = [lax.rem(ahead + s * ride + 8 * i, ring_rows)
           for i in range(ride // 8)]
    get = lax.rem(s * seg, ring_rows)
    qkv, probs = {}, {}

    def project_part(h, k0, k1):
      words = slice(k0 * _LANES // 2, k1 * _LANES // 2)
      w = _cat_cols([_as_bf16(wqkv_s[h, m, words]) for m in range(3)])
      return _dot(_cat_cols(lhs[k0:k1]), w)

    def project(h):
      if h == 0:
        part_s[...] = project_part(h, 0, kt // 2)
        r = part_s[...] + project_part(h, kt // 2, kt)
      else:
        r = project_part(h, 0, kt)
      for m in range(3):
        for i in range(ride // 8):
          work[ring(h, m, put[i], 8)] = r[
              n_mem + 8 * i:n_mem + 8 * i + 8, _block(m)]
      qkv[h] = [r[0:n_mem, _block(m)] for m in range(3)]

    def fetch(h, m):
      return jnp.concatenate([qkv[h][m], work[ring(h, m, get, seg)]], axis=0)

    queries, keys_t, values = {}, {}, {}

    def softmax(t, sc):
      sc = jnp.where(visible, sc * scale, hidden)
      members = window[:len(teams[t])]
      top = [jnp.max(jnp.where(w, sc, -jnp.inf), axis=-1, keepdims=True)
             for w in members]
      p = jnp.exp(sc - by_window(top))
      probs[t] = (p, [jnp.sum(jnp.where(w, p, 0.0), axis=-1, keepdims=True)
                      for w in members])

    def emit(t, outs):
      for h, o, denom in zip(teams[t], outs, probs[t][1]):
        inv = pltpu.reciprocal(denom, approx=True)
        o_s[:, _block(h)] = o * (inv * (2.0 - denom * inv))

    def attend(t):
      if 1 <= t < len(teams) and len(teams[t - 1]) == team:
        p = probs[t - 1][0]
        inside = _dot(by_window(queries[t]), diagonal(keys_t[t]))
        both = [_dot(jnp.where(window[c], p, queries[t][c]),
                     off_diagonal(keys_t[t], values[t - 1], c))
                for c in range(team)]
        softmax(t, by_window(both) + inside)
        inside = _dot(p, diagonal(values[t - 1]))
        emit(t - 1,
             [jnp.where(window[c], inside, both[c]) for c in range(team)])
        return
      if t < len(teams):
        k = keys_t[t].astype(_BF16)
        softmax(t, by_window([_dot(q, k) for q in queries[t]]))
      if t >= 1:
        v = values[t - 1].astype(_BF16)
        emit(t - 1, [_dot(jnp.where(w, probs[t - 1][0], 0.0), v)
                     for w in window[:len(teams[t - 1])]])

    acc, done = None, 0

    def out_project(n):
      nonlocal acc, done
      lo, hi = done * _LANES, (done + n) * _LANES
      w = _cat_cols([_as_bf16(wo_s[k, lo // 2:hi // 2]) for k in range(kt)])
      r = _dot(o_s[:, lo:hi], w)
      acc = r if acc is None else acc + r
      done += n

    ends = {members[-1]: t for t, members in enumerate(teams)}
    for h in range(heads + team + _LAG_ATTEND):
      if h < heads:
        project(h)
      if h in ends:
        t = ends[h]
        queries[t] = [fetch(n, 0) for n in teams[t]]
        keys_t[t] = stack_rows([fetch(n, 1) for n in teams[t]]).T
      if h - _LAG_FETCH_V in ends:
        t = ends[h - _LAG_FETCH_V]
        values[t] = stack_rows([fetch(n, 2) for n in teams[t]])
      if h >= heads:
        out_project(_OUT_HEADS)
      if h - _LAG_ATTEND in ends:
        attend(ends[h - _LAG_ATTEND])
    attend(len(teams))
    assert len(fillers) <= _OUT_EXTRA
    for n in range(_OUT_EXTRA):
      out_project(_OUT_HEADS)
      if n < len(fillers):
        fillers[n]()
    out_project(heads - done)

    g = work[area("gate", s * seg, seg)]
    rows = pl.ds(pl.multiple_of(s * seg, seg), seg)
    for k in range(kt):
      mix = area("mix", k * seq + s * seg, seg)
      mixed = g * acc[n_mem:, _block(k)] + work[mix]
      work[mix] = mixed
      out_s[rows, _block(k)] = mixed.astype(_BF16)
    return [acc[0:n_mem, _block(k)] for k in range(kt)]

  def steps(i, carry):
    pl.when(i < ffn_iters)(lambda: _wait(ffn_copies(i)))

    @pl.when(i == ffn_iters)
    def _():
      add_ffn()
      out_copy(0, ffn_iters * _UNROLL).start()

    groups = ffn_groups(i)
    per_step = len(groups) // _UNROLL
    mem = [mem_s[:, _block(k)] for k in range(kt)]
    for u in range(_UNROLL):
      mem = step(i * _UNROLL + u, mem, groups[u * per_step:(u + 1) * per_step])
    mem_s[...] = _cat_cols(mem)
    pl.when(i + 2 < ffn_iters)(lambda: _start(ffn_copies(i + 2)))
    pl.when(i >= ffn_iters)(lambda: out_copy(i * _UNROLL, _UNROLL).start())
    return carry

  mem_s[...] = mem0_s[...].astype(_F32)
  _wait([wo_copy(n) for n in range(kt)])
  lax.fori_loop(0, n_seg // _UNROLL, steps, 0)
  pltpu.make_async_copy(out_s, out_hbm, sem_out).wait()


@functools.partial(jax.jit, static_argnames=("A_seg_len",))
def pallas_gated_mix__memory_aug_recurrent_mem_tr__moe_arch_mod__prompt_kernel(
    A_x: jax.Array,
    A_mem0: jax.Array,
    A_Wq: jax.Array,
    A_Wk: jax.Array,
    A_Wv: jax.Array,
    A_Wo: jax.Array,
    A_seg_len: int,
    B_x: jax.Array,
    B_w_r: jax.Array,
    B_w_gate: jax.Array,
    B_w_up: jax.Array,
    B_w_down: jax.Array,
    gate_w: jax.Array,
):
  del B_x
  batch, seq, dm = A_x.shape
  _, heads, dh = A_Wq.shape
  n_mem = A_mem0.shape[1]
  seg = int(A_seg_len)
  assert (batch, seq, dm, heads, dh) == (1, 2048, 1024, 32, _LANES)
  assert (n_mem, seg, B_w_down.shape[0]) == (8, 32, 3584)
  kt = dm // _LANES
  ring_rows = seq // 4 + seg
  width = _FFN_BLOCKS * _LANES

  hbm = pl.BlockSpec(memory_space=pl.ANY)
  out = pl.pallas_call(
      functools.partial(_kernel, heads=heads, seg=seg, ring_rows=ring_rows),
      out_shape=jax.ShapeDtypeStruct((seq, dm), A_x.dtype),
      in_specs=[hbm] * 11,
      out_specs=hbm,
      scratch_shapes=[
          pltpu.VMEM((seq, dm), _BF16),
          pltpu.VMEM((heads, 3, dm // 2, _LANES), _U32),
          pltpu.VMEM((kt, heads * dh // 2, _LANES), _U32),
          pltpu.VMEM((2, dm, width), _BF16),
          pltpu.VMEM((2, dm, width), _BF16),
          pltpu.VMEM((2, width, dm), _BF16),
          pltpu.VMEM((seq, dm), _BF16),
          pltpu.VMEM(
              (_work_layout(seq, kt, heads, ring_rows)["end"], _LANES), _F32),
          pltpu.VMEM((n_mem + seg, heads * dh), _F32),
          pltpu.VMEM((n_mem, dm), _F32),
          pltpu.VMEM((seg, 3 * _LANES), _F32),
          pltpu.VMEM((_FFN_BLOCKS, 2, 2, _TOP_C, _LANES), _F32),
          pltpu.VMEM((_TOP_C, dm), _F32),
          pltpu.VMEM((n_mem, dm), _BF16),
          pltpu.VMEM((kt, _LANES), _BF16),
          pltpu.VMEM((kt, _LANES), _BF16),
          pltpu.SMEM((_TOP_C,), jnp.int32),
          pltpu.SemaphoreType.DMA((8,)),
          pltpu.SemaphoreType.DMA((6,)),
          pltpu.SemaphoreType.DMA((4,)),
          pltpu.SemaphoreType.DMA,
      ],
      compiler_params=pltpu.CompilerParams(
          vmem_limit_bytes=100 * 2**20,
          disable_bounds_checks=True,
          disable_semaphore_checks=True,
      ),
      name="gated_rmt_mod",
  )(
      A_x.reshape(seq, dm),
      A_mem0.reshape(n_mem, dm),
      A_Wq.reshape(dm // 2, 2, heads, dh),
      A_Wk.reshape(dm // 2, 2, heads, dh),
      A_Wv.reshape(dm // 2, 2, heads, dh),
      A_Wo.reshape(heads * dh, dm),
      B_w_r.reshape(kt, _LANES),
      B_w_gate,
      B_w_up,
      B_w_down,
      gate_w.reshape(kt, _LANES),
  )
  return out.reshape(batch, seq, dm)
```

```python
import functools

import jax
import jax.experimental.pallas as pl
import jax.experimental.pallas.tpu as pltpu
import jax.numpy as jnp
import numpy as np
from jax import lax

_BF16 = jnp.bfloat16
_F32 = jnp.float32
_U32 = jnp.uint32
_LANES = 128
_TOP_C = 8

_UNROLL = 4
_FFN_BLOCKS = 2
_CHUNK = 128
_LAG_ATTEND = 4
_LAG_FETCH_Q = 2
_LAG_FETCH_V = 5
_OUT_HEADS = 2
_OUT_EXTRA = 5


def _as_bf16(words):
  return pltpu.bitcast(words, _BF16)


def _cat_cols(parts):
  return parts[0] if len(parts) == 1 else jnp.concatenate(parts, axis=1)


def _block(n):
  return slice(n * _LANES, (n + 1) * _LANES)


def _dot(a, b):
  return jnp.dot(a, b, preferred_element_type=_F32)


def _reduce_all(op, a):
  return op(op(a, axis=1, keepdims=True), axis=0, keepdims=True)


def _start(copies):
  for copy in copies:
    copy.start()


def _wait(copies):
  for copy in copies:
    copy.wait()


def _work_layout(seq, kt, heads, ring_rows):
  sizes = (
      ("ring", 3 * heads * ring_rows),
      ("mix", kt * seq),
      ("gate", seq),
      ("score", seq // _LANES),
      ("taken", seq // _LANES),
      ("r_sel", _TOP_C),
      ("x_sel", kt * _TOP_C),
      ("end", 0),
  )
  starts = np.cumsum([0] + [n for _, n in sizes])
  return {name: int(start) for (name, _), start in zip(sizes, starts)}


def _kernel(
    x_hbm, mem0_hbm, wq_hbm, wk_hbm, wv_hbm, wo_hbm, wr_hbm, wg_hbm, wu_hbm,
    wd_hbm, gw_hbm,
    out_hbm,
    x_s, wqkv_s, wo_s, wg_s, wu_s, wd_s, out_s, work, o_s, mem_s, part_s, pre_s,
    y_s, mem0_s, wr_s, gw_s, idx_s, sem_x, sem_w, sem_misc, sem_out,
    *, heads, seg, ring_rows,
):
  seq, dm = x_hbm.shape
  n_mem = mem0_hbm.shape[0]
  kt = dm // _LANES
  n_seg = seq // seg
  n_rows = n_mem + seg
  ride = seg - n_mem
  ahead = seq - n_seg * ride
  x_rows = ahead // 2
  ffn_iters = wd_hbm.shape[0] // (_FFN_BLOCKS * _LANES)
  sub = lax.broadcasted_iota(jnp.int32, (8, _LANES), 0)
  lane = lax.broadcasted_iota(jnp.int32, (8, _LANES), 1)

  layout = _work_layout(seq, kt, heads, ring_rows)

  def area(name, row, n):
    start = layout[name] + row
    if n % 8 == 0 and not isinstance(start, int):
      start = pl.multiple_of(start, 8)
    return pl.ds(start, n)

  def ring(h, m, row, n):
    return area("ring", (3 * h + m) * ring_rows + row, n)

  def x_copies(j):
    n = x_rows // 2
    parts = [pl.ds(pl.multiple_of(j * x_rows + i * n, n), n) for i in range(2)]
    return [pltpu.make_async_copy(x_hbm.at[rows], x_s.at[rows], sem_x.at[j])
            for rows in parts]

  def w_copies(j, m, sem):
    words = (wq_hbm, wk_hbm, wv_hbm)[m].bitcast(_U32)
    return [pltpu.make_async_copy(
        words.at[:, p, j], wqkv_s.at[2 * j + p, m], sem_w.at[sem])
            for p in range(2)]

  def pair_copies(j):
    sem = j % 6 if isinstance(j, int) else lax.rem(j, 6)
    return [copy for m in range(3) for copy in w_copies(j, m, sem)]

  def wo_copy(n):
    cols = pl.ds(pl.multiple_of(n * _LANES, _LANES), _LANES)
    return pltpu.make_async_copy(
        wo_hbm.at[:, cols], wo_s.at[n].bitcast(_BF16), sem_misc.at[0])

  def ffn_copies(i):
    width = _FFN_BLOCKS * _LANES
    f = pl.ds(pl.multiple_of(i * width, width), width)
    sem = sem_misc.at[2 + (i & 1)]
    return [pltpu.make_async_copy(wg_hbm.at[:, f], wg_s.at[i & 1], sem),
            pltpu.make_async_copy(wu_hbm.at[:, f], wu_s.at[i & 1], sem),
            pltpu.make_async_copy(wd_hbm.at[f], wd_s.at[i & 1], sem)]

  small_copies = [
      pltpu.make_async_copy(src, dst, sem_misc.at[1])
      for src, dst in ((mem0_hbm, mem0_s), (wr_hbm, wr_s), (gw_hbm, gw_s))]

  def out_copy(first, n):
    rows = pl.ds(pl.multiple_of(first * seg, seg), n * seg)
    return pltpu.make_async_copy(out_s.at[rows], out_hbm.at[rows], sem_out)

  first_w = [w_copies(0, m, sem) for m, sem in enumerate((0, 4, 5))]
  _start(x_copies(0) + first_w[0] + x_copies(1) + first_w[1])

  def gate_and_score(t0, score):
    gw = gw_s[...].astype(_F32)
    wr = wr_s[...].astype(_F32)
    rows = pl.ds(pl.multiple_of(t0, 16), 16)
    xs = [x_s[rows, _block(k)].astype(_F32) for k in range(kt)]
    logit = functools.reduce(jnp.add, [xs[k] * gw[k:k + 1] for k in range(kt)])
    r = functools.reduce(jnp.add, [xs[k] * wr[k:k + 1] for k in range(kt)])
    g = jax.nn.sigmoid(jnp.sum(logit, axis=-1, keepdims=True))
    r = jnp.sum(r, axis=-1, keepdims=True)
    work[area("gate", t0, 16)] = jnp.broadcast_to(g, (16, _LANES))
    for k in range(kt):
      work[area("mix", k * seq + t0, 16)] = (1.0 - g) * xs[k]
    for u in range(2):
      for n in range(len(score)):
        here = (n * _LANES + lane) * 8 == t0 + 8 * u
        score[n] = jnp.where(here, r[8 * u:8 * u + 8], score[n])

  def route_next(c):
    n = seq // _LANES
    score = work[area("score", 0, n)].astype(_BF16).astype(_F32)
    row = lax.broadcasted_iota(jnp.int32, score.shape, 0)
    col = lax.broadcasted_iota(jnp.int32, score.shape, 1)
    tok = ((row >> 3) * (8 * _LANES) + col * 8 + (row & 7)).astype(_F32)
    taken = work[area("taken", 0, n)]
    free = taken == 0.0
    cand = jnp.where(free & (score == score), score, -jnp.inf)
    best = _reduce_all(jnp.max, cand)
    pick = _reduce_all(
        jnp.min, jnp.where(free & (cand == best), tok, float(seq)))
    chosen = tok == pick
    work[area("taken", 0, n)] = jnp.where(
        chosen, jnp.where(c >= 0, 1.0, 0.0), taken)
    r_c = _reduce_all(jnp.sum, jnp.where(chosen, score, 0.0))
    r_sel = area("r_sel", 0, _TOP_C)
    work[r_sel] = jnp.where(sub == c, r_c, work[r_sel])
    t = jnp.clip(pick.astype(jnp.int32)[0, 0], 0, seq - 1)
    idx_s[jnp.maximum(c, 0)] = t
    rows = pl.ds(pl.multiple_of(jnp.where(c >= 0, (t >> 4) * 16, 0), 16), 16)
    row16 = lax.broadcasted_iota(jnp.int32, (16, _LANES), 0)
    for k in range(kt):
      blk = x_s[rows, _block(k)].astype(_F32)
      xt = jnp.sum(jnp.where(row16 == (t & 15), blk, 0.0), axis=0,
                   keepdims=True)
      x_sel = area("x_sel", k * _TOP_C, _TOP_C)
      work[x_sel] = jnp.where(sub == c, xt, work[x_sel])

  chunks = ahead // _CHUNK
  slots = 6 * chunks

  def untangle(j, m):
    even = wqkv_s[2 * j, m]
    odd = wqkv_s[2 * j + 1, m]
    wqkv_s[2 * j, m] = (even & np.uint32(0xFFFF)) | (odd << 16)
    wqkv_s[2 * j + 1, m] = (even >> 16) | (odd & np.uint32(0xFFFF0000))

  def project_chunk(h, m, c, side_work=None):
    xa = x_s[c * _CHUNK:(c + 1) * _CHUNK]
    w = _as_bf16(wqkv_s[h, m])
    if side_work is not None:
      side_work()
    work[ring(h, m, c * _CHUNK, _CHUNK)] = _dot(xa, w)

  def project_pair(j, side_work):
    untangle(j, 0)
    for m in range(3):
      for p in range(2):
        for c in range(chunks):
          def between(m=m, p=p, c=c):
            if p == 1 and m < 2 and c == 0:
              untangle(j, m + 1)
            side_work((2 * m + p) * chunks + c)

          project_chunk(2 * j + p, m, c, between)

  def first_pairs():
    _wait(x_copies(0) + first_w[0])
    _start(small_copies + first_w[2])
    untangle(0, 0)
    for c in range(chunks):
      if c * _CHUNK == x_rows:
        _wait(x_copies(1))
        _start(pair_copies(1))
      for p in range(2):
        project_chunk(p, 0, c)
    for m in (1, 2):
      _wait(first_w[m])
      _start(pair_copies(2) if m == 1 else pair_copies(3) + x_copies(2))
      untangle(0, m)
      for p in range(2):
        for c in range(chunks):
          project_chunk(p, m, c)
    _wait(small_copies + pair_copies(1))

    def side_work(slot):
      if slot == slots - 1:
        _start(pair_copies(4) + pair_copies(5) + x_copies(3) + x_copies(4)
               + x_copies(5))

    project_pair(1, side_work)

  rounds = heads // 4 - 1
  scoring = rounds - _TOP_C // 2
  pieces = -(-seq // (16 * scoring))
  gate_slots = 2 * slots - 10

  def other_pairs(i, carry):
    _wait(pair_copies(2 * i + 2) + pair_copies(2 * i + 3))
    for n in range(3):
      j = 3 * i + n
      pl.when((j >= 2) & (j < seq // x_rows))(lambda j=j: _wait(x_copies(j)))
    first = jnp.minimum(i * pieces * 16, seq - pieces * 16)
    pages = [area("score", 8 * n, 8) for n in range(seq // (8 * _LANES))]
    score = [work[page] for page in pages]

    def side_work(slot):
      for n in range(pieces):
        if n * gate_slots // pieces == slot:
          gate_and_score(first + 16 * n, score)
      if slot == gate_slots:
        for page, value in zip(pages, score):
          work[page] = value
      for v in range(2):
        if slot == gate_slots + 4 * (v + 1):
          route_next(2 * (i - scoring) + v)
      if slot == 2 * slots - 1:
        pl.when(i + 2 < rounds)(lambda: _start(
            pair_copies(2 * i + 6) + pair_copies(2 * i + 7)))
        pl.when(i == 0)(lambda: _start(x_copies(6) + x_copies(7)))
        pl.when((i >= 1) & (i <= kt // 2))(
            lambda: _start([wo_copy(2 * i - 2), wo_copy(2 * i - 1)]))
        pl.when(i + 2 == rounds)(lambda: _start(ffn_copies(0) + ffn_copies(1)))

    for u in range(2):
      project_pair(2 * i + 2 + u, lambda slot, u=u: side_work(u * slots + slot))
    return carry

  n_small = layout["end"] - layout["score"]
  work[area("score", 0, n_small)] = jnp.zeros((n_small, _LANES), _F32)
  y_s[...] = jnp.zeros(y_s.shape, _F32)
  first_pairs()
  lax.fori_loop(0, rounds, other_pairs, 0)

  def ffn_groups(i):
    x_sel = [work[area("x_sel", k * _TOP_C, _TOP_C)] for k in range(kt)]
    act = {}

    def widen(b, which, part):
      ks = slice(part * kt // 2, (part + 1) * kt // 2)
      w = (wg_s, wu_s)[which][
          i & 1, ks.start * _LANES:ks.stop * _LANES, _block(b)]
      pre_s[b, which, part] = _dot(_cat_cols(x_sel[ks]), w)

    def narrow(b, part):
      if part == 0:
        gate, up = (pre_s[b, n, 0] + pre_s[b, n, 1] for n in range(2))
        act[b] = gate * jax.nn.sigmoid(gate) * up
      cols = slice(part * dm // 2, (part + 1) * dm // 2)
      y_s[:, cols] += _dot(act[b], wd_s[i & 1, _block(b), cols])

    return (
        [functools.partial(widen, b, which, part) for b in range(_FFN_BLOCKS)
         for which in range(2) for part in range(2)]
        + [functools.partial(narrow, b, part) for b in range(_FFN_BLOCKS)
           for part in range(2)])

  def add_ffn():
    keep = jnp.zeros((8, _LANES), _F32)
    for c in range(_TOP_C):
      keep = jnp.where(sub == c, 1.0 - work[area("gate", idx_s[c], 1)], keep)
    keep = keep * jax.nn.sigmoid(work[area("r_sel", 0, _TOP_C)])
    y = [y_s[:, _block(k)] * keep for k in range(kt)]
    for c in range(_TOP_C):
      t0 = pl.multiple_of((idx_s[c] >> 3) * 8, 8)
      hit = sub == (idx_s[c] & 7)
      old = [work[area("mix", k * seq + t0, 8)] for k in range(kt)]
      for k in range(kt):
        new = jnp.where(hit, old[k] + y[k][c:c + 1], old[k])
        work[area("mix", k * seq + t0, 8)] = new
        out_s[pl.ds(t0, 8), _block(k)] = new.astype(_BF16)

  scale = float(_LANES) ** -0.5

  team = _LANES // n_rows
  qi = lax.broadcasted_iota(jnp.int32, (n_rows, _LANES), 0)
  col = lax.broadcasted_iota(jnp.int32, (1, _LANES), 1)
  window = [(col >= c * n_rows) & (col < (c + 1) * n_rows) for c in range(team)]
  ki = col - sum(jnp.where(window[c], c * n_rows, 0) for c in range(team))
  visible = ((qi < n_mem) | (qi >= ki)) & (col < team * n_rows)
  hidden = jnp.where(col < team * n_rows, -1e9, -jnp.inf).astype(_F32)
  teams = ([tuple(range(heads % team))] if heads % team else []) + [
      tuple(range(h, h + team)) for h in range(heads % team, heads, team)]

  def by_window(parts):
    out = parts[-1]
    for c in range(len(parts) - 1):
      out = jnp.where(window[c], parts[c], out)
    return out

  def stack_rows(rows):
    pad = _LANES - sum(r.shape[0] for r in rows)
    return jnp.concatenate(rows + [jnp.zeros((pad, _LANES), _F32)], axis=0)

  def diagonal(tile):
    return stack_rows(
        [jnp.where(window[c], tile[c * n_rows:(c + 1) * n_rows], 0.0)
         for c in range(team)]).astype(_BF16)

  def off_diagonal(keys_t, values, c):
    lo, hi = c * n_rows, (c + 1) * n_rows
    rows = [jnp.where(window[c], keys_t[:lo], 0.0)] if lo else []
    rows += [jnp.where(window[c], 0.0, values[lo:hi]),
             jnp.where(window[c], keys_t[hi:], 0.0)]
    return jnp.concatenate(rows, axis=0).astype(_BF16)

  def step(s, mem, fillers):
    tokens = pl.ds(pl.multiple_of(ahead + s * ride, 8), ride)
    lhs = [
        jnp.concatenate([mem[k], x_s[tokens, _block(k)].astype(_F32)], axis=0
                        ).astype(_BF16) for k in range(kt)]
    put = [lax.rem(ahead + s * ride + 8 * i, ring_rows)
           for i in range(ride // 8)]
    get = lax.rem(s * seg, ring_rows)
    qkv, probs = {}, {}

    def project_part(h, k0, k1):
      words = slice(k0 * _LANES // 2, k1 * _LANES // 2)
      w = _cat_cols([_as_bf16(wqkv_s[h, m, words]) for m in range(3)])
      return _dot(_cat_cols(lhs[k0:k1]), w)

    def project(h):
      if h == 0:
        part_s[...] = project_part(h, 0, kt // 2)
        r = part_s[...] + project_part(h, kt // 2, kt)
      else:
        r = project_part(h, 0, kt)
      for m in range(3):
        for i in range(ride // 8):
          work[ring(h, m, put[i], 8)] = r[
              n_mem + 8 * i:n_mem + 8 * i + 8, _block(m)]
      qkv[h] = [r[0:n_mem, _block(m)] for m in range(3)]

    def fetch(h, m):
      return jnp.concatenate([qkv[h][m], work[ring(h, m, get, seg)]], axis=0)

    queries, keys_t, values = {}, {}, {}

    def softmax(t, sc):
      sc = jnp.where(visible, sc * scale, hidden)
      members = window[:len(teams[t])]
      top = [jnp.max(jnp.where(w, sc, -jnp.inf), axis=-1, keepdims=True)
             for w in members]
      p = jnp.exp(sc - by_window(top))
      probs[t] = (p, [jnp.sum(jnp.where(w, p, 0.0), axis=-1, keepdims=True)
                      for w in members])

    def emit(t, outs):
      for h, o, denom in zip(teams[t], outs, probs[t][1]):
        inv = pltpu.reciprocal(denom, approx=True)
        o_s[:, _block(h)] = o * (inv * (2.0 - denom * inv))

    def attend(t):
      if 1 <= t < len(teams) and len(teams[t - 1]) == team:
        p = probs[t - 1][0]
        o_inside = _dot(p, diagonal(values[t - 1]))
        both = [_dot(jnp.where(window[c], p, queries[t][c]),
                     off_diagonal(keys_t[t], values[t - 1], c))
                for c in range(team)]
        sc_inside = _dot(by_window(queries[t]), diagonal(keys_t[t]))
        softmax(t, by_window(both) + sc_inside)
        emit(t - 1,
             [jnp.where(window[c], o_inside, both[c]) for c in range(team)])
        return
      if t < len(teams):
        k = keys_t[t].astype(_BF16)
        softmax(t, by_window([_dot(q, k) for q in queries[t]]))
      if t >= 1:
        v = values[t - 1].astype(_BF16)
        emit(t - 1, [_dot(jnp.where(w, probs[t - 1][0], 0.0), v)
                     for w in window[:len(teams[t - 1])]])

    acc, done = None, 0

    def out_project(n):
      nonlocal acc, done
      lo, hi = done * _LANES, (done + n) * _LANES
      w = _cat_cols([_as_bf16(wo_s[k, lo // 2:hi // 2]) for k in range(kt)])
      r = _dot(o_s[:, lo:hi], w)
      acc = r if acc is None else acc + r
      done += n

    ends = {members[-1]: t for t, members in enumerate(teams)}
    for h in range(heads + team + _LAG_ATTEND):
      if h < heads:
        project(h)
      if h in ends:
        t = ends[h]
        keys_t[t] = stack_rows([fetch(n, 1) for n in teams[t]]).T
      if h - _LAG_FETCH_Q in ends:
        t = ends[h - _LAG_FETCH_Q]
        queries[t] = [fetch(n, 0) for n in teams[t]]
      if h - _LAG_FETCH_V in ends:
        t = ends[h - _LAG_FETCH_V]
        values[t] = stack_rows([fetch(n, 2) for n in teams[t]])
      if h >= heads:
        out_project(_OUT_HEADS)
      if h - _LAG_ATTEND in ends:
        attend(ends[h - _LAG_ATTEND])
    attend(len(teams))
    assert len(fillers) <= _OUT_EXTRA
    for n in range(_OUT_EXTRA):
      out_project(_OUT_HEADS)
      if n < len(fillers):
        fillers[n]()
    out_project(heads - done)

    g = work[area("gate", s * seg, seg)]
    rows = pl.ds(pl.multiple_of(s * seg, seg), seg)
    for k in range(kt):
      mix = area("mix", k * seq + s * seg, seg)
      mixed = g * acc[n_mem:, _block(k)] + work[mix]
      work[mix] = mixed
      out_s[rows, _block(k)] = mixed.astype(_BF16)
    return [acc[0:n_mem, _block(k)] for k in range(kt)]

  def steps(i, carry):
    pl.when(i < ffn_iters)(lambda: _wait(ffn_copies(i)))

    @pl.when(i == ffn_iters)
    def _():
      add_ffn()
      out_copy(0, ffn_iters * _UNROLL).start()

    groups = ffn_groups(i)
    per_step = len(groups) // _UNROLL
    mem = [mem_s[:, _block(k)] for k in range(kt)]
    for u in range(_UNROLL):
      mem = step(i * _UNROLL + u, mem, groups[u * per_step:(u + 1) * per_step])
    mem_s[...] = _cat_cols(mem)
    pl.when(i + 2 < ffn_iters)(lambda: _start(ffn_copies(i + 2)))
    pl.when(i >= ffn_iters)(lambda: out_copy(i * _UNROLL, _UNROLL).start())
    return carry

  mem_s[...] = mem0_s[...].astype(_F32)
  _wait([wo_copy(n) for n in range(kt)])
  lax.fori_loop(0, n_seg // _UNROLL, steps, 0)
  pltpu.make_async_copy(out_s, out_hbm, sem_out).wait()


@functools.partial(jax.jit, static_argnames=("A_seg_len",))
def pallas_gated_mix__memory_aug_recurrent_mem_tr__moe_arch_mod__prompt_kernel(
    A_x: jax.Array,
    A_mem0: jax.Array,
    A_Wq: jax.Array,
    A_Wk: jax.Array,
    A_Wv: jax.Array,
    A_Wo: jax.Array,
    A_seg_len: int,
    B_x: jax.Array,
    B_w_r: jax.Array,
    B_w_gate: jax.Array,
    B_w_up: jax.Array,
    B_w_down: jax.Array,
    gate_w: jax.Array,
):
  del B_x
  batch, seq, dm = A_x.shape
  _, heads, dh = A_Wq.shape
  n_mem = A_mem0.shape[1]
  seg = int(A_seg_len)
  assert (batch, seq, dm, heads, dh) == (1, 2048, 1024, 32, _LANES)
  assert (n_mem, seg, B_w_down.shape[0]) == (8, 32, 3584)
  kt = dm // _LANES
  ring_rows = seq // 4 + seg
  width = _FFN_BLOCKS * _LANES

  hbm = pl.BlockSpec(memory_space=pl.ANY)
  out = pl.pallas_call(
      functools.partial(_kernel, heads=heads, seg=seg, ring_rows=ring_rows),
      out_shape=jax.ShapeDtypeStruct((seq, dm), A_x.dtype),
      in_specs=[hbm] * 11,
      out_specs=hbm,
      scratch_shapes=[
          pltpu.VMEM((seq, dm), _BF16),
          pltpu.VMEM((heads, 3, dm // 2, _LANES), _U32),
          pltpu.VMEM((kt, heads * dh // 2, _LANES), _U32),
          pltpu.VMEM((2, dm, width), _BF16),
          pltpu.VMEM((2, dm, width), _BF16),
          pltpu.VMEM((2, width, dm), _BF16),
          pltpu.VMEM((seq, dm), _BF16),
          pltpu.VMEM(
              (_work_layout(seq, kt, heads, ring_rows)["end"], _LANES), _F32),
          pltpu.VMEM((n_mem + seg, heads * dh), _F32),
          pltpu.VMEM((n_mem, dm), _F32),
          pltpu.VMEM((seg, 3 * _LANES), _F32),
          pltpu.VMEM((_FFN_BLOCKS, 2, 2, _TOP_C, _LANES), _F32),
          pltpu.VMEM((_TOP_C, dm), _F32),
          pltpu.VMEM((n_mem, dm), _BF16),
          pltpu.VMEM((kt, _LANES), _BF16),
          pltpu.VMEM((kt, _LANES), _BF16),
          pltpu.SMEM((_TOP_C,), jnp.int32),
          pltpu.SemaphoreType.DMA((8,)),
          pltpu.SemaphoreType.DMA((6,)),
          pltpu.SemaphoreType.DMA((4,)),
          pltpu.SemaphoreType.DMA,
      ],
      compiler_params=pltpu.CompilerParams(
          vmem_limit_bytes=100 * 2**20,
          disable_bounds_checks=True,
          disable_semaphore_checks=True,
      ),
      name="gated_rmt_mod",
  )(
      A_x.reshape(seq, dm),
      A_mem0.reshape(n_mem, dm),
      A_Wq.reshape(dm // 2, 2, heads, dh),
      A_Wk.reshape(dm // 2, 2, heads, dh),
      A_Wv.reshape(dm // 2, 2, heads, dh),
      A_Wo.reshape(heads * dh, dm),
      B_w_r.reshape(kt, _LANES),
      B_w_gate,
      B_w_up,
      B_w_down,
      gate_w.reshape(kt, _LANES),
  )
  return out.reshape(batch, seq, dm)
```
